```python
import jax
import jax.numpy as jnp

def _softmax(x, axis=-1):
    return jax.nn.softmax(x, axis=axis)
def _gelu(x):
    return jax.nn.gelu(x, approximate=True)
def _silu(x):
    return jax.nn.silu(x)
def _sigmoid(x):
    return jax.nn.sigmoid(x)
def _layernorm(x, axis=-1, eps=1e-5):
    m = jnp.mean(x, axis=axis, keepdims=True)
    v = jnp.var(x, axis=axis, keepdims=True)
    return (x - m) / jnp.sqrt(v + eps)
def _scatter_add(tgt, idx, src, axis=0):
    return tgt.at[idx].add(src)
def _segment_sum(src, seg, n):
    return jax.ops.segment_sum(src, seg, n)
class _Rng:
    def __init__(self, key):
        self._k = key
    def _next(self):
        self._k, sub = jax.random.split(self._k)
        return sub
    def normal(self, shape):
        return jax.random.normal(self._next(), shape, dtype=jnp.bfloat16)
    def randint(self, lo, hi, shape):
        return jax.random.randint(self._next(), shape, lo, hi, dtype=jnp.int32)
    def uniform(self, shape, lo=0.0, hi=1.0):
        return jax.random.uniform(self._next(), shape, jnp.bfloat16, lo, hi)
    def permutation(self, n):
        return jax.random.permutation(self._next(), n)


kernel_name = 'interleave_layers__compressed_kv_cla__moe_arch_mod__decode'

def setup_inputs():
    _rng = _Rng(jax.random.key(int.from_bytes(__import__("os").urandom(4), "little")))
    _w = (lambda a: (lambda t: t.astype(jnp.bfloat16) if jnp.issubdtype(t.dtype, jnp.floating) else t)(jnp.asarray(a)))
    def _A_setup():
        B, H, Sq, Sk, D, M = 1, 32, 1, 4096, 128, 640
        Dc = 4 * D
        return {
            "x": _w((lambda *s: _rng.normal(s) * 0.05)(B, Sq, M)),
            "c_kv": _w((lambda *s: _rng.normal(s) * 0.05)(B, Sk, Dc)),
            "w_q": _w((lambda *s: _rng.normal(s) * 0.05)(M, H, D) * (M ** -0.5)),
            "w_uk": _w((lambda *s: _rng.normal(s) * 0.05)(Dc, H, D) * (Dc ** -0.5)),
            "w_uv": _w((lambda *s: _rng.normal(s) * 0.05)(Dc, H, D) * (Dc ** -0.5)),
            "w_o": _w((lambda *s: _rng.normal(s) * 0.05)(H, D, M) * ((H * D) ** -0.5)),
        }
    _A_in = _A_setup()

    def _B_setup():
        B, S, D, F, C = 1, 1, 640, 1728, 1
        return {
            "x": _w((lambda *s: _rng.normal(s) * 0.05)(B, S, D)),
            "w_r": _w((lambda *s: _rng.normal(s) * 0.05)(D)),
            "w_gate": _w((lambda *s: _rng.normal(s) * 0.05)(D, F)),
            "w_up": _w((lambda *s: _rng.normal(s) * 0.05)(D, F)),
            "w_down": _w((lambda *s: _rng.normal(s) * 0.05)(F, D)),
        }
    _B_in = _B_setup()

    return {
        "A_x": _A_in["x"],
        "A_c_kv": _A_in["c_kv"],
        "A_w_q": _A_in["w_q"],
        "A_w_uk": _A_in["w_uk"],
        "A_w_uv": _A_in["w_uv"],
        "A_w_o": _A_in["w_o"],
        "B_x": _B_in["x"],
        "B_w_r": _B_in["w_r"],
        "B_w_gate": _B_in["w_gate"],
        "B_w_up": _B_in["w_up"],
        "B_w_down": _B_in["w_down"],
    }

def reference(A_x, A_c_kv, A_w_q, A_w_uk, A_w_uv, A_w_o, B_x, B_w_r, B_w_gate, B_w_up, B_w_down):
    def _A_ref(x, c_kv, w_q, w_uk, w_uv, w_o):
        B, Sq, M = x.shape[0], x.shape[1], x.shape[2]
        Sk = c_kv.shape[1]
        H, D = w_q.shape[1], w_q.shape[2]
        q = jnp.einsum("bqm,mhd->bhqd", x, w_q)
        k = jnp.einsum("bkc,chd->bhkd", c_kv, w_uk)
        v = jnp.einsum("bkc,chd->bhkd", c_kv, w_uv)
        scores = jnp.einsum("bhqd,bhkd->bhqk", q, k) * (D ** -0.5)
        off = Sk - Sq
        qi = jnp.arange(Sq)[:, None]
        kj = jnp.arange(Sk)[None, :]
        cmask = kj <= (qi + off)
        scores = jnp.where(cmask[None, None], scores, -1e9)
        p = _softmax(scores, axis=-1)
        ctx = jnp.einsum("bhqk,bhkd->bhqd", p, v)
        return jnp.einsum("bhqd,hdm->bqm", ctx, w_o)

    def _B_ref(x, w_r, w_gate, w_up, w_down):
        B, S, D = x.shape
        C = 1
        r = x @ w_r
        idx = jnp.argsort(-r, axis=-1)[:, :C]
        idx_e = jnp.repeat(idx.reshape(B, C, 1), D, axis=2)
        x_sel = jnp.take_along_axis(x, idx_e, axis=1)
        g = _silu(x_sel @ w_gate)
        u = x_sel @ w_up
        y = (g * u) @ w_down
        r_sel = _sigmoid(jnp.take_along_axis(r, idx, axis=1))
        y = y * r_sel.reshape(B, C, 1)
        b_off = (jnp.arange(B) * S).reshape(B, 1)
        flat_idx = (idx + b_off).reshape(B * C)
        zero = (x * 0.0).reshape(B * S, D)
        upd = _scatter_add(zero, flat_idx, y.reshape(B * C, D), axis=0)
        return x + upd.reshape(B, S, D)

    x = A_x
    x = x + _A_ref(_layernorm(x, axis=-1), A_c_kv, A_w_q, A_w_uk, A_w_uv, A_w_o)
    x = x + _B_ref(_layernorm(x, axis=-1), B_w_r, B_w_gate, B_w_up, B_w_down)
    x = x + _A_ref(_layernorm(x, axis=-1), A_c_kv, A_w_q, A_w_uk, A_w_uv, A_w_o)
    x = x + _B_ref(_layernorm(x, axis=-1), B_w_r, B_w_gate, B_w_up, B_w_down)
    return x
```

```python
import functools

import jax
import jax.numpy as jnp
from jax import lax
from jax.experimental import pallas as pl
from jax.experimental.pallas import tpu as pltpu

M = 640
H = 32
D = 128
DC = 512
SK = 4096
F = 1728
FP = 1792
NFB = FP // 128
EPS = 1e-5

SQ = 322
SV = 258

BF = jnp.bfloat16
F32 = jnp.float32
U32 = jnp.uint32


def _bf(u32_val):
    return pltpu.bitcast(u32_val, BF)


def _u32(bf_val):
    return pltpu.bitcast(bf_val, U32)


def _dup(v8):
    return jnp.concatenate([v8, v8], axis=0).astype(BF)


def _dot(a, b):
    return jnp.dot(a, b, preferred_element_type=F32)


def _dot_nt(a, b):
    return lax.dot_general(a, b, (((1,), (1,)), ((), ())), preferred_element_type=F32)


def _layernorm(x8):
    mean = jnp.sum(x8, axis=1, keepdims=True) * (1.0 / M)
    xc = x8 - mean
    var = jnp.sum(xc * xc, axis=1, keepdims=True) * (1.0 / M)
    return xc * lax.rsqrt(var + EPS)


def _eye():
    r = lax.broadcasted_iota(jnp.int32, (128, 128), 0)
    c = lax.broadcasted_iota(jnp.int32, (128, 128), 1)
    return jnp.where(r == c, 1.0, 0.0).astype(BF)


def _transpose_tile(eye, tile):
    return _u32(_dot_nt(eye, tile).astype(BF))


def _chunks():
    ch = []
    ch += [("wq", i * 128, 128) for i in range(5)]
    ch += [("wuk", i * 128, 128) for i in range(4)]
    ch += [("ckv", i * 1024, 1024) for i in range(4)]
    ch += [("wg", 0, 512), ("wg", 512, 512), ("wg", 1024, 704)]
    ch += [("wu", 0, 512), ("wu", 512, 512), ("wu", 1024, 704)]
    ch += [("wuv", i * 128, 128) for i in range(4)]
    ch += [("wo", i * 1024, 1024) for i in range(4)]
    ch += [("wd", 0, 512), ("wd", 512, 512), ("wd", 1024, 384), ("wd", 1408, 320)]
    return ch


CHUNKS = _chunks()
NCH = len(CHUNKS)
WINDOW = 4


def _kernel(x_hbm, ckv_hbm, wq_hbm, wuk_hbm, wuv_hbm, wo_hbm, wr_hbm, wg_hbm, wu_hbm, wd_hbm,
            o_ref,
            x_s, wr_s, wq_n, wuk_n, wuv_n, ckv_n, wo_n, wg_n, wu_n, wd_n,
            WQ, UP, UT, UV, CKT, CK, GT, UPT, QD, CL,
            sems, small_sems):
    hbm = dict(wq=wq_hbm, wuk=wuk_hbm, wuv=wuv_hbm, wo=wo_hbm, wg=wg_hbm, wu=wu_hbm, wd=wd_hbm,
               ckv=ckv_hbm.at[0])
    vm = dict(wq=wq_n, wuk=wuk_n, wuv=wuv_n, wo=wo_n, wg=wg_n, wu=wu_n, wd=wd_n, ckv=ckv_n)

    def chunk_copy(i):
        name, r0, n = CHUNKS[i]
        if name == "wo":
            src = hbm[name].at[pl.ds(r0 // 128, n // 128)]
            dst = vm[name].at[pl.ds(r0 // 128, n // 128)]
        else:
            src = hbm[name].at[pl.ds(r0, n)]
            dst = vm[name].at[pl.ds(r0, n)]
        return pltpu.make_async_copy(src, dst, sems.at[i])

    state = {"next": 0}

    def issue(upto):
        while state["next"] < min(upto, NCH):
            chunk_copy(state["next"]).start()
            state["next"] += 1

    def wait(i):
        chunk_copy(i).wait()
        issue(i + 1 + WINDOW)

    def idx(name):
        return [i for i, c in enumerate(CHUNKS) if c[0] == name]

    issue(1)
    cx = pltpu.make_async_copy(x_hbm, x_s, small_sems.at[0])
    cr = pltpu.make_async_copy(wr_hbm, wr_s, small_sems.at[1])
    cx.start()
    cr.start()
    issue(WINDOW)
    wd_n[pl.ds(F, FP - F), :] = jnp.zeros((FP - F, M), BF)

    def repack(src_n, dst, stride, j0, nj):
        def body(j, c):
            a = _u32(src_n[2 * j])
            b = _u32(src_n[2 * j + 1])
            lo = (a & jnp.uint32(0xFFFF)) | (b << 16)
            hi = (a >> 16) | (b & jnp.uint32(0xFFFF0000))
            dst[pl.ds(j, 16, stride=2 * stride), :] = lo
            dst[pl.ds(stride + j, 16, stride=2 * stride), :] = hi
            return c
        lax.fori_loop(j0, j0 + nj, body, 0, unroll=4)

    def prep_wuk_transpose(cb):
        eye = _eye()

        def body(h, c):
            tile = _bf(UP[pl.ds(h * SV + cb * 64, 64), :])
            UT[pl.ds((cb * H + h) * 64, 64), :] = _transpose_tile(eye, tile)
            return c
        lax.fori_loop(0, H, body, 0, unroll=4)

    def prep_ckv(kb0, nkb):
        eye = _eye()

        def body(kb, c):
            r0 = pl.multiple_of(kb * 128, 128)
            for cb in range(4):
                tile = ckv_n[pl.ds(r0, 128), pl.ds(cb * 128, 128)]
                CK[pl.ds(cb * 2048 + kb * 64, 64), :] = _u32(tile)
                CKT[pl.ds((kb * 4 + cb) * 64, 64), :] = _transpose_tile(eye, tile)
            return c
        lax.fori_loop(kb0, kb0 + nkb, body, 0)

    def prep_ffn(src_n, dst, r0, n):
        eye = _eye()
        nfull = n // 128

        def body(nb, c):
            row = pl.multiple_of(nb * 128, 128)
            for kb in range(5):
                tile = src_n[pl.ds(row, 128), pl.ds(kb * 128, 128)]
                dst[pl.ds((nb * 5 + kb) * 64, 64), :] = _transpose_tile(eye, tile)
            return c
        lax.fori_loop(r0 // 128, r0 // 128 + nfull, body, 0)
        if n % 128:
            nb = r0 // 128 + nfull
            for kb in range(5):
                half = src_n[pl.ds(nb * 128, 64), pl.ds(kb * 128, 128)]
                tile = jnp.concatenate([half, jnp.zeros((64, 128), BF)], axis=0)
                dst[pl.ds((nb * 5 + kb) * 64, 64), :] = _transpose_tile(eye, tile)

    sub = lax.broadcasted_iota(jnp.int32, (8, 128), 0)

    def stage_q(xd):
        for h in range(H):
            w = _bf(WQ[pl.ds(h * SQ, 320), :])
            r = _dot(xd, w)[0:8] * (D ** -0.5)
            QD[pl.ds(h * 8, 8), :] = _u32(_dup(r))

    def stage_qabs():
        qa = []
        for cb in range(4):
            acc = [jnp.zeros((8, 128), F32) for _ in range(4)]
            for h in range(H):
                qd = _bf(QD[pl.ds(h * 8, 8), :])
                w = _bf(UT[pl.ds((cb * H + h) * 64, 64), :])
                r = _dot(qd, w)[0:8]
                acc[h // 8] = jnp.where(sub == h % 8, r, acc[h // 8])
            qa.append(jnp.concatenate(acc, axis=0).astype(BF))
        return jnp.concatenate(qa, axis=1)

    def scores(qa, nb0, nnb):
        return jnp.concatenate(
            [_dot(qa, _bf(CKT[pl.ds(nb * 256, 256), :])) for nb in range(nb0, nb0 + nnb)], axis=1)

    def pv(p, kb0, nkb):
        return jnp.concatenate(
            [_dot(p, _bf(CK[pl.ds(cb * 2048 + kb0 * 64, nkb * 64), :])) for cb in range(4)], axis=1)

    def stage_attn(qa):
        sa = scores(qa, 0, 16)
        sb = scores(qa, 16, 16)
        ma = jnp.max(sa, axis=1, keepdims=True)
        pa = jnp.exp(sa - ma)
        la = jnp.sum(pa, axis=1, keepdims=True)
        ca = pv(pa.astype(BF), 0, 16)
        m = jnp.maximum(ma, jnp.max(sb, axis=1, keepdims=True))
        pb = jnp.exp(sb - m)
        lb = jnp.sum(pb, axis=1, keepdims=True)
        cbv = pv(pb.astype(BF), 16, 16)
        alpha = jnp.exp(ma - m)
        inv = 1.0 / (alpha * la + lb)
        cl = (alpha * ca + cbv) * inv
        bits = pltpu.bitcast(cl.astype(BF).astype(F32), U32)
        dupw = bits | (bits >> 16)
        for cb in range(4):
            CL[pl.ds(cb * H, H), :] = dupw[:, cb * 128:(cb + 1) * 128]

    def stage_ctx():
        for h in range(H):
            lhs = jnp.concatenate(
                [_bf(CL[pl.ds(cb * H + h, 8, stride=0), :]) for cb in range(4)], axis=1)
            r = _dot(lhs, _bf(UV[pl.ds(h * SV, 256), :]))[0:8]
            QD[pl.ds(h * 8, 8), :] = _u32(_dup(r))

    def stage_out(h0, nh, acc):
        for h in range(h0, h0 + nh):
            acc = acc + _dot(_bf(QD[pl.ds(h * 8, 8), :]), wo_n[h])[0:8]
        return acc

    def stage_gate_up(xd):
        hd = []
        for nb in range(NFB):
            g = _dot(xd, _bf(GT[pl.ds(nb * 320, 320), :]))[0:8]
            u = _dot(xd, _bf(UPT[pl.ds(nb * 320, 320), :]))[0:8]
            hd.append(_dup(g * jax.nn.sigmoid(g) * u))
        return hd

    def stage_down(hd, nb0, nb1, acc):
        for nb in range(nb0, nb1):
            acc = acc + _dot(hd[nb], wd_n[pl.ds(nb * 128, 128), :])[0:8]
        return acc

    def gate_scalar(xn, wr8):
        r = jnp.sum(xn * wr8, axis=1, keepdims=True)
        return jax.nn.sigmoid(r)

    cx.wait()
    cr.wait()
    x = jnp.broadcast_to(x_s[0].astype(F32), (8, M))
    wr8 = jnp.broadcast_to(wr_s[...].reshape(1, M).astype(F32), (8, M))

    for k, i in enumerate(idx("wq")):
        wait(i)
        repack(wq_n, WQ, SQ, k * 64, 64)
    xn = _layernorm(x)
    stage_q(_dup(xn))
    for k, i in enumerate(idx("wuk")):
        wait(i)
        repack(wuk_n, UP, SV, k * 64, 64)
        prep_wuk_transpose(k)
    qa = stage_qabs()
    for k, i in enumerate(idx("ckv")):
        wait(i)
        prep_ckv(k * 8, 8)
    stage_attn(qa)
    for i in idx("wg"):
        wait(i)
        prep_ffn(wg_n, GT, CHUNKS[i][1], CHUNKS[i][2])
    for i in idx("wu"):
        wait(i)
        prep_ffn(wu_n, UPT, CHUNKS[i][1], CHUNKS[i][2])
    for k, i in enumerate(idx("wuv")):
        wait(i)
        repack(wuv_n, UV, SV, k * 64, 64)
    stage_ctx()
    acc = jnp.zeros((8, M), F32)
    for k, i in enumerate(idx("wo")):
        wait(i)
        acc = stage_out(k * 8, 8, acc)
    x = x + acc
    xn = _layernorm(x)
    hd = stage_gate_up(_dup(xn))
    sg = gate_scalar(xn, wr8)
    acc = jnp.zeros((8, M), F32)
    for i in idx("wd"):
        wait(i)
        r0, n = CHUNKS[i][1], CHUNKS[i][2]
        acc = stage_down(hd, r0 // 128, -(-(r0 + n) // 128), acc)
    x = x + xn + acc * sg

    xn = _layernorm(x)
    stage_q(_dup(xn))
    qa = stage_qabs()
    stage_attn(qa)
    stage_ctx()
    x = x + stage_out(0, H, jnp.zeros((8, M), F32))
    xn = _layernorm(x)
    hd = stage_gate_up(_dup(xn))
    sg = gate_scalar(xn, wr8)
    x = x + xn + stage_down(hd, 0, NFB, jnp.zeros((8, M), F32)) * sg

    o_ref[0] = x[0:1].astype(BF)


@jax.jit
def pallas_interleave_layers__compressed_kv_cla__moe_arch_mod__decode_kernel(
    A_x: jax.Array,
    A_c_kv: jax.Array,
    A_w_q: jax.Array,
    A_w_uk: jax.Array,
    A_w_uv: jax.Array,
    A_w_o: jax.Array,
    B_x: jax.Array,
    B_w_r: jax.Array,
    B_w_gate: jax.Array,
    B_w_up: jax.Array,
    B_w_down: jax.Array,
):
    del B_x
    any_spec = pl.BlockSpec(memory_space=pl.ANY)
    scratch = [
        pltpu.VMEM((1, 1, M), BF),
        pltpu.VMEM((M,), BF),
        pltpu.VMEM((M, H, D), BF),
        pltpu.VMEM((DC, H, D), BF),
        pltpu.VMEM((DC, H, D), BF),
        pltpu.VMEM((SK, DC), BF),
        pltpu.VMEM((H, D, M), BF),
        pltpu.VMEM((F, M), BF),
        pltpu.VMEM((F, M), BF),
        pltpu.VMEM((FP, M), BF),
        pltpu.VMEM((H * SQ, 128), U32),
        pltpu.VMEM((H * SV, 128), U32),
        pltpu.VMEM((4 * H * 64, 128), U32),
        pltpu.VMEM((H * SV, 128), U32),
        pltpu.VMEM((32 * 4 * 64, 128), U32),
        pltpu.VMEM((4 * 2048, 128), U32),
        pltpu.VMEM((NFB * 320, 128), U32),
        pltpu.VMEM((NFB * 320, 128), U32),
        pltpu.VMEM((H * 8, 128), U32),
        pltpu.VMEM((4 * H, 128), U32),
        pltpu.SemaphoreType.DMA((NCH,)),
        pltpu.SemaphoreType.DMA((2,)),
    ]
    return pl.pallas_call(
        _kernel,
        out_shape=jax.ShapeDtypeStruct((1, 1, M), BF),
        in_specs=[any_spec] * 10,
        out_specs=pl.BlockSpec(memory_space=pltpu.VMEM),
        scratch_shapes=scratch,
        compiler_params=pltpu.CompilerParams(vmem_limit_bytes=100 * 1024 * 1024),
    )(A_x, A_c_kv, A_w_q, A_w_uk, A_w_uv, A_w_o, B_w_r, B_w_gate.T, B_w_up.T, B_w_down)
```

```python
import functools

import jax
import jax.numpy as jnp
from jax import lax
from jax.experimental import pallas as pl
from jax.experimental.pallas import tpu as pltpu

M = 640
H = 32
D = 128
DC = 512
SK = 4096
F = 1728
FP = 1792
NFB = FP // 128
EPS = 1e-5

SQ = 322
SV = 258

BF = jnp.bfloat16
F32 = jnp.float32
U32 = jnp.uint32


def _bf(u32_val):
    return pltpu.bitcast(u32_val, BF)


def _u32(bf_val):
    return pltpu.bitcast(bf_val, U32)


def _dup(v8):
    return jnp.concatenate([v8, v8], axis=0).astype(BF)


def _dot(a, b):
    return jnp.dot(a, b, preferred_element_type=F32)


def _dot_nt(a, b):
    return lax.dot_general(a, b, (((1,), (1,)), ((), ())), preferred_element_type=F32)


def _layernorm(x8):
    mean = jnp.sum(x8, axis=1, keepdims=True) * (1.0 / M)
    xc = x8 - mean
    var = jnp.sum(xc * xc, axis=1, keepdims=True) * (1.0 / M)
    return xc * lax.rsqrt(var + EPS)


def _eye():
    r = lax.broadcasted_iota(jnp.int32, (128, 128), 0)
    c = lax.broadcasted_iota(jnp.int32, (128, 128), 1)
    return jnp.where(r == c, 1.0, 0.0).astype(BF)


def _transpose_tile(eye, tile):
    return _u32(_dot_nt(eye, tile).astype(BF))


def _chunks():
    ch = []
    ch += [("wq", i * 128, 128) for i in range(5)]
    ch += [("wuk", i * 128, 128) for i in range(4)]
    ch += [("ckv", i * 1024, 1024) for i in range(4)]
    ch += [("wg", 0, 512), ("wg", 512, 512), ("wg", 1024, 704)]
    ch += [("wu", 0, 512), ("wu", 512, 512), ("wu", 1024, 704)]
    ch += [("wuv", i * 128, 128) for i in range(4)]
    ch += [("wo", i * 1024, 1024) for i in range(4)]
    ch += [("wd", 0, 512), ("wd", 512, 512), ("wd", 1024, 512), ("wd", 1536, 192)]
    return ch


CHUNKS = _chunks()
NCH = len(CHUNKS)

DEFAULT_CFG = dict(window=64, phase2=True, compute1=True, scopes=False, u_uk=16, u_ckv=4, u_rp=4)


class _NoScope:
    def __enter__(self):
        return self

    def __exit__(self, *a):
        return False


def _kernel(cfg, x_hbm, ckv_hbm, wq_hbm, wuk_hbm, wuv_hbm, wo_hbm, wr_hbm, wg_hbm, wu_hbm, wd_hbm,
            o_ref,
            x_s, wr_s, wq_n, wuk_n, wuv_n, ckv_n, wo_n, wg_n, wu_n, wd_n,
            WQ, UP, UT, UV, CKT, CK, GT, UPT, QD, CL,
            sems):
    hbm = dict(wq=wq_hbm, wuk=wuk_hbm, wuv=wuv_hbm, wo=wo_hbm, wg=wg_hbm, wu=wu_hbm, wd=wd_hbm,
               ckv=ckv_hbm.at[0])
    vm = dict(wq=wq_n, wuk=wuk_n, wuv=wuv_n, wo=wo_n, wg=wg_n, wu=wu_n, wd=wd_n, ckv=ckv_n)

    def chunk_copy(i):
        name, r0, n = CHUNKS[i]
        if name == "wo":
            src = hbm[name].at[pl.ds(r0 // 128, n // 128)]
            dst = vm[name].at[pl.ds(r0 // 128, n // 128)]
        else:
            src = hbm[name].at[pl.ds(r0, n)]
            dst = vm[name].at[pl.ds(r0, n)]
        return pltpu.make_async_copy(src, dst, sems.at[i])

    state = {"next": 0}

    def issue(upto):
        while state["next"] < min(upto, NCH):
            chunk_copy(state["next"]).start()
            state["next"] += 1

    WINDOW = cfg["window"]

    def scope(name):
        return jax.named_scope(name) if cfg["scopes"] else _NoScope()

    def wait(i):
        with scope("wait%02d_%s" % (i, CHUNKS[i][0])):
            chunk_copy(i).wait()
        issue(i + 1 + WINDOW)

    def idx(name):
        return [i for i, c in enumerate(CHUNKS) if c[0] == name]

    cx = pltpu.make_async_copy(x_hbm, x_s, sems.at[NCH])
    cr = pltpu.make_async_copy(wr_hbm, wr_s, sems.at[NCH + 1])
    cx.start()
    cr.start()
    issue(WINDOW)
    wd_n[pl.ds(F, FP - F), :] = jnp.zeros((FP - F, M), BF)

    def repack(src_n, dst, stride, j0, nj):
        def body(j, c):
            a = _u32(src_n[2 * j])
            b = _u32(src_n[2 * j + 1])
            lo = (a & jnp.uint32(0xFFFF)) | (b << 16)
            hi = (a >> 16) | (b & jnp.uint32(0xFFFF0000))
            dst[pl.ds(j, 16, stride=2 * stride), :] = lo
            dst[pl.ds(stride + j, 16, stride=2 * stride), :] = hi
            return c
        lax.fori_loop(j0, j0 + nj, body, 0, unroll=cfg["u_rp"])

    def prep_wuk_transpose(cb):
        eye = _eye()

        def body(h, c):
            tile = _bf(UP[pl.ds(h * SV + cb * 64, 64), :])
            UT[pl.ds((cb * H + h) * 64, 64), :] = _transpose_tile(eye, tile)
            return c
        lax.fori_loop(0, H, body, 0, unroll=cfg["u_uk"])

    def prep_ckv(kb0, nkb):
        eye = _eye()

        def body(kb, c):
            r0 = pl.multiple_of(kb * 128, 128)
            for cb in range(4):
                tile = ckv_n[pl.ds(r0, 128), pl.ds(cb * 128, 128)]
                CK[pl.ds(cb * 2048 + kb * 64, 64), :] = _u32(tile)
                CKT[pl.ds((kb * 4 + cb) * 64, 64), :] = _transpose_tile(eye, tile)
            return c
        lax.fori_loop(kb0, kb0 + nkb, body, 0, unroll=cfg["u_ckv"])

    def prep_ffn(src_n, dst, r0, n):
        eye = _eye()
        nfull = n // 128

        def body(nb, c):
            row = pl.multiple_of(nb * 128, 128)
            for kb in range(5):
                tile = src_n[pl.ds(row, 128), pl.ds(kb * 128, 128)]
                dst[pl.ds((nb * 5 + kb) * 64, 64), :] = _transpose_tile(eye, tile)
            return c
        lax.fori_loop(r0 // 128, r0 // 128 + nfull, body, 0, unroll=True)
        if n % 128:
            nb = r0 // 128 + nfull
            for kb in range(5):
                half = src_n[pl.ds(nb * 128, 64), pl.ds(kb * 128, 128)]
                tile = jnp.concatenate([half, jnp.zeros((64, 128), BF)], axis=0)
                dst[pl.ds((nb * 5 + kb) * 64, 64), :] = _transpose_tile(eye, tile)

    sub = lax.broadcasted_iota(jnp.int32, (8, 128), 0)

    def stage_q(xd):
        for h in range(H):
            w = _bf(WQ[pl.ds(h * SQ, 320), :])
            r = _dot(xd, w)[0:8] * (D ** -0.5)
            QD[pl.ds(h * 8, 8), :] = _u32(_dup(r))

    def stage_qabs():
        qa = []
        for cb in range(4):
            acc = [jnp.zeros((8, 128), F32) for _ in range(4)]
            for h in range(H):
                qd = _bf(QD[pl.ds(h * 8, 8), :])
                w = _bf(UT[pl.ds((cb * H + h) * 64, 64), :])
                r = _dot(qd, w)[0:8]
                acc[h // 8] = jnp.where(sub == h % 8, r, acc[h // 8])
            qa.append(jnp.concatenate(acc, axis=0).astype(BF))
        return jnp.concatenate(qa, axis=1)

    def scores(qa, nb0, nnb):
        return jnp.concatenate(
            [_dot(qa, _bf(CKT[pl.ds(nb * 256, 256), :])) for nb in range(nb0, nb0 + nnb)], axis=1)

    def pv(p, kb0, nkb):
        return jnp.concatenate(
            [_dot(p, _bf(CK[pl.ds(cb * 2048 + kb0 * 64, nkb * 64), :])) for cb in range(4)], axis=1)

    def stage_attn(qa):
        sa = scores(qa, 0, 16)
        sb = scores(qa, 16, 16)
        ma = jnp.max(sa, axis=1, keepdims=True)
        pa = jnp.exp(sa - ma)
        la = jnp.sum(pa, axis=1, keepdims=True)
        ca = pv(pa.astype(BF), 0, 16)
        m = jnp.maximum(ma, jnp.max(sb, axis=1, keepdims=True))
        pb = jnp.exp(sb - m)
        lb = jnp.sum(pb, axis=1, keepdims=True)
        cbv = pv(pb.astype(BF), 16, 16)
        alpha = jnp.exp(ma - m)
        inv = 1.0 / (alpha * la + lb)
        cl = (alpha * ca + cbv) * inv
        bits = pltpu.bitcast(cl.astype(BF).astype(F32), U32)
        dupw = bits | (bits >> 16)
        for cb in range(4):
            CL[pl.ds(cb * H, H), :] = dupw[:, cb * 128:(cb + 1) * 128]

    def stage_ctx():
        for h in range(H):
            lhs = jnp.concatenate(
                [_bf(CL[pl.ds(cb * H + h, 8, stride=0), :]) for cb in range(4)], axis=1)
            r = _dot(lhs, _bf(UV[pl.ds(h * SV, 256), :]))[0:8]
            QD[pl.ds(h * 8, 8), :] = _u32(_dup(r))

    def stage_out(h0, nh, acc):
        for h in range(h0, h0 + nh):
            acc = acc + _dot(_bf(QD[pl.ds(h * 8, 8), :]), wo_n[h])[0:8]
        return acc

    def stage_gate_up(xd):
        hd = []
        for nb in range(NFB):
            g = _dot(xd, _bf(GT[pl.ds(nb * 320, 320), :]))[0:8]
            u = _dot(xd, _bf(UPT[pl.ds(nb * 320, 320), :]))[0:8]
            hd.append(_dup(g * jax.nn.sigmoid(g) * u))
        return hd

    def stage_down(hd, nb0, nb1, acc):
        for nb in range(nb0, nb1):
            acc = acc + _dot(hd[nb], wd_n[pl.ds(nb * 128, 128), :])[0:8]
        return acc

    def gate_scalar(xn, wr8):
        r = jnp.sum(xn * wr8, axis=1, keepdims=True)
        return jax.nn.sigmoid(r)

    cx.wait()
    cr.wait()
    x = jnp.broadcast_to(x_s[0].astype(F32), (8, M))
    wr8 = jnp.broadcast_to(wr_s[...].reshape(1, M).astype(F32), (8, M))

    if not cfg["compute1"]:
        for i in range(NCH):
            wait(i)
        o_ref[0] = x[0:1].astype(BF)
        return

    for k, i in enumerate(idx("wq")):
        wait(i)
        with scope("p_wq"):
            repack(wq_n, WQ, SQ, k * 64, 64)
    with scope("s1_q"):
        xn = _layernorm(x)
        stage_q(_dup(xn))
    for k, i in enumerate(idx("wuk")):
        wait(i)
        with scope("p_wuk"):
            repack(wuk_n, UP, SV, k * 64, 64)
            prep_wuk_transpose(k)
    with scope("s1_qabs"):
        qa = stage_qabs()
    for k, i in enumerate(idx("ckv")):
        wait(i)
        with scope("p_ckv"):
            prep_ckv(k * 8, 8)
    with scope("s1_attn"):
        stage_attn(qa)
    for i in idx("wg"):
        wait(i)
        with scope("p_wg"):
            prep_ffn(wg_n, GT, CHUNKS[i][1], CHUNKS[i][2])
    for i in idx("wu"):
        wait(i)
        with scope("p_wu"):
            prep_ffn(wu_n, UPT, CHUNKS[i][1], CHUNKS[i][2])
    for k, i in enumerate(idx("wuv")):
        wait(i)
        with scope("p_wuv"):
            repack(wuv_n, UV, SV, k * 64, 64)
    with scope("s1_ctx"):
        stage_ctx()
    acc = jnp.zeros((8, M), F32)
    for k, i in enumerate(idx("wo")):
        wait(i)
        with scope("s1_out"):
            acc = stage_out(k * 8, 8, acc)
    with scope("s2_gu"):
        x = x + acc
        xn = _layernorm(x)
        hd = stage_gate_up(_dup(xn))
        sg = gate_scalar(xn, wr8)
    acc = jnp.zeros((8, M), F32)
    for i in idx("wd"):
        wait(i)
        r0, n = CHUNKS[i][1], CHUNKS[i][2]
        with scope("s2_down"):
            acc = stage_down(hd, r0 // 128, -(-(r0 + n) // 128), acc)
    x = x + xn + acc * sg

    if cfg["phase2"]:
        with scope("phase2"):
            xn = _layernorm(x)
            stage_q(_dup(xn))
            qa = stage_qabs()
            stage_attn(qa)
            stage_ctx()
            x = x + stage_out(0, H, jnp.zeros((8, M), F32))
            xn = _layernorm(x)
            hd = stage_gate_up(_dup(xn))
            sg = gate_scalar(xn, wr8)
            x = x + xn + stage_down(hd, 0, NFB, jnp.zeros((8, M), F32)) * sg

    o_ref[0] = x[0:1].astype(BF)


def _run(cfg, A_x, A_c_kv, A_w_q, A_w_uk, A_w_uv, A_w_o, B_w_r, B_w_gate, B_w_up, B_w_down):
    any_spec = pl.BlockSpec(memory_space=pl.ANY)
    scratch = [
        pltpu.VMEM((1, 1, M), BF),
        pltpu.VMEM((M,), BF),
        pltpu.VMEM((M, H, D), BF),
        pltpu.VMEM((DC, H, D), BF),
        pltpu.VMEM((DC, H, D), BF),
        pltpu.VMEM((SK, DC), BF),
        pltpu.VMEM((H, D, M), BF),
        pltpu.VMEM((F, M), BF),
        pltpu.VMEM((F, M), BF),
        pltpu.VMEM((FP, M), BF),
        pltpu.VMEM((H * SQ, 128), U32),
        pltpu.VMEM((H * SV, 128), U32),
        pltpu.VMEM((4 * H * 64, 128), U32),
        pltpu.VMEM((H * SV, 128), U32),
        pltpu.VMEM((32 * 4 * 64, 128), U32),
        pltpu.VMEM((4 * 2048, 128), U32),
        pltpu.VMEM((NFB * 320, 128), U32),
        pltpu.VMEM((NFB * 320, 128), U32),
        pltpu.VMEM((H * 8, 128), U32),
        pltpu.VMEM((4 * H, 128), U32),
        pltpu.SemaphoreType.DMA((NCH + 2,)),
    ]
    return pl.pallas_call(
        functools.partial(_kernel, cfg),
        out_shape=jax.ShapeDtypeStruct((1, 1, M), BF),
        in_specs=[any_spec] * 10,
        out_specs=pl.BlockSpec(memory_space=pltpu.VMEM),
        scratch_shapes=scratch,
        compiler_params=pltpu.CompilerParams(vmem_limit_bytes=100 * 1024 * 1024),
    )(A_x, A_c_kv, A_w_q, A_w_uk, A_w_uv, A_w_o, B_w_r, B_w_gate.T, B_w_up.T, B_w_down)


def build(**overrides):
    cfg = dict(DEFAULT_CFG, **overrides)

    @jax.jit
    def fn(A_x, A_c_kv, A_w_q, A_w_uk, A_w_uv, A_w_o, B_x, B_w_r, B_w_gate, B_w_up, B_w_down):
        return _run(cfg, A_x, A_c_kv, A_w_q, A_w_uk, A_w_uv, A_w_o, B_w_r, B_w_gate, B_w_up, B_w_down)
    return fn


@jax.jit
def pallas_interleave_layers__compressed_kv_cla__moe_arch_mod__decode_kernel(
    A_x: jax.Array,
    A_c_kv: jax.Array,
    A_w_q: jax.Array,
    A_w_uk: jax.Array,
    A_w_uv: jax.Array,
    A_w_o: jax.Array,
    B_x: jax.Array,
    B_w_r: jax.Array,
    B_w_gate: jax.Array,
    B_w_up: jax.Array,
    B_w_down: jax.Array,
):
    del B_x
    return _run(DEFAULT_CFG, A_x, A_c_kv, A_w_q, A_w_uk, A_w_uv, A_w_o, B_w_r, B_w_gate, B_w_up,
                B_w_down)
```

```python
import functools

import jax
import jax.numpy as jnp
from jax import lax
from jax.experimental import pallas as pl
from jax.experimental.pallas import tpu as pltpu

M = 640
H = 32
D = 128
DC = 512
SK = 4096
F = 1728
EPS = 1e-5

SQ = 322
SP = 9
SV = 258

BF = jnp.bfloat16
F32 = jnp.float32
U32 = jnp.uint32


def _bf(u32_val):
    return pltpu.bitcast(u32_val, BF)


def _u32(bf_val):
    return pltpu.bitcast(bf_val, U32)


def _dup(v8):
    return jnp.concatenate([v8, v8], axis=0).astype(BF)


def _dot(a, b):
    return jnp.dot(a, b, preferred_element_type=F32)


def _dot_nt(a, b):
    return lax.dot_general(a, b, (((1,), (1,)), ((), ())), preferred_element_type=F32)


def _split(v8):
    hi = pltpu.bitcast(pltpu.bitcast(v8, U32) & jnp.uint32(0xFFFF0000), F32)
    return jnp.concatenate([hi, v8 - hi], axis=0).astype(BF)


def _dot2(a16, b):
    r = _dot(a16, b)
    return r[0:8] + r[8:16]


def _ln_stats(x8):
    s1 = jnp.sum(x8, axis=1, keepdims=True)
    s2 = jnp.sum(x8 * x8, axis=1, keepdims=True)
    mean = s1 * (1.0 / M)
    var = jnp.maximum(s2 * (1.0 / M) - mean * mean, 0.0)
    return mean, lax.rsqrt(var + EPS)


def _swiglu(g, u):
    a = 0.5 * g
    b = a * u
    return b * jnp.tanh(a) + b


def _lane_blocks_sum(p):
    n = p.shape[1] // 128
    acc = p[:, 0:128]
    for i in range(1, n):
        acc = acc + p[:, i * 128:(i + 1) * 128]
    return acc


def _row_total(a8):
    return jnp.broadcast_to(jnp.sum(a8, axis=0, keepdims=True), a8.shape)


def _eye():
    r = lax.broadcasted_iota(jnp.int32, (128, 128), 0)
    c = lax.broadcasted_iota(jnp.int32, (128, 128), 1)
    return jnp.where(r == c, 1.0, 0.0).astype(BF)


def _transpose_tile(eye, tile):
    return _u32(_dot_nt(eye, tile).astype(BF))


def _chunks(cfg):
    fm = cfg["fm"]
    nm = cfg["nm"]
    ch = []
    ch += [("wq", i * 128, 128) for i in range(5)]
    ch += [("wuk", i * 128, 128) for i in range(4)]
    ch += [("ckv", i * 1024, 1024) for i in range(4)]
    ch += [("wuv", i * 128, 128) for i in range(4)]
    ch += [("wo", h0, min(8, H - h0)) for h0 in range(nm, H, 8)]
    ch += [("wo", h0, min(8, nm - h0)) for h0 in range(0, nm, 8)]
    for name in ("wg", "wu"):
        ch += [(name, fm, F - fm)]
        ch += [(name, r0, min(512, fm - r0)) for r0 in range(0, fm, 512)]
    ch += [("wd", fm, F - fm)]
    r0 = 0
    while r0 < fm - 128:
        n = min(512, fm - 128 - r0)
        ch.append(("wd", r0, n))
        r0 += n
    ch.append(("wd", fm - 128, 128))
    return ch


DEFAULT_CFG = dict(phase2=True, compute1=True, scopes=False, u_uk=16, u_ckv=4, u_rp=4,
                   nm=16, fm=1024)


class _NoScope:
    def __enter__(self):
        return self

    def __exit__(self, *a):
        return False


def _kernel(cfg, x_hbm, ckv_hbm, wq_hbm, wuk_hbm, wuv_hbm, wo_hbm, wr_hbm, wg_hbm, wu_hbm, wd_hbm,
            o_ref,
            x_s, wr_s, wq_n, wuk_n, wuv_n, ckv_n, wo_n, wg_n, wu_n, wd_n,
            WQ, UP, UT, UV, CKT, CK, GT, UPT, QD, CL,
            WQT, UTF, UVT, WOF, GF, UF, DF, CSA, CSG, CSU, CLF, QAR, PS,
            sems):
    NM = cfg["nm"]
    NV = H - NM
    FM = cfg["fm"]
    NFM = FM // 128
    NG = (F - FM) // 8
    CHUNKS = _chunks(cfg)
    NCH = len(CHUNKS)

    hbm = dict(wq=wq_hbm, wuk=wuk_hbm, wuv=wuv_hbm, wo=wo_hbm, wg=wg_hbm, wu=wu_hbm, wd=wd_hbm,
               ckv=ckv_hbm.at[0])
    vm = dict(wq=wq_n, wuk=wuk_n, wuv=wuv_n, wo=wo_n, wg=wg_n, wu=wu_n, wd=wd_n, ckv=ckv_n)

    def chunk_copy(i):
        name, r0, n = CHUNKS[i]
        return pltpu.make_async_copy(hbm[name].at[pl.ds(r0, n)], vm[name].at[pl.ds(r0, n)],
                                     sems.at[i])

    def scope(name):
        return jax.named_scope(name) if cfg["scopes"] else _NoScope()

    def wait(i):
        with scope("wait%02d_%s" % (i, CHUNKS[i][0])):
            chunk_copy(i).wait()

    def idx(name):
        return [i for i, c in enumerate(CHUNKS) if c[0] == name]

    cx = pltpu.make_async_copy(x_hbm, x_s, sems.at[NCH])
    cr = pltpu.make_async_copy(wr_hbm, wr_s, sems.at[NCH + 1])
    cx.start()
    cr.start()
    for i in range(NCH):
        chunk_copy(i).start()

    def repack(src_n, dst, stride, j0, nj):
        def body(j, c):
            a = _u32(src_n[2 * j])
            b = _u32(src_n[2 * j + 1])
            lo = (a & jnp.uint32(0xFFFF)) | (b << 16)
            hi = (a >> 16) | (b & jnp.uint32(0xFFFF0000))
            dst[pl.ds(j, 16, stride=2 * stride), :] = lo
            dst[pl.ds(stride + j, 16, stride=2 * stride), :] = hi
            return c
        lax.fori_loop(j0, j0 + nj, body, 0, unroll=cfg["u_rp"])

    def vpu_transposes(src, stride, kb, dst):
        eye = _eye()

        def body(hv, c):
            tile = _bf(src[pl.ds((NM + hv) * stride + kb * 64, 64), :])
            row = pl.multiple_of(hv * 128, 128)
            dst[pl.ds(row, 128), pl.ds(kb * 128, 128)] = _dot_nt(eye, tile)
            return c
        lax.fori_loop(0, NV, body, 0, unroll=True)

    def prep_wuk_transpose(cb):
        eye = _eye()

        def body(h, c):
            tile = _bf(UP[pl.ds(h * SV + cb * 64, 64), :])
            UT[pl.ds((cb * NM + h) * 64, 64), :] = _transpose_tile(eye, tile)
            return c
        lax.fori_loop(0, NM, body, 0, unroll=True)

    def prep_ckv(kb0, nkb):
        eye = _eye()

        def body(kb, c):
            r0 = pl.multiple_of(kb * 128, 128)
            for cb in range(4):
                tile = ckv_n[pl.ds(r0, 128), pl.ds(cb * 128, 128)]
                CK[pl.ds(cb * 2048 + kb * 64, 64), :] = _u32(tile)
                CKT[pl.ds((kb * 4 + cb) * 64, 64), :] = _transpose_tile(eye, tile)
            return c
        lax.fori_loop(kb0, kb0 + nkb, body, 0, unroll=cfg["u_ckv"])

    def prep_ffn_mxu(src_n, dst, r0, n):
        eye = _eye()

        def body(nb, c):
            row = pl.multiple_of(nb * 128, 128)
            for kb in range(5):
                tile = src_n[pl.ds(row, 128), pl.ds(kb * 128, 128)]
                dst[pl.ds((nb * 5 + kb) * 64, 64), :] = _transpose_tile(eye, tile)
            return c
        lax.fori_loop(r0 // 128, (r0 + n) // 128, body, 0, unroll=True)

    def unpack_rows(src, r0, n, dst):
        step = 32 if n % 32 == 0 else 16

        def body(i, c):
            r = pl.multiple_of(i * step, step)
            dst[pl.ds(r, step), :] = src[pl.ds(r0 + r, step), :].astype(F32)
            return c
        lax.fori_loop(0, n // step, body, 0)
        assert n % step == 0

    def unpack_wo(h0, nh):
        def body(h, c):
            row = pl.multiple_of((h - NM) * 128, 128)
            WOF[pl.ds(row, 128), :] = wo_n[h].astype(F32)
            return c
        lax.fori_loop(h0, h0 + nh, body, 0)

    def front_mxu_q(xs):
        for h in range(NM):
            QD[pl.ds(h * 8, 8), :] = _u32(_split(_dot2(xs, _bf(WQ[pl.ds(h * SQ, 320), :]))))

    def front_mxu_qabs():
        for cb in range(4):
            for h in range(NM):
                r = _dot2(_bf(QD[pl.ds(h * 8, 8), :]), _bf(UT[pl.ds((cb * NM + h) * 64, 64), :]))
                QAR[pl.ds(h, 1), pl.ds(cb * 128, 128)] = r[0:1]

    def front_vpu(xn):
        for hv in range(NV):
            a = [None] * 4
            for g in range(16):
                rows = pl.ds(hv * 128 + g * 8, 8)
                qc = jnp.sum(_lane_blocks_sum(WQT[rows, :] * xn), axis=1, keepdims=True)
                for cb in range(4):
                    t = UTF[rows, pl.ds(cb * 128, 128)] * qc
                    a[cb] = t if a[cb] is None else a[cb] + t
            for cb in range(4):
                PS[pl.ds((cb * NV + hv) * SP, 8), :] = a[cb]
        for cb in range(4):
            for hv0 in range(0, NV, 8):
                n = min(8, NV - hv0)
                tot = None
                for s_ in range(8):
                    t = PS[pl.ds((cb * NV + hv0) * SP + s_, n, stride=SP), :]
                    tot = t if tot is None else tot + t
                QAR[pl.ds(NM + hv0, n), pl.ds(cb * 128, 128)] = tot

    def finish_front(mean, rstd):
        raw = QAR[...]
        row = lax.broadcasted_iota(jnp.int32, (H, 1), 0)
        mean32 = jnp.concatenate([mean] * 4, axis=0)
        rstd32 = jnp.concatenate([rstd] * 4, axis=0)
        off = jnp.where(row < NM, mean32, 0.0)
        mul = jnp.where(row < NM, rstd32, 1.0) * (D ** -0.5)
        return ((raw - off * CSA[...]) * mul).astype(BF)

    def scores(qa, nb0, nnb):
        return jnp.concatenate(
            [_dot(qa, _bf(CKT[pl.ds(nb * 256, 256), :])) for nb in range(nb0, nb0 + nnb)], axis=1)

    def pv(p, kb0, nkb):
        return jnp.concatenate(
            [_dot(p, _bf(CK[pl.ds(cb * 2048 + kb0 * 64, nkb * 64), :])) for cb in range(4)], axis=1)

    def stage_attn(qa):
        sa = scores(qa, 0, 16)
        sb = scores(qa, 16, 16)
        ma = jnp.max(sa, axis=1, keepdims=True)
        pa = jnp.exp(sa - ma)
        la = jnp.sum(pa, axis=1, keepdims=True)
        ca = pv(pa.astype(BF), 0, 16)
        m = jnp.maximum(ma, jnp.max(sb, axis=1, keepdims=True))
        pb = jnp.exp(sb - m)
        lb = jnp.sum(pb, axis=1, keepdims=True)
        cbv = pv(pb.astype(BF), 16, 16)
        alpha = jnp.exp(ma - m)
        inv = 1.0 / (alpha * la + lb)
        cl = (alpha * ca + cbv) * inv
        bits = pltpu.bitcast(cl.astype(BF).astype(F32), U32)
        dupw = bits | (bits >> 16)
        for cb in range(4):
            CL[pl.ds(cb * H, H), :] = dupw[:, cb * 128:(cb + 1) * 128]
            CLF[pl.ds(cb * H, H), :] = cl[:, cb * 128:(cb + 1) * 128]

    def ctx_mxu():
        for h in range(NM):
            lhs = jnp.concatenate(
                [_bf(CL[pl.ds(cb * H + h, 8, stride=0), :]) for cb in range(4)], axis=1)
            r = _dot(lhs, _bf(UV[pl.ds(h * SV, 256), :]))[0:8]
            QD[pl.ds(h * 8, 8), :] = _u32(_dup(r))

    def out_mxu(h0, nh, acc):
        for h in range(h0, h0 + nh):
            acc = acc + _dot(_bf(QD[pl.ds(h * 8, 8), :]), wo_n[h])[0:8]
        return acc

    def back_vpu(h0, nh, acc):
        for h in range(h0, h0 + nh):
            hv = h - NM
            cl = jnp.concatenate(
                [CLF[pl.ds(cb * H + h, 8, stride=0), :] for cb in range(4)], axis=1)
            for g in range(16):
                rows = pl.ds(hv * 128 + g * 8, 8)
                cc = jnp.sum(_lane_blocks_sum(UVT[rows, :] * cl), axis=1, keepdims=True)
                acc = acc + WOF[rows, :] * cc
        return acc

    def gate_up_mxu_raw(xs):
        g = [_dot2(xs, _bf(GT[pl.ds(nb * 320, 320), :])) for nb in range(NFM)]
        u = [_dot2(xs, _bf(UPT[pl.ds(nb * 320, 320), :])) for nb in range(NFM)]
        return g, u

    def gate_up_mxu(xs, mean, rstd):
        g, u = gate_up_mxu_raw(xs)
        hd = []
        for nb in range(NFM):
            cols = pl.ds(nb * 128, 128)
            gg = (g[nb] - mean * CSG[:, cols]) * rstd
            uu = (u[nb] - mean * CSU[:, cols]) * rstd
            hd.append(_dup(_swiglu(gg, uu)))
        return hd

    def down_mxu(hd, nb0, nb1, acc):
        for nb in range(nb0, nb1):
            acc = acc + _dot(hd[nb], wd_n[pl.ds(nb * 128, 128), :])[0:8]
        return acc

    def ffn_vpu(xn):
        acc = None
        for g in range(NG):
            rows = pl.ds(g * 8, 8)
            gc = jnp.sum(_lane_blocks_sum(GF[rows, :] * xn), axis=1, keepdims=True)
            uc = jnp.sum(_lane_blocks_sum(UF[rows, :] * xn), axis=1, keepdims=True)
            t = DF[rows, :] * _swiglu(gc, uc)
            acc = t if acc is None else acc + t
        return acc

    def gate_scalar(xn, wr8):
        return jax.nn.sigmoid(jnp.sum(xn * wr8, axis=1, keepdims=True))

    ones_split = jnp.concatenate([jnp.ones((8, M), BF), jnp.zeros((8, M), BF)], axis=0)

    cx.wait()
    cr.wait()
    x = jnp.broadcast_to(x_s[0].astype(F32), (8, M))
    wr8 = jnp.broadcast_to(wr_s[...].reshape(1, M).astype(F32), (8, M))

    if not cfg["compute1"]:
        for i in range(NCH):
            wait(i)
        o_ref[0] = x[0:1].astype(BF)
        return

    for k, i in enumerate(idx("wq")):
        wait(i)
        with scope("p_wq"):
            repack(wq_n, WQ, SQ, k * 64, 64)
            vpu_transposes(WQ, SQ, k, WQT)
    with scope("s1_csq"):
        front_mxu_q(ones_split)
    for k, i in enumerate(idx("wuk")):
        wait(i)
        with scope("p_wuk"):
            repack(wuk_n, UP, SV, k * 64, 64)
            prep_wuk_transpose(k)
            vpu_transposes(UP, SV, k, UTF)
    with scope("s1_csa"):
        front_mxu_qabs()
        CSA[pl.ds(0, NM), :] = QAR[pl.ds(0, NM), :]
        CSA[pl.ds(NM, NV), :] = jnp.zeros((NV, DC), F32)
    with scope("s1_front"):
        mean, rstd = _ln_stats(x)
        front_mxu_q(_split(x))
        front_mxu_qabs()
        front_vpu((x - mean) * rstd)
        qa = finish_front(mean, rstd)
    for k, i in enumerate(idx("ckv")):
        wait(i)
        with scope("p_ckv"):
            prep_ckv(k * 8, 8)
    with scope("s1_attn"):
        stage_attn(qa)
    for k, i in enumerate(idx("wuv")):
        wait(i)
        with scope("p_wuv"):
            repack(wuv_n, UV, SV, k * 64, 64)
            vpu_transposes(UV, SV, k, UVT)
    with scope("s1_ctx"):
        ctx_mxu()
    acc_v = jnp.zeros((8, M), F32)
    acc_m = jnp.zeros((8, M), F32)
    for i in idx("wo"):
        wait(i)
        h0, nh = CHUNKS[i][1], CHUNKS[i][2]
        with scope("s1_out"):
            if h0 >= NM:
                unpack_wo(h0, nh)
                acc_v = back_vpu(h0, nh, acc_v)
            else:
                acc_m = out_mxu(h0, nh, acc_m)
    x = x + acc_m + _row_total(acc_v)
    for name, nat, tr, fl in (("wg", wg_n, GT, GF), ("wu", wu_n, UPT, UF)):
        for i in idx(name):
            wait(i)
            r0, n = CHUNKS[i][1], CHUNKS[i][2]
            with scope("p_" + name):
                if r0 >= FM:
                    unpack_rows(nat, r0, n, fl)
                else:
                    prep_ffn_mxu(nat, tr, r0, n)
    with scope("s2_cs"):
        g, u = gate_up_mxu_raw(ones_split)
        CSG[...] = jnp.concatenate(g, axis=1)
        CSU[...] = jnp.concatenate(u, axis=1)
    wd_idx = idx("wd")
    wait(wd_idx[0])
    with scope("p_wd"):
        unpack_rows(wd_n, FM, F - FM, DF)
    with scope("s2_gu"):
        mean, rstd = _ln_stats(x)
        xn = (x - mean) * rstd
        hd = gate_up_mxu(_split(x), mean, rstd)
        acc_v = ffn_vpu(xn)
        sg = gate_scalar(xn, wr8)
    acc_m = _row_total(acc_v)
    for i in wd_idx[1:]:
        wait(i)
        r0, n = CHUNKS[i][1], CHUNKS[i][2]
        with scope("s2_down"):
            acc_m = down_mxu(hd, r0 // 128, (r0 + n) // 128, acc_m)
    x = x + xn + acc_m * sg

    if cfg["phase2"]:
        with scope("phase2"):
            mean, rstd = _ln_stats(x)
            front_mxu_q(_split(x))
            front_mxu_qabs()
            front_vpu((x - mean) * rstd)
            stage_attn(finish_front(mean, rstd))
            ctx_mxu()
            acc_m = out_mxu(0, NM, jnp.zeros((8, M), F32))
            acc_v = back_vpu(NM, NV, jnp.zeros((8, M), F32))
            x = x + acc_m + _row_total(acc_v)
            mean, rstd = _ln_stats(x)
            xn = (x - mean) * rstd
            hd = gate_up_mxu(_split(x), mean, rstd)
            acc_v = ffn_vpu(xn)
            sg = gate_scalar(xn, wr8)
            y = down_mxu(hd, 0, NFM, _row_total(acc_v))
            x = x + xn + y * sg

    o_ref[0] = x[0:1].astype(BF)


def _run(cfg, A_x, A_c_kv, A_w_q, A_w_uk, A_w_uv, A_w_o, B_w_r, B_w_gate, B_w_up, B_w_down):
    any_spec = pl.BlockSpec(memory_space=pl.ANY)
    nm = cfg["nm"]
    nv = H - nm
    fm = cfg["fm"]
    nch = len(_chunks(cfg))
    scratch = [
        pltpu.VMEM((1, 1, M), BF),
        pltpu.VMEM((M,), BF),
        pltpu.VMEM((M, H, D), BF),
        pltpu.VMEM((DC, H, D), BF),
        pltpu.VMEM((DC, H, D), BF),
        pltpu.VMEM((SK, DC), BF),
        pltpu.VMEM((H, D, M), BF),
        pltpu.VMEM((F, M), BF),
        pltpu.VMEM((F, M), BF),
        pltpu.VMEM((F, M), BF),
        pltpu.VMEM((H * SQ, 128), U32),
        pltpu.VMEM((H * SV, 128), U32),
        pltpu.VMEM((4 * nm * 64, 128), U32),
        pltpu.VMEM((H * SV, 128), U32),
        pltpu.VMEM((32 * 4 * 64, 128), U32),
        pltpu.VMEM((4 * 2048, 128), U32),
        pltpu.VMEM((fm // 128 * 320, 128), U32),
        pltpu.VMEM((fm // 128 * 320, 128), U32),
        pltpu.VMEM((H * 8, 128), U32),
        pltpu.VMEM((4 * H, 128), U32),
        pltpu.VMEM((nv * 128, M), F32),
        pltpu.VMEM((nv * 128, DC), F32),
        pltpu.VMEM((nv * 128, DC), F32),
        pltpu.VMEM((nv * 128, M), F32),
        pltpu.VMEM((F - fm, M), F32),
        pltpu.VMEM((F - fm, M), F32),
        pltpu.VMEM((F - fm, M), F32),
        pltpu.VMEM((H, DC), F32),
        pltpu.VMEM((8, fm), F32),
        pltpu.VMEM((8, fm), F32),
        pltpu.VMEM((4 * H, 128), F32),
        pltpu.VMEM((H, DC), F32),
        pltpu.VMEM((4 * nv * SP, 128), F32),
        pltpu.SemaphoreType.DMA((nch + 2,)),
    ]
    return pl.pallas_call(
        functools.partial(_kernel, cfg),
        out_shape=jax.ShapeDtypeStruct((1, 1, M), BF),
        in_specs=[any_spec] * 10,
        out_specs=pl.BlockSpec(memory_space=pltpu.VMEM),
        scratch_shapes=scratch,
        compiler_params=pltpu.CompilerParams(vmem_limit_bytes=110 * 1024 * 1024),
    )(A_x, A_c_kv, A_w_q, A_w_uk, A_w_uv, A_w_o, B_w_r, B_w_gate.T, B_w_up.T, B_w_down)


def build(**overrides):
    cfg = dict(DEFAULT_CFG, **overrides)

    @jax.jit
    def fn(A_x, A_c_kv, A_w_q, A_w_uk, A_w_uv, A_w_o, B_x, B_w_r, B_w_gate, B_w_up, B_w_down):
        return _run(cfg, A_x, A_c_kv, A_w_q, A_w_uk, A_w_uv, A_w_o, B_w_r, B_w_gate, B_w_up, B_w_down)
    return fn


@jax.jit
def pallas_interleave_layers__compressed_kv_cla__moe_arch_mod__decode_kernel(
    A_x: jax.Array,
    A_c_kv: jax.Array,
    A_w_q: jax.Array,
    A_w_uk: jax.Array,
    A_w_uv: jax.Array,
    A_w_o: jax.Array,
    B_x: jax.Array,
    B_w_r: jax.Array,
    B_w_gate: jax.Array,
    B_w_up: jax.Array,
    B_w_down: jax.Array,
):
    del B_x
    return _run(DEFAULT_CFG, A_x, A_c_kv, A_w_q, A_w_uk, A_w_uv, A_w_o, B_w_r, B_w_gate, B_w_up,
                B_w_down)
```

```python
import functools

import jax
import jax.numpy as jnp
from jax import lax
from jax.experimental import pallas as pl
from jax.experimental.pallas import tpu as pltpu

M = 640
H = 32
D = 128
DC = 512
SK = 4096
F = 1728
EPS = 1e-5

SQ = 322
SP = 9
SV = 258

BF = jnp.bfloat16
F32 = jnp.float32
U32 = jnp.uint32


def _bf(u32_val):
    return pltpu.bitcast(u32_val, BF)


def _u32(bf_val):
    return pltpu.bitcast(bf_val, U32)


def _dup(v8):
    return jnp.concatenate([v8, v8], axis=0).astype(BF)


def _dot(a, b):
    return jnp.dot(a, b, preferred_element_type=F32)


def _dot_nt(a, b):
    return lax.dot_general(a, b, (((1,), (1,)), ((), ())), preferred_element_type=F32)


def _split(v8):
    hi = pltpu.bitcast(pltpu.bitcast(v8, U32) & jnp.uint32(0xFFFF0000), F32)
    return jnp.concatenate([hi, v8 - hi], axis=0).astype(BF)


def _dot2(a16, b):
    r = _dot(a16, b)
    return r[0:8] + r[8:16]


def _ln_stats(x8):
    s1 = jnp.sum(x8, axis=1, keepdims=True)
    s2 = jnp.sum(x8 * x8, axis=1, keepdims=True)
    mean = s1 * (1.0 / M)
    var = jnp.maximum(s2 * (1.0 / M) - mean * mean, 0.0)
    return mean, lax.rsqrt(var + EPS)


def _swiglu(g, u):
    a = 0.5 * g
    b = a * u
    return b * jnp.tanh(a) + b


def _lane_blocks_sum(p):
    n = p.shape[1] // 128
    acc = p[:, 0:128]
    for i in range(1, n):
        acc = acc + p[:, i * 128:(i + 1) * 128]
    return acc


def _row_total(a8):
    return jnp.broadcast_to(jnp.sum(a8, axis=0, keepdims=True), a8.shape)


def _eye():
    r = lax.broadcasted_iota(jnp.int32, (128, 128), 0)
    c = lax.broadcasted_iota(jnp.int32, (128, 128), 1)
    return jnp.where(r == c, 1.0, 0.0).astype(BF)


def _transpose_tile(eye, tile):
    return _u32(_dot_nt(eye, tile).astype(BF))


def _chunks(cfg):
    fm = cfg["fm"]
    nm = cfg["nm"]
    ch = []
    ch += [("wq", i * 128, 128) for i in range(5)]
    ch += [("wuk", i * 128, 128) for i in range(4)]
    ch += [("ckv", i * 1024, 1024) for i in range(4)]
    ch += [("wuv", i * 128, 128) for i in range(4)]
    ch += [("wo", h0, min(8, H - h0)) for h0 in range(nm, H, 8)]
    ch += [("wo", h0, min(8, nm - h0)) for h0 in range(0, nm, 8)]
    for name in ("wg", "wu"):
        ch += [(name, fm, F - fm)]
        ch += [(name, r0, min(512, fm - r0)) for r0 in range(0, fm, 512)]
    ch += [("wd", fm, F - fm)]
    r0 = 0
    while r0 < fm - 128:
        n = min(512, fm - 128 - r0)
        ch.append(("wd", r0, n))
        r0 += n
    ch.append(("wd", fm - 128, 128))
    return ch


DEFAULT_CFG = dict(phase2=True, compute1=True, scopes=False, u_uk=16, u_ckv=4, u_rp=4,
                   nm=16, fm=1024, chain=True, nsem=8)


class _NoScope:
    def __enter__(self):
        return self

    def __exit__(self, *a):
        return False


def _kernel(cfg, x_hbm, ckv_hbm, wq_hbm, wuk_hbm, wuv_hbm, wo_hbm, wr_hbm, wg_hbm, wu_hbm, wd_hbm,
            o_ref,
            x_s, wr_s, wq_n, wuk_n, wuv_n, ckv_n, wo_n, wg_n, wu_n, wd_n,
            WQ, UP, UT, UV, CKT, CK, GT, UPT, QD, CL,
            WQT, UTF, UVT, WOF, GF, UF, DF, CSA, CSG, CSU, CLF, QAR, PS, WOU, WDU, FLAG,
            sems):
    NM = cfg["nm"]
    NV = H - NM
    FM = cfg["fm"]
    NFM = FM // 128
    NG = (F - FM) // 8
    CHUNKS = _chunks(cfg)
    NCH = len(CHUNKS)
    NSEM = min(cfg["nsem"], NCH)

    hbm = dict(wq=wq_hbm, wuk=wuk_hbm, wuv=wuv_hbm, wo=wo_hbm, wg=wg_hbm, wu=wu_hbm, wd=wd_hbm,
               ckv=ckv_hbm.at[0])
    vm = dict(wq=wq_n, wuk=wuk_n, wuv=wuv_n, wo=wo_n, wg=wg_n, wu=wu_n, wd=wd_n, ckv=ckv_n)

    def chunk_copy(i):
        name, r0, n = CHUNKS[i]
        return pltpu.make_async_copy(hbm[name].at[pl.ds(r0, n)], vm[name].at[pl.ds(r0, n)],
                                     sems.at[i % NSEM])

    def scope(name):
        return jax.named_scope(name) if cfg["scopes"] else _NoScope()

    def wait(i):
        with scope("wait%02d_%s" % (i, CHUNKS[i][0])):
            chunk_copy(i).wait()
        if i + NSEM < NCH:
            chunk_copy(i + NSEM).start()

    def idx(name):
        return [i for i, c in enumerate(CHUNKS) if c[0] == name]

    cx = pltpu.make_async_copy(x_hbm, x_s, sems.at[NSEM])
    cr = pltpu.make_async_copy(wr_hbm, wr_s, sems.at[NSEM + 1])
    cx.start()
    cr.start()
    for i in range(NSEM):
        chunk_copy(i).start()

    FLAG[...] = jnp.ones((8, 128), jnp.int32)

    def repack(src_n, dst, stride, j0, nj):
        def body(j, c):
            a = _u32(src_n[2 * j])
            b = _u32(src_n[2 * j + 1])
            lo = (a & jnp.uint32(0xFFFF)) | (b << 16)
            hi = (a >> 16) | (b & jnp.uint32(0xFFFF0000))
            dst[pl.ds(j, 16, stride=2 * stride), :] = lo
            dst[pl.ds(stride + j, 16, stride=2 * stride), :] = hi
            return c
        lax.fori_loop(j0, j0 + nj, body, 0, unroll=cfg["u_rp"])

    def vpu_transposes(src, stride, kb, dst):
        eye = _eye()

        def body(hv, c):
            tile = _bf(src[pl.ds((NM + hv) * stride + kb * 64, 64), :])
            row = pl.multiple_of(hv * 128, 128)
            dst[pl.ds(row, 128), pl.ds(kb * 128, 128)] = _dot_nt(eye, tile)
            return c
        lax.fori_loop(0, NV, body, 0, unroll=True)

    def prep_wuk_transpose(cb):
        eye = _eye()

        def body(h, c):
            tile = _bf(UP[pl.ds(h * SV + cb * 64, 64), :])
            UT[pl.ds((cb * NM + h) * 64, 64), :] = _transpose_tile(eye, tile)
            return c
        lax.fori_loop(0, NM, body, 0, unroll=True)

    def prep_ckv(kb0, nkb):
        eye = _eye()

        def body(kb, c):
            r0 = pl.multiple_of(kb * 128, 128)
            for cb in range(4):
                tile = ckv_n[pl.ds(r0, 128), pl.ds(cb * 128, 128)]
                CK[pl.ds(cb * 2048 + kb * 64, 64), :] = _u32(tile)
                CKT[pl.ds((kb * 4 + cb) * 64, 64), :] = _transpose_tile(eye, tile)
            return c
        lax.fori_loop(kb0, kb0 + nkb, body, 0, unroll=cfg["u_ckv"])

    def prep_ffn_mxu(src_n, dst, r0, n):
        eye = _eye()

        def body(nb, c):
            row = pl.multiple_of(nb * 128, 128)
            for kb in range(5):
                tile = src_n[pl.ds(row, 128), pl.ds(kb * 128, 128)]
                dst[pl.ds((nb * 5 + kb) * 64, 64), :] = _transpose_tile(eye, tile)
            return c
        lax.fori_loop(r0 // 128, (r0 + n) // 128, body, 0, unroll=True)

    def unpack_rows(src, r0, n, dst):
        step = 32 if n % 32 == 0 else 16

        def body(i, c):
            r = pl.multiple_of(i * step, step)
            dst[pl.ds(r, step), :] = src[pl.ds(r0 + r, step), :].astype(F32)
            return c
        lax.fori_loop(0, n // step, body, 0)
        assert n % step == 0

    def unpack_wo(h0, nh):
        def body(h, c):
            row = pl.multiple_of((h - NM) * 128, 128)
            WOF[pl.ds(row, 128), :] = wo_n[h].astype(F32)
            return c
        lax.fori_loop(h0, h0 + nh, body, 0)

    def front_mxu_q(xs):
        for h in range(NM):
            QD[pl.ds(h * 8, 8), :] = _u32(_split(_dot2(xs, _bf(WQ[pl.ds(h * SQ, 320), :]))))

    def front_mxu_qabs():
        for cb in range(4):
            for h in range(NM):
                r = _dot2(_bf(QD[pl.ds(h * 8, 8), :]), _bf(UT[pl.ds((cb * NM + h) * 64, 64), :]))
                QAR[pl.ds(cb * H + h, 1), :] = r[0:1]

    def front_vpu(xn):
        always = FLAG[...] != 0
        a = [None] * 4
        for hv in range(NV):
            for g in range(16):
                rows = pl.ds(hv * 128 + g * 8, 8)
                qc = jnp.sum(_lane_blocks_sum(WQT[rows, :] * xn), axis=1, keepdims=True)
                for cb in range(4):
                    t = UTF[rows, pl.ds(cb * 128, 128)] * qc
                    if g > 0:
                        a[cb] = a[cb] + t
                    elif hv > 0 and cfg["chain"]:
                        a[cb] = jnp.where(always, t, a[cb])
                    else:
                        a[cb] = t
            for cb in range(4):
                PS[pl.ds((cb * NV + hv) * SP, 8), :] = a[cb]
        for cb in range(4):
            for hv0 in range(0, NV, 8):
                n = min(8, NV - hv0)
                tot = None
                for s_ in range(8):
                    t = PS[pl.ds((cb * NV + hv0) * SP + s_, n, stride=SP), :]
                    tot = t if tot is None else tot + t
                QAR[pl.ds(cb * H + NM + hv0, n), :] = tot

    def finish_front(mean, rstd):
        row = lax.broadcasted_iota(jnp.int32, (H, 1), 0)
        mean32 = jnp.concatenate([mean] * 4, axis=0)
        rstd32 = jnp.concatenate([rstd] * 4, axis=0)
        off = jnp.where(row < NM, mean32, 0.0)
        mul = jnp.where(row < NM, rstd32, 1.0) * (D ** -0.5)
        return jnp.concatenate(
            [((QAR[pl.ds(cb * H, H), :] - off * CSA[pl.ds(cb * H, H), :]) * mul).astype(BF)
             for cb in range(4)], axis=1)

    def scores(qa, nb0, nnb):
        return jnp.concatenate(
            [_dot(qa, _bf(CKT[pl.ds(nb * 256, 256), :])) for nb in range(nb0, nb0 + nnb)], axis=1)

    def pv(p, kb0, nkb):
        return jnp.concatenate(
            [_dot(p, _bf(CK[pl.ds(cb * 2048 + kb0 * 64, nkb * 64), :])) for cb in range(4)], axis=1)

    def stage_attn(qa):
        sa = scores(qa, 0, 16)
        sb = scores(qa, 16, 16)
        ma = jnp.max(sa, axis=1, keepdims=True)
        pa = jnp.exp(sa - ma)
        la = jnp.sum(pa, axis=1, keepdims=True)
        ca = pv(pa.astype(BF), 0, 16)
        m = jnp.maximum(ma, jnp.max(sb, axis=1, keepdims=True))
        pb = jnp.exp(sb - m)
        lb = jnp.sum(pb, axis=1, keepdims=True)
        cbv = pv(pb.astype(BF), 16, 16)
        alpha = jnp.exp(ma - m)
        inv = 1.0 / (alpha * la + lb)
        cl = (alpha * ca + cbv) * inv
        bits = pltpu.bitcast(cl.astype(BF).astype(F32), U32)
        dupw = bits | (bits >> 16)
        for cb in range(4):
            CL[pl.ds(cb * H, H), :] = dupw[:, cb * 128:(cb + 1) * 128]
            CLF[pl.ds(cb * H, H), :] = cl[:, cb * 128:(cb + 1) * 128]

    def ctx_mxu():
        for h in range(NM):
            lhs = jnp.concatenate(
                [_bf(CL[pl.ds(cb * H + h, 8, stride=0), :]) for cb in range(4)], axis=1)
            r = _dot(lhs, _bf(UV[pl.ds(h * SV, 256), :]))[0:8]
            QD[pl.ds(h * 8, 8), :] = _u32(_dup(r))

    def out_mxu(h0, nh, acc, first):
        for h in range(h0, h0 + nh):
            if first:
                w = wo_n[h]
                for mb in range(5):
                    WOU[pl.ds((h * 5 + mb) * 64, 64), :] = _u32(w[:, mb * 128:(mb + 1) * 128])
            else:
                w = jnp.concatenate(
                    [_bf(WOU[pl.ds((h * 5 + mb) * 64, 64), :]) for mb in range(5)], axis=1)
            acc = acc + _dot(_bf(QD[pl.ds(h * 8, 8), :]), w)[0:8]
        return acc

    def back_vpu(h0, nh, acc):
        for h in range(h0, h0 + nh):
            hv = h - NM
            cl = jnp.concatenate(
                [CLF[pl.ds(cb * H + h, 8, stride=0), :] for cb in range(4)], axis=1)
            for g in range(16):
                rows = pl.ds(hv * 128 + g * 8, 8)
                cc = jnp.sum(_lane_blocks_sum(UVT[rows, :] * cl), axis=1, keepdims=True)
                acc = acc + WOF[rows, :] * cc
        return acc

    def gate_up_mxu_raw(xs):
        g = [_dot2(xs, _bf(GT[pl.ds(nb * 320, 320), :])) for nb in range(NFM)]
        u = [_dot2(xs, _bf(UPT[pl.ds(nb * 320, 320), :])) for nb in range(NFM)]
        return g, u

    def gate_up_mxu(xs, mean, rstd):
        g, u = gate_up_mxu_raw(xs)
        hd = []
        for nb in range(NFM):
            cols = pl.ds(nb * 128, 128)
            gg = (g[nb] - mean * CSG[:, cols]) * rstd
            uu = (u[nb] - mean * CSU[:, cols]) * rstd
            hd.append(_dup(_swiglu(gg, uu)))
        return hd

    def down_mxu(hd, nb0, nb1, acc, first):
        for nb in range(nb0, nb1):
            if first:
                w = wd_n[pl.ds(nb * 128, 128), :]
                for mb in range(5):
                    WDU[pl.ds((nb * 5 + mb) * 64, 64), :] = _u32(w[:, mb * 128:(mb + 1) * 128])
            else:
                w = jnp.concatenate(
                    [_bf(WDU[pl.ds((nb * 5 + mb) * 64, 64), :]) for mb in range(5)], axis=1)
            acc = acc + _dot(hd[nb], w)[0:8]
        return acc

    def ffn_vpu(xn):
        acc = None
        for g in range(NG):
            rows = pl.ds(g * 8, 8)
            gc = jnp.sum(_lane_blocks_sum(GF[rows, :] * xn), axis=1, keepdims=True)
            uc = jnp.sum(_lane_blocks_sum(UF[rows, :] * xn), axis=1, keepdims=True)
            t = DF[rows, :] * _swiglu(gc, uc)
            acc = t if acc is None else acc + t
        return acc

    def gate_scalar(xn, wr8):
        return jax.nn.sigmoid(jnp.sum(xn * wr8, axis=1, keepdims=True))

    ones_split = jnp.concatenate([jnp.ones((8, M), BF), jnp.zeros((8, M), BF)], axis=0)

    cx.wait()
    cr.wait()
    x = jnp.broadcast_to(x_s[0].astype(F32), (8, M))
    wr8 = jnp.broadcast_to(wr_s[...].reshape(1, M).astype(F32), (8, M))

    if not cfg["compute1"]:
        for i in range(NCH):
            wait(i)
        o_ref[0] = x[0:1].astype(BF)
        return

    for k, i in enumerate(idx("wq")):
        wait(i)
        with scope("p_wq"):
            repack(wq_n, WQ, SQ, k * 64, 64)
            vpu_transposes(WQ, SQ, k, WQT)
    with scope("s1_csq"):
        front_mxu_q(ones_split)
    for k, i in enumerate(idx("wuk")):
        wait(i)
        with scope("p_wuk"):
            repack(wuk_n, UP, SV, k * 64, 64)
            prep_wuk_transpose(k)
            vpu_transposes(UP, SV, k, UTF)
    with scope("s1_csa"):
        front_mxu_qabs()
        for cb in range(4):
            CSA[pl.ds(cb * H, NM), :] = QAR[pl.ds(cb * H, NM), :]
            CSA[pl.ds(cb * H + NM, NV), :] = jnp.zeros((NV, 128), F32)
    with scope("s1_front"):
        mean, rstd = _ln_stats(x)
        front_mxu_q(_split(x))
        front_mxu_qabs()
        front_vpu((x - mean) * rstd)
        qa = finish_front(mean, rstd)
    for k, i in enumerate(idx("ckv")):
        wait(i)
        with scope("p_ckv"):
            prep_ckv(k * 8, 8)
    with scope("s1_attn"):
        stage_attn(qa)
    for k, i in enumerate(idx("wuv")):
        wait(i)
        with scope("p_wuv"):
            repack(wuv_n, UV, SV, k * 64, 64)
            vpu_transposes(UV, SV, k, UVT)
    with scope("s1_ctx"):
        ctx_mxu()
    acc_v = jnp.zeros((8, M), F32)
    acc_m = jnp.zeros((8, M), F32)
    for i in idx("wo"):
        wait(i)
        h0, nh = CHUNKS[i][1], CHUNKS[i][2]
        with scope("s1_out"):
            if h0 >= NM:
                unpack_wo(h0, nh)
                acc_v = back_vpu(h0, nh, acc_v)
            else:
                acc_m = out_mxu(h0, nh, acc_m, True)
    x = x + acc_m + _row_total(acc_v)
    for name, nat, tr, fl in (("wg", wg_n, GT, GF), ("wu", wu_n, UPT, UF)):
        for i in idx(name):
            wait(i)
            r0, n = CHUNKS[i][1], CHUNKS[i][2]
            with scope("p_" + name):
                if r0 >= FM:
                    unpack_rows(nat, r0, n, fl)
                else:
                    prep_ffn_mxu(nat, tr, r0, n)
    with scope("s2_cs"):
        g, u = gate_up_mxu_raw(ones_split)
        CSG[...] = jnp.concatenate(g, axis=1)
        CSU[...] = jnp.concatenate(u, axis=1)
    wd_idx = idx("wd")
    wait(wd_idx[0])
    with scope("p_wd"):
        unpack_rows(wd_n, FM, F - FM, DF)
    with scope("s2_gu"):
        mean, rstd = _ln_stats(x)
        xn = (x - mean) * rstd
        hd = gate_up_mxu(_split(x), mean, rstd)
        acc_v = ffn_vpu(xn)
        sg = gate_scalar(xn, wr8)
    acc_m = _row_total(acc_v)
    for i in wd_idx[1:]:
        wait(i)
        r0, n = CHUNKS[i][1], CHUNKS[i][2]
        with scope("s2_down"):
            acc_m = down_mxu(hd, r0 // 128, (r0 + n) // 128, acc_m, True)
    x = x + xn + acc_m * sg

    if cfg["phase2"]:
        with scope("phase2"):
            mean, rstd = _ln_stats(x)
            front_mxu_q(_split(x))
            front_mxu_qabs()
            front_vpu((x - mean) * rstd)
            stage_attn(finish_front(mean, rstd))
            ctx_mxu()
            acc_m = out_mxu(0, NM, jnp.zeros((8, M), F32), False)
            acc_v = back_vpu(NM, NV, jnp.zeros((8, M), F32))
            x = x + acc_m + _row_total(acc_v)
            mean, rstd = _ln_stats(x)
            xn = (x - mean) * rstd
            hd = gate_up_mxu(_split(x), mean, rstd)
            acc_v = ffn_vpu(xn)
            sg = gate_scalar(xn, wr8)
            y = down_mxu(hd, 0, NFM, _row_total(acc_v), False)
            x = x + xn + y * sg

    o_ref[0] = x[0:1].astype(BF)


def _run(cfg, A_x, A_c_kv, A_w_q, A_w_uk, A_w_uv, A_w_o, B_w_r, B_w_gate, B_w_up, B_w_down):
    any_spec = pl.BlockSpec(memory_space=pl.ANY)
    nm = cfg["nm"]
    nv = H - nm
    fm = cfg["fm"]
    nsem = min(cfg["nsem"], len(_chunks(cfg)))
    scratch = [
        pltpu.VMEM((1, 1, M), BF),
        pltpu.VMEM((M,), BF),
        pltpu.VMEM((M, H, D), BF),
        pltpu.VMEM((DC, H, D), BF),
        pltpu.VMEM((DC, H, D), BF),
        pltpu.VMEM((SK, DC), BF),
        pltpu.VMEM((H, D, M), BF),
        pltpu.VMEM((F, M), BF),
        pltpu.VMEM((F, M), BF),
        pltpu.VMEM((F, M), BF),
        pltpu.VMEM((H * SQ, 128), U32),
        pltpu.VMEM((H * SV, 128), U32),
        pltpu.VMEM((4 * nm * 64, 128), U32),
        pltpu.VMEM((H * SV, 128), U32),
        pltpu.VMEM((32 * 4 * 64, 128), U32),
        pltpu.VMEM((4 * 2048, 128), U32),
        pltpu.VMEM((fm // 128 * 320, 128), U32),
        pltpu.VMEM((fm // 128 * 320, 128), U32),
        pltpu.VMEM((H * 8, 128), U32),
        pltpu.VMEM((4 * H, 128), U32),
        pltpu.VMEM((nv * 128, M), F32),
        pltpu.VMEM((nv * 128, DC), F32),
        pltpu.VMEM((nv * 128, DC), F32),
        pltpu.VMEM((nv * 128, M), F32),
        pltpu.VMEM((F - fm, M), F32),
        pltpu.VMEM((F - fm, M), F32),
        pltpu.VMEM((F - fm, M), F32),
        pltpu.VMEM((4 * H, 128), F32),
        pltpu.VMEM((8, fm), F32),
        pltpu.VMEM((8, fm), F32),
        pltpu.VMEM((4 * H, 128), F32),
        pltpu.VMEM((4 * H, 128), F32),
        pltpu.VMEM((4 * nv * SP, 128), F32),
        pltpu.VMEM((nm * 5 * 64, 128), U32),
        pltpu.VMEM((fm // 128 * 5 * 64, 128), U32),
        pltpu.VMEM((8, 128), jnp.int32),
        pltpu.SemaphoreType.DMA((nsem + 2,)),
    ]
    return pl.pallas_call(
        functools.partial(_kernel, cfg),
        out_shape=jax.ShapeDtypeStruct((1, 1, M), BF),
        in_specs=[any_spec] * 10,
        out_specs=pl.BlockSpec(memory_space=pltpu.VMEM),
        scratch_shapes=scratch,
        compiler_params=pltpu.CompilerParams(vmem_limit_bytes=110 * 1024 * 1024),
    )(A_x, A_c_kv, A_w_q, A_w_uk, A_w_uv, A_w_o, B_w_r, B_w_gate.T, B_w_up.T, B_w_down)


def build(**overrides):
    cfg = dict(DEFAULT_CFG, **overrides)

    @jax.jit
    def fn(A_x, A_c_kv, A_w_q, A_w_uk, A_w_uv, A_w_o, B_x, B_w_r, B_w_gate, B_w_up, B_w_down):
        return _run(cfg, A_x, A_c_kv, A_w_q, A_w_uk, A_w_uv, A_w_o, B_w_r, B_w_gate, B_w_up, B_w_down)
    return fn


@jax.jit
def pallas_interleave_layers__compressed_kv_cla__moe_arch_mod__decode_kernel(
    A_x: jax.Array,
    A_c_kv: jax.Array,
    A_w_q: jax.Array,
    A_w_uk: jax.Array,
    A_w_uv: jax.Array,
    A_w_o: jax.Array,
    B_x: jax.Array,
    B_w_r: jax.Array,
    B_w_gate: jax.Array,
    B_w_up: jax.Array,
    B_w_down: jax.Array,
):
    del B_x
    return _run(DEFAULT_CFG, A_x, A_c_kv, A_w_q, A_w_uk, A_w_uv, A_w_o, B_w_r, B_w_gate, B_w_up,
                B_w_down)
```

```python
import functools

import jax
import jax.numpy as jnp
from jax import lax
from jax.experimental import pallas as pl
from jax.experimental.pallas import tpu as pltpu

M = 640
H = 32
D = 128
DC = 512
SK = 4096
F = 1728
EPS = 1e-5

SQ = 322
SP = 9
SV = 258

BF = jnp.bfloat16
F32 = jnp.float32
U32 = jnp.uint32


def _bf(u32_val):
    return pltpu.bitcast(u32_val, BF)


def _u32(bf_val):
    return pltpu.bitcast(bf_val, U32)


def _dup(v8):
    return jnp.concatenate([v8, v8], axis=0).astype(BF)


def _dot(a, b):
    return jnp.dot(a, b, preferred_element_type=F32)


def _dot_nt(a, b):
    return lax.dot_general(a, b, (((1,), (1,)), ((), ())), preferred_element_type=F32)


def _split(v8):
    hi = pltpu.bitcast(pltpu.bitcast(v8, U32) & jnp.uint32(0xFFFF0000), F32)
    return jnp.concatenate([hi, v8 - hi], axis=0).astype(BF)


def _dot2(a16, b):
    r = _dot(a16, b)
    return r[0:8] + r[8:16]


def _ln_stats(x8):
    s1 = jnp.sum(x8, axis=1, keepdims=True)
    s2 = jnp.sum(x8 * x8, axis=1, keepdims=True)
    mean = s1 * (1.0 / M)
    var = jnp.maximum(s2 * (1.0 / M) - mean * mean, 0.0)
    return mean, lax.rsqrt(var + EPS)


def _swiglu(g, u):
    a = 0.5 * g
    b = a * u
    return b * jnp.tanh(a) + b


def _lane_blocks_sum(p):
    n = p.shape[1] // 128
    acc = p[:, 0:128]
    for i in range(1, n):
        acc = acc + p[:, i * 128:(i + 1) * 128]
    return acc


def _row_total(a8):
    return jnp.broadcast_to(jnp.sum(a8, axis=0, keepdims=True), a8.shape)


def _eye():
    r = lax.broadcasted_iota(jnp.int32, (128, 128), 0)
    c = lax.broadcasted_iota(jnp.int32, (128, 128), 1)
    return jnp.where(r == c, 1.0, 0.0).astype(BF)


def _transpose_tile(eye, tile):
    return _u32(_dot_nt(eye, tile).astype(BF))


def _chunks(cfg):
    fm = cfg["fm"]
    nm = cfg["nm"]
    ch = []
    ch += [("wq", i * 128, 128) for i in range(5)]
    ch += [("wuk", i * 128, 128) for i in range(4)]
    ch += [("ckv", i * 1024, 1024) for i in range(4)]
    ch += [("wuv", i * 128, 128) for i in range(4)]
    ch += [("wo", h0, min(8, H - h0)) for h0 in range(nm, H, 8)]
    ch += [("wo", h0, min(8, nm - h0)) for h0 in range(0, nm, 8)]
    for name in ("wg", "wu"):
        ch += [(name, fm, F - fm)]
        ch += [(name, r0, min(512, fm - r0)) for r0 in range(0, fm, 512)]
    ch += [("wd", fm, F - fm)]
    r0 = 0
    while r0 < fm - 128:
        n = min(512, fm - 128 - r0)
        ch.append(("wd", r0, n))
        r0 += n
    ch.append(("wd", fm - 128, 128))
    return ch


DEFAULT_CFG = dict(phase2=True, compute1=True, scopes=False, u_uk=16, u_ckv=4, u_rp=4,
                   nm=17, fm=1024, gate=True, lag=2, beta=1.0, nsem=6)


class _NoScope:
    def __enter__(self):
        return self

    def __exit__(self, *a):
        return False


def _kernel(cfg, x_hbm, ckv_hbm, wq_hbm, wuk_hbm, wuv_hbm, wo_hbm, wr_hbm, wg_hbm, wu_hbm, wd_hbm,
            o_ref,
            x_s, wr_s, wq_n, wuk_n, wuv_n, ckv_n, wo_n, wg_n, wu_n, wd_n,
            WQ, UP, UT, UV, CKT, CK, GT, UPT, QD, CL,
            WQT, UTF, UVT, WOF, GF, UF, DF, CSA, CSG, CSU, CLF, QAR, PS, WOU, WDU, FLAG,
            sems):
    NM = cfg["nm"]
    NV = H - NM
    FM = cfg["fm"]
    NFM = FM // 128
    NG = (F - FM) // 8
    CHUNKS = _chunks(cfg)
    NCH = len(CHUNKS)
    NSEM = min(cfg["nsem"], NCH)

    hbm = dict(wq=wq_hbm, wuk=wuk_hbm, wuv=wuv_hbm, wo=wo_hbm, wg=wg_hbm, wu=wu_hbm, wd=wd_hbm,
               ckv=ckv_hbm.at[0])
    vm = dict(wq=wq_n, wuk=wuk_n, wuv=wuv_n, wo=wo_n, wg=wg_n, wu=wu_n, wd=wd_n, ckv=ckv_n)

    def chunk_copy(i):
        name, r0, n = CHUNKS[i]
        return pltpu.make_async_copy(hbm[name].at[pl.ds(r0, n)], vm[name].at[pl.ds(r0, n)],
                                     sems.at[i % NSEM])

    def scope(name):
        return jax.named_scope(name) if cfg["scopes"] else _NoScope()

    def wait(i):
        with scope("wait%02d_%s" % (i, CHUNKS[i][0])):
            chunk_copy(i).wait()
        if i + NSEM < NCH:
            chunk_copy(i + NSEM).start()

    def idx(name):
        return [i for i, c in enumerate(CHUNKS) if c[0] == name]

    cx = pltpu.make_async_copy(x_hbm, x_s, sems.at[NSEM])
    cr = pltpu.make_async_copy(wr_hbm, wr_s, sems.at[NSEM + 1])
    cx.start()
    cr.start()
    for i in range(NSEM):
        chunk_copy(i).start()

    FLAG[...] = jnp.ones((8, 128), jnp.int32)

    def repack(src_n, dst, stride, j0, nj):
        def body(j, c):
            a = _u32(src_n[2 * j])
            b = _u32(src_n[2 * j + 1])
            lo = (a & jnp.uint32(0xFFFF)) | (b << 16)
            hi = (a >> 16) | (b & jnp.uint32(0xFFFF0000))
            dst[pl.ds(j, 16, stride=2 * stride), :] = lo
            dst[pl.ds(stride + j, 16, stride=2 * stride), :] = hi
            return c
        lax.fori_loop(j0, j0 + nj, body, 0, unroll=cfg["u_rp"])

    def vpu_transposes(src, stride, kb, dst):
        eye = _eye()

        def body(hv, c):
            tile = _bf(src[pl.ds((NM + hv) * stride + kb * 64, 64), :])
            row = pl.multiple_of(hv * 128, 128)
            dst[pl.ds(row, 128), pl.ds(kb * 128, 128)] = _dot_nt(eye, tile)
            return c
        lax.fori_loop(0, NV, body, 0, unroll=True)

    def prep_wuk_transpose(cb):
        eye = _eye()

        def body(h, c):
            tile = _bf(UP[pl.ds(h * SV + cb * 64, 64), :])
            UT[pl.ds((cb * NM + h) * 64, 64), :] = _transpose_tile(eye, tile)
            return c
        lax.fori_loop(0, NM, body, 0, unroll=True)

    def prep_ckv(kb0, nkb):
        eye = _eye()

        def body(kb, c):
            r0 = pl.multiple_of(kb * 128, 128)
            for cb in range(4):
                tile = ckv_n[pl.ds(r0, 128), pl.ds(cb * 128, 128)]
                CK[pl.ds(cb * 2048 + kb * 64, 64), :] = _u32(tile)
                CKT[pl.ds((kb * 4 + cb) * 64, 64), :] = _transpose_tile(eye, tile)
            return c
        lax.fori_loop(kb0, kb0 + nkb, body, 0, unroll=cfg["u_ckv"])

    def prep_ffn_mxu(src_n, dst, r0, n):
        eye = _eye()

        def body(nb, c):
            row = pl.multiple_of(nb * 128, 128)
            for kb in range(5):
                tile = src_n[pl.ds(row, 128), pl.ds(kb * 128, 128)]
                dst[pl.ds((nb * 5 + kb) * 64, 64), :] = _transpose_tile(eye, tile)
            return c
        lax.fori_loop(r0 // 128, (r0 + n) // 128, body, 0, unroll=True)

    def centered(v):
        return v - jnp.sum(v, axis=1, keepdims=True) * (1.0 / M)

    def unpack_rows(src, r0, n, dst, center):
        step = 16
        nit = n // step
        unroll = max(u for u in range(1, 13) if nit % u == 0)

        def body(i, c):
            r = pl.multiple_of(i * step, step)
            v = src[pl.ds(r0 + r, step), :].astype(F32)
            dst[pl.ds(r, step), :] = centered(v) if center else v
            return c
        lax.fori_loop(0, nit, body, 0, unroll=unroll)

    def center_wqt():
        for i in range(NV * 8):
            rows = pl.ds(i * 16, 16)
            WQT[rows, :] = centered(WQT[rows, :])

    def unpack_wo(h0, nh):
        def body(h, c):
            row = pl.multiple_of((h - NM) * 128, 128)
            WOF[pl.ds(row, 128), :] = wo_n[h].astype(F32)
            return c
        lax.fori_loop(h0, h0 + nh, body, 0)

    def gate(v, marks, frac):
        if not marks or frac <= 0.0:
            return v
        total = marks[-1][0]
        pick = None
        for done, val in marks:
            if done <= frac * total:
                pick = val
        if pick is None:
            return v
        always = FLAG[...] != 0
        return jnp.concatenate(
            [jnp.where(always, v[:, i * 128:(i + 1) * 128], pick) for i in range(v.shape[1] // 128)],
            axis=1)

    def front_mxu_q(xs, marks):
        for h in range(NM):
            r = _dot2(xs, _bf(WQ[pl.ds(h * SQ, 320), :]))
            QD[pl.ds(h * 8, 8), :] = _u32(_split(r))
            marks.append(((marks[-1][0] if marks else 0) + 5, r))

    def front_mxu_qabs(marks):
        for cb in range(4):
            for h in range(NM):
                r = _dot2(_bf(QD[pl.ds(h * 8, 8), :]), _bf(UT[pl.ds((cb * NM + h) * 64, 64), :]))
                QAR[pl.ds(cb * H + h, 1), :] = r[0:1]
                marks.append(((marks[-1][0] if marks else 0) + 1, r))

    def front_vpu(xn, marks):
        a = [None] * 4
        for hv in range(NV):
            xh = gate(xn, marks, cfg["beta"] * (hv - cfg["lag"]) / NV)
            for g in range(16):
                rows = pl.ds(hv * 128 + g * 8, 8)
                qc = jnp.sum(_lane_blocks_sum(WQT[rows, :] * xh), axis=1, keepdims=True)
                for cb in range(4):
                    t = UTF[rows, pl.ds(cb * 128, 128)] * qc
                    a[cb] = a[cb] + t if g > 0 else t
            for cb in range(4):
                PS[pl.ds((cb * NV + hv) * SP, 8), :] = a[cb]
        for cb in range(4):
            for hv0 in range(0, NV, 8):
                n = min(8, NV - hv0)
                tot = None
                for s_ in range(8):
                    t = PS[pl.ds((cb * NV + hv0) * SP + s_, n, stride=SP), :]
                    tot = t if tot is None else tot + t
                QAR[pl.ds(cb * H + NM + hv0, n), :] = tot

    def finish_front(mean, rstd):
        row = lax.broadcasted_iota(jnp.int32, (H, 1), 0)
        mean32 = jnp.concatenate([mean] * 4, axis=0)
        rstd32 = jnp.concatenate([rstd] * 4, axis=0)
        off = jnp.where(row < NM, mean32, 0.0)
        mul = rstd32 * (D ** -0.5)
        return jnp.concatenate(
            [((QAR[pl.ds(cb * H, H), :] - off * CSA[pl.ds(cb * H, H), :]) * mul).astype(BF)
             for cb in range(4)], axis=1)

    def scores(qa, nb0, nnb):
        return jnp.concatenate(
            [_dot(qa, _bf(CKT[pl.ds(nb * 256, 256), :])) for nb in range(nb0, nb0 + nnb)], axis=1)

    def pv(p, kb0, nkb):
        return jnp.concatenate(
            [_dot(p, _bf(CK[pl.ds(cb * 2048 + kb0 * 64, nkb * 64), :])) for cb in range(4)], axis=1)

    def stage_attn(qa):
        sa = scores(qa, 0, 16)
        sb = scores(qa, 16, 16)
        ma = jnp.max(sa, axis=1, keepdims=True)
        pa = jnp.exp(sa - ma)
        la = jnp.sum(pa, axis=1, keepdims=True)
        ca = pv(pa.astype(BF), 0, 16)
        m = jnp.maximum(ma, jnp.max(sb, axis=1, keepdims=True))
        pb = jnp.exp(sb - m)
        lb = jnp.sum(pb, axis=1, keepdims=True)
        cbv = pv(pb.astype(BF), 16, 16)
        alpha = jnp.exp(ma - m)
        inv = 1.0 / (alpha * la + lb)
        cl = (alpha * ca + cbv) * inv
        bits = pltpu.bitcast(cl.astype(BF).astype(F32), U32)
        dupw = bits | (bits >> 16)
        for cb in range(4):
            CL[pl.ds(cb * H, H), :] = dupw[:, cb * 128:(cb + 1) * 128]
            CLF[pl.ds(cb * H, H), :] = cl[:, cb * 128:(cb + 1) * 128]

    def ctx_mxu(marks):
        for h in range(NM):
            lhs = jnp.concatenate(
                [_bf(CL[pl.ds(cb * H + h, 8, stride=0), :]) for cb in range(4)], axis=1)
            r = _dot(lhs, _bf(UV[pl.ds(h * SV, 256), :]))[0:8]
            QD[pl.ds(h * 8, 8), :] = _u32(_dup(r))
            marks.append(((marks[-1][0] if marks else 0) + 4, r))

    def out_mxu(h0, nh, acc, first, marks):
        for h in range(h0, h0 + nh):
            if first:
                w = wo_n[h]
                for mb in range(5):
                    WOU[pl.ds((h * 5 + mb) * 64, 64), :] = _u32(w[:, mb * 128:(mb + 1) * 128])
            else:
                w = jnp.concatenate(
                    [_bf(WOU[pl.ds((h * 5 + mb) * 64, 64), :]) for mb in range(5)], axis=1)
            r = _dot(_bf(QD[pl.ds(h * 8, 8), :]), w)[0:8]
            acc = acc + r
            marks.append(((marks[-1][0] if marks else 0) + 5, r[:, 0:128]))
        return acc

    def back_vpu(h0, nh, acc, marks):
        for h in range(h0, h0 + nh):
            hv = h - NM
            cl = jnp.concatenate(
                [CLF[pl.ds(cb * H + h, 8, stride=0), :] for cb in range(4)], axis=1)
            cl = gate(cl, marks, cfg["beta"] * (hv - cfg["lag"]) / NV)
            for g in range(16):
                rows = pl.ds(hv * 128 + g * 8, 8)
                cc = jnp.sum(_lane_blocks_sum(UVT[rows, :] * cl), axis=1, keepdims=True)
                acc = acc + WOF[rows, :] * cc
        return acc

    def gate_up_mxu_raw(xs, marks):
        g, u = [], []
        for nb in range(NFM):
            g.append(_dot2(xs, _bf(GT[pl.ds(nb * 320, 320), :])))
            marks.append(((marks[-1][0] if marks else 0) + 5, g[-1]))
            u.append(_dot2(xs, _bf(UPT[pl.ds(nb * 320, 320), :])))
            marks.append((marks[-1][0] + 5, u[-1]))
        return g, u

    def gate_up_mxu(xs, mean, rstd, marks):
        g, u = gate_up_mxu_raw(xs, marks)
        hd = []
        for nb in range(NFM):
            cols = pl.ds(nb * 128, 128)
            gg = (g[nb] - mean * CSG[:, cols]) * rstd
            uu = (u[nb] - mean * CSU[:, cols]) * rstd
            hd.append(_dup(_swiglu(gg, uu)))
        return hd

    def down_mxu(hd, nb0, nb1, acc, first, marks):
        for nb in range(nb0, nb1):
            if first:
                w = wd_n[pl.ds(nb * 128, 128), :]
                for mb in range(5):
                    WDU[pl.ds((nb * 5 + mb) * 64, 64), :] = _u32(w[:, mb * 128:(mb + 1) * 128])
            else:
                w = jnp.concatenate(
                    [_bf(WDU[pl.ds((nb * 5 + mb) * 64, 64), :]) for mb in range(5)], axis=1)
            r = _dot(hd[nb], w)[0:8]
            acc = acc + r
            marks.append(((marks[-1][0] if marks else 0) + 5, r[:, 0:128]))
        return acc

    def ffn_vpu(x8, rstd, marks):
        acc = None
        xg = x8
        for g in range(NG):
            if g % 8 == 0:
                xg = gate(x8, marks, cfg["beta"] * (g - 8 * cfg["lag"]) / NG)
            rows = pl.ds(g * 8, 8)
            gc = jnp.sum(_lane_blocks_sum(GF[rows, :] * xg), axis=1, keepdims=True)
            uc = jnp.sum(_lane_blocks_sum(UF[rows, :] * xg), axis=1, keepdims=True)
            t = DF[rows, :] * _swiglu(gc * rstd, uc * rstd)
            acc = t if acc is None else acc + t
        return acc

    def gate_scalar(xn, wr8):
        return jax.nn.sigmoid(jnp.sum(xn * wr8, axis=1, keepdims=True))

    ones_split = jnp.concatenate([jnp.ones((8, M), BF), jnp.zeros((8, M), BF)], axis=0)

    cx.wait()
    cr.wait()
    x = jnp.broadcast_to(x_s[0].astype(F32), (8, M))
    wr8 = jnp.broadcast_to(wr_s[...].reshape(1, M).astype(F32), (8, M))

    if not cfg["compute1"]:
        for i in range(NCH):
            wait(i)
        o_ref[0] = x[0:1].astype(BF)
        return

    for k, i in enumerate(idx("wq")):
        wait(i)
        with scope("p_wq"):
            repack(wq_n, WQ, SQ, k * 64, 64)
            vpu_transposes(WQ, SQ, k, WQT)
    with scope("s1_csq"):
        center_wqt()
        front_mxu_q(ones_split, [])
    for k, i in enumerate(idx("wuk")):
        wait(i)
        with scope("p_wuk"):
            repack(wuk_n, UP, SV, k * 64, 64)
            prep_wuk_transpose(k)
            vpu_transposes(UP, SV, k, UTF)
    with scope("s1_csa"):
        front_mxu_qabs([])
        for cb in range(4):
            CSA[pl.ds(cb * H, NM), :] = QAR[pl.ds(cb * H, NM), :]
            CSA[pl.ds(cb * H + NM, NV), :] = jnp.zeros((NV, 128), F32)
    with scope("s1_front"):
        mean, rstd = _ln_stats(x)
        front_mxu_q(_split(x), [])
        front_mxu_qabs([])
        front_vpu(x, [])
        qa = finish_front(mean, rstd)
    for k, i in enumerate(idx("ckv")):
        wait(i)
        with scope("p_ckv"):
            prep_ckv(k * 8, 8)
    with scope("s1_attn"):
        stage_attn(qa)
    for k, i in enumerate(idx("wuv")):
        wait(i)
        with scope("p_wuv"):
            repack(wuv_n, UV, SV, k * 64, 64)
            vpu_transposes(UV, SV, k, UVT)
    with scope("s1_ctx"):
        ctx_mxu([])
    acc_v = jnp.zeros((8, M), F32)
    acc_m = jnp.zeros((8, M), F32)
    for i in idx("wo"):
        wait(i)
        h0, nh = CHUNKS[i][1], CHUNKS[i][2]
        with scope("s1_out"):
            if h0 >= NM:
                unpack_wo(h0, nh)
                acc_v = back_vpu(h0, nh, acc_v, [])
            else:
                acc_m = out_mxu(h0, nh, acc_m, True, [])
    x = x + acc_m + _row_total(acc_v)
    for name, nat, tr, fl in (("wg", wg_n, GT, GF), ("wu", wu_n, UPT, UF)):
        for i in idx(name):
            wait(i)
            r0, n = CHUNKS[i][1], CHUNKS[i][2]
            with scope("p_" + name):
                if r0 >= FM:
                    unpack_rows(nat, r0, n, fl, True)
                else:
                    prep_ffn_mxu(nat, tr, r0, n)
    with scope("s2_cs"):
        g, u = gate_up_mxu_raw(ones_split, [])
        CSG[...] = jnp.concatenate(g, axis=1)
        CSU[...] = jnp.concatenate(u, axis=1)
    wd_idx = idx("wd")
    wait(wd_idx[0])
    with scope("p_wd"):
        unpack_rows(wd_n, FM, F - FM, DF, False)
    with scope("s2_gu"):
        mean, rstd = _ln_stats(x)
        xn = (x - mean) * rstd
        hd = gate_up_mxu(_split(x), mean, rstd, [])
        acc_v = ffn_vpu(x, rstd, [])
        sg = gate_scalar(xn, wr8)
    acc_m = _row_total(acc_v)
    for i in wd_idx[1:]:
        wait(i)
        r0, n = CHUNKS[i][1], CHUNKS[i][2]
        with scope("s2_down"):
            acc_m = down_mxu(hd, r0 // 128, (r0 + n) // 128, acc_m, True, [])
    x = x + xn + acc_m * sg

    if cfg["phase2"]:
        with scope("phase2"):
            mean, rstd = _ln_stats(x)
            marks = []
            front_mxu_q(_split(x), marks)
            front_mxu_qabs(marks)
            front_vpu(x, marks if cfg["gate"] else [])
            stage_attn(finish_front(mean, rstd))
            marks = []
            ctx_mxu(marks)
            acc_m = out_mxu(0, NM, jnp.zeros((8, M), F32), False, marks)
            acc_v = back_vpu(NM, NV, jnp.zeros((8, M), F32), marks if cfg["gate"] else [])
            x = x + acc_m + _row_total(acc_v)
            mean, rstd = _ln_stats(x)
            xn = (x - mean) * rstd
            marks = []
            hd = gate_up_mxu(_split(x), mean, rstd, marks)
            y = down_mxu(hd, 0, NFM, jnp.zeros((8, M), F32), False, marks)
            acc_v = ffn_vpu(x, rstd, marks if cfg["gate"] else [])
            sg = gate_scalar(xn, wr8)
            x = x + xn + (y + _row_total(acc_v)) * sg

    o_ref[0] = x[0:1].astype(BF)


def _run(cfg, A_x, A_c_kv, A_w_q, A_w_uk, A_w_uv, A_w_o, B_w_r, B_w_gate, B_w_up, B_w_down):
    any_spec = pl.BlockSpec(memory_space=pl.ANY)
    nm = cfg["nm"]
    nv = H - nm
    fm = cfg["fm"]
    nsem = min(cfg["nsem"], len(_chunks(cfg)))
    scratch = [
        pltpu.VMEM((1, 1, M), BF),
        pltpu.VMEM((M,), BF),
        pltpu.VMEM((M, H, D), BF),
        pltpu.VMEM((DC, H, D), BF),
        pltpu.VMEM((DC, H, D), BF),
        pltpu.VMEM((SK, DC), BF),
        pltpu.VMEM((H, D, M), BF),
        pltpu.VMEM((F, M), BF),
        pltpu.VMEM((F, M), BF),
        pltpu.VMEM((F, M), BF),
        pltpu.VMEM((H * SQ, 128), U32),
        pltpu.VMEM((H * SV, 128), U32),
        pltpu.VMEM((4 * nm * 64, 128), U32),
        pltpu.VMEM((H * SV, 128), U32),
        pltpu.VMEM((32 * 4 * 64, 128), U32),
        pltpu.VMEM((4 * 2048, 128), U32),
        pltpu.VMEM((fm // 128 * 320, 128), U32),
        pltpu.VMEM((fm // 128 * 320, 128), U32),
        pltpu.VMEM((H * 8, 128), U32),
        pltpu.VMEM((4 * H, 128), U32),
        pltpu.VMEM((nv * 128, M), F32),
        pltpu.VMEM((nv * 128, DC), F32),
        pltpu.VMEM((nv * 128, DC), F32),
        pltpu.VMEM((nv * 128, M), F32),
        pltpu.VMEM((F - fm, M), F32),
        pltpu.VMEM((F - fm, M), F32),
        pltpu.VMEM((F - fm, M), F32),
        pltpu.VMEM((4 * H, 128), F32),
        pltpu.VMEM((8, fm), F32),
        pltpu.VMEM((8, fm), F32),
        pltpu.VMEM((4 * H, 128), F32),
        pltpu.VMEM((4 * H, 128), F32),
        pltpu.VMEM((4 * nv * SP, 128), F32),
        pltpu.VMEM((nm * 5 * 64, 128), U32),
        pltpu.VMEM((fm // 128 * 5 * 64, 128), U32),
        pltpu.VMEM((8, 128), jnp.int32),
        pltpu.SemaphoreType.DMA((nsem + 2,)),
    ]
    return pl.pallas_call(
        functools.partial(_kernel, cfg),
        out_shape=jax.ShapeDtypeStruct((1, 1, M), BF),
        in_specs=[any_spec] * 10,
        out_specs=pl.BlockSpec(memory_space=pltpu.VMEM),
        scratch_shapes=scratch,
        compiler_params=pltpu.CompilerParams(vmem_limit_bytes=110 * 1024 * 1024),
    )(A_x, A_c_kv, A_w_q, A_w_uk, A_w_uv, A_w_o, B_w_r, B_w_gate.T, B_w_up.T, B_w_down)


def build(**overrides):
    cfg = dict(DEFAULT_CFG, **overrides)

    @jax.jit
    def fn(A_x, A_c_kv, A_w_q, A_w_uk, A_w_uv, A_w_o, B_x, B_w_r, B_w_gate, B_w_up, B_w_down):
        return _run(cfg, A_x, A_c_kv, A_w_q, A_w_uk, A_w_uv, A_w_o, B_w_r, B_w_gate, B_w_up, B_w_down)
    return fn


@jax.jit
def pallas_interleave_layers__compressed_kv_cla__moe_arch_mod__decode_kernel(
    A_x: jax.Array,
    A_c_kv: jax.Array,
    A_w_q: jax.Array,
    A_w_uk: jax.Array,
    A_w_uv: jax.Array,
    A_w_o: jax.Array,
    B_x: jax.Array,
    B_w_r: jax.Array,
    B_w_gate: jax.Array,
    B_w_up: jax.Array,
    B_w_down: jax.Array,
):
    del B_x
    return _run(DEFAULT_CFG, A_x, A_c_kv, A_w_q, A_w_uk, A_w_uv, A_w_o, B_w_r, B_w_gate, B_w_up,
                B_w_down)
```

```python
import functools

import jax
import jax.numpy as jnp
from jax import lax
from jax.experimental import pallas as pl
from jax.experimental.pallas import tpu as pltpu

M = 640
H = 32
D = 128
DC = 512
SK = 4096
F = 1728
EPS = 1e-5

SQ = 322
SP = 9
SV = 258

BF = jnp.bfloat16
F32 = jnp.float32
U32 = jnp.uint32


def _bf(u32_val):
    return pltpu.bitcast(u32_val, BF)


def _u32(bf_val):
    return pltpu.bitcast(bf_val, U32)


def _dup(v8):
    return jnp.concatenate([v8, v8], axis=0).astype(BF)


def _dot(a, b):
    return jnp.dot(a, b, preferred_element_type=F32)


def _dot_nt(a, b):
    return lax.dot_general(a, b, (((1,), (1,)), ((), ())), preferred_element_type=F32)


def _split(v8):
    hi = pltpu.bitcast(pltpu.bitcast(v8, U32) & jnp.uint32(0xFFFF0000), F32)
    return jnp.concatenate([hi, v8 - hi], axis=0).astype(BF)


def _dot2(a16, b):
    r = _dot(a16, b)
    return r[0:8] + r[8:16]


def _ln_stats(x8):
    s1 = jnp.sum(x8, axis=1, keepdims=True)
    s2 = jnp.sum(x8 * x8, axis=1, keepdims=True)
    mean = s1 * (1.0 / M)
    var = jnp.maximum(s2 * (1.0 / M) - mean * mean, 0.0)
    return mean, lax.rsqrt(var + EPS)


def _swiglu(g, u):
    a = 0.5 * g
    b = a * u
    return b * jnp.tanh(a) + b


def _bcast_row(ref, row):
    return jnp.broadcast_to(ref[pl.ds(row, 1), :], (8, 128))


def _lane_blocks_sum(p):
    n = p.shape[1] // 128
    acc = p[:, 0:128]
    for i in range(1, n):
        acc = acc + p[:, i * 128:(i + 1) * 128]
    return acc


def _row_total(a8):
    return jnp.broadcast_to(jnp.sum(a8, axis=0, keepdims=True), a8.shape)


def _eye():
    r = lax.broadcasted_iota(jnp.int32, (128, 128), 0)
    c = lax.broadcasted_iota(jnp.int32, (128, 128), 1)
    return jnp.where(r == c, 1.0, 0.0).astype(BF)


def _transpose_tile(eye, tile):
    return _u32(_dot_nt(eye, tile).astype(BF))


def _chunks(cfg):
    fm = cfg["fm"]
    nm = cfg["nmb"]
    ch = []
    ch += [("wq", i * 128, 128) for i in range(5)]
    ch += [("wuk", i * 128, 128) for i in range(4)]
    ch += [("ckv", i * 1024, 1024) for i in range(4)]
    ch += [("wuv", i * 128, 128) for i in range(4)]
    ch += [("wo", h0, min(8, H - h0)) for h0 in range(nm, H, 8)]
    ch += [("wo", h0, min(8, nm - h0)) for h0 in range(0, nm, 8)]
    for name in ("wg", "wu"):
        ch += [(name, fm, F - fm)]
        ch += [(name, r0, min(512, fm - r0)) for r0 in range(0, fm, 512)]
    late = cfg["late"]
    ch += [("wd", fm, F - fm - late)]
    r0 = 0
    while r0 < fm - 128:
        n = min(512, fm - 128 - r0)
        ch.append(("wd", r0, n))
        r0 += n
    ch.append(("wd", fm - 128, 128))
    if late:
        ch.append(("wd", F - late, late))
    return ch


DEFAULT_CFG = dict(phase2=True, compute1=True, scopes=False, u_uk=16, u_ckv=4, u_rp=4,
                   nmf=17, nmb=17, fm=1024, gate=True, nsem=5,
                   lag_f=2, beta_f=1.0, lag_b=3, beta_b=1.0, lag_n=8, beta_n=1.0, gstep=8, late=128, small_after=0)


class _NoScope:
    def __enter__(self):
        return self

    def __exit__(self, *a):
        return False


def _kernel(cfg, x_hbm, ckv_hbm, wq_hbm, wuk_hbm, wuv_hbm, wo_hbm, wr_hbm, wg_hbm, wu_hbm, wd_hbm,
            o_ref,
            x_s, wr_s, wq_n, wuk_n, wuv_n, ckv_n, wo_n, wg_n, wu_n, wd_n,
            WQ, UP, UT, UV, CKT, CK, GT, UPT, QD, CL,
            WQT, UTF, UVT, WOF, GF, UF, DF, CSA, CSG, CSU, CLF, QAR, PS, WOU, WDU, FLAG,
            sems):
    NMF = cfg["nmf"]
    NVF = H - NMF
    NMB = cfg["nmb"]
    NVB = H - NMB
    FM = cfg["fm"]
    NFM = FM // 128
    NG = (F - FM) // 8
    CHUNKS = _chunks(cfg)
    NCH = len(CHUNKS)
    NSEM = min(cfg["nsem"], NCH)

    hbm = dict(wq=wq_hbm, wuk=wuk_hbm, wuv=wuv_hbm, wo=wo_hbm, wg=wg_hbm, wu=wu_hbm, wd=wd_hbm,
               ckv=ckv_hbm.at[0])
    vm = dict(wq=wq_n, wuk=wuk_n, wuv=wuv_n, wo=wo_n, wg=wg_n, wu=wu_n, wd=wd_n, ckv=ckv_n)

    def chunk_copy(i):
        name, r0, n = CHUNKS[i]
        return pltpu.make_async_copy(hbm[name].at[pl.ds(r0, n)], vm[name].at[pl.ds(r0, n)],
                                     sems.at[(i + 2) % NSEM])

    def scope(name):
        return jax.named_scope(name) if cfg["scopes"] else _NoScope()

    def wait(i):
        with scope("wait%02d_%s" % (i, CHUNKS[i][0])):
            chunk_copy(i).wait()
        if i + NSEM < NCH:
            chunk_copy(i + NSEM).start()

    def idx(name):
        return [i for i, c in enumerate(CHUNKS) if c[0] == name]

    cx = pltpu.make_async_copy(x_hbm, x_s, sems.at[0])
    cr = pltpu.make_async_copy(wr_hbm, wr_s, sems.at[1])
    for i in range(NSEM - 2):
        if i == cfg["small_after"]:
            cx.start()
            cr.start()
        chunk_copy(i).start()

    FLAG[...] = jnp.ones((8, 128), jnp.int32)

    def repack(src_n, dst, stride, j0, nj):
        def body(j, c):
            a = _u32(src_n[2 * j])
            b = _u32(src_n[2 * j + 1])
            lo = (a & jnp.uint32(0xFFFF)) | (b << 16)
            hi = (a >> 16) | (b & jnp.uint32(0xFFFF0000))
            dst[pl.ds(j, 16, stride=2 * stride), :] = lo
            dst[pl.ds(stride + j, 16, stride=2 * stride), :] = hi
            return c
        lax.fori_loop(j0, j0 + nj, body, 0, unroll=cfg["u_rp"])

    def vpu_transposes(src, stride, kb, dst, NM):
        eye = _eye()

        def body(hv, c):
            tile = _bf(src[pl.ds((NM + hv) * stride + kb * 64, 64), :])
            row = pl.multiple_of(hv * 128, 128)
            dst[pl.ds(row, 128), pl.ds(kb * 128, 128)] = _dot_nt(eye, tile)
            return c
        lax.fori_loop(0, H - NM, body, 0, unroll=True)

    def prep_wuk_transpose(cb):
        eye = _eye()

        def body(h, c):
            tile = _bf(UP[pl.ds(h * SV + cb * 64, 64), :])
            UT[pl.ds((cb * NMF + h) * 64, 64), :] = _transpose_tile(eye, tile)
            return c
        lax.fori_loop(0, NMF, body, 0, unroll=True)

    def prep_ckv(kb0, nkb):
        eye = _eye()

        def body(kb, c):
            r0 = pl.multiple_of(kb * 128, 128)
            for cb in range(4):
                tile = ckv_n[pl.ds(r0, 128), pl.ds(cb * 128, 128)]
                CK[pl.ds(cb * 2048 + kb * 64, 64), :] = _u32(tile)
                CKT[pl.ds((kb * 4 + cb) * 64, 64), :] = _transpose_tile(eye, tile)
            return c
        lax.fori_loop(kb0, kb0 + nkb, body, 0, unroll=cfg["u_ckv"])

    def prep_ffn_mxu(src_n, dst, r0, n):
        eye = _eye()

        def body(nb, c):
            row = pl.multiple_of(nb * 128, 128)
            for kb in range(5):
                tile = src_n[pl.ds(row, 128), pl.ds(kb * 128, 128)]
                dst[pl.ds((nb * 5 + kb) * 64, 64), :] = _transpose_tile(eye, tile)
            return c
        lax.fori_loop(r0 // 128, (r0 + n) // 128, body, 0, unroll=True)

    def centered(v):
        return v - jnp.sum(v, axis=1, keepdims=True) * (1.0 / M)

    def unpack_rows(src, r0, n, dst, center):
        step = 16
        nit = n // step
        unroll = max(u for u in range(1, 13) if nit % u == 0)

        def body(i, c):
            r = pl.multiple_of(i * step, step)
            v = src[pl.ds(r0 + r, step), :].astype(F32)
            dst[pl.ds(r, step), :] = centered(v) if center else v
            return c
        lax.fori_loop(0, nit, body, 0, unroll=unroll)

    def center_wqt():
        for i in range(NVF * 8):
            rows = pl.ds(i * 16, 16)
            WQT[rows, :] = centered(WQT[rows, :])

    def unpack_wo(h0, nh):
        def body(h, c):
            row = pl.multiple_of((h - NMB) * 128, 128)
            WOF[pl.ds(row, 128), :] = wo_n[h].astype(F32)
            return c
        lax.fori_loop(h0, h0 + nh, body, 0)

    def gate(v, marks, frac):
        if not marks or frac <= 0.0:
            return v
        total = marks[-1][0]
        pick = None
        for done, val in marks:
            if done <= frac * total:
                pick = val
        if pick is None:
            return v
        always = FLAG[...] != 0
        return jnp.concatenate(
            [jnp.where(always, v[:, i * 128:(i + 1) * 128], pick) for i in range(v.shape[1] // 128)],
            axis=1)

    def front_mxu_q(xs, marks):
        for h in range(NMF):
            r = _dot2(xs, _bf(WQ[pl.ds(h * SQ, 320), :]))
            QD[pl.ds(h * 8, 8), :] = _u32(_split(r))
            marks.append(((marks[-1][0] if marks else 0) + 5, r))

    def front_mxu_qabs(marks):
        for cb in range(4):
            for h in range(NMF):
                r = _dot2(_bf(QD[pl.ds(h * 8, 8), :]), _bf(UT[pl.ds((cb * NMF + h) * 64, 64), :]))
                QAR[pl.ds(cb * H + h, 1), :] = r[0:1]
                marks.append(((marks[-1][0] if marks else 0) + 1, r))

    def front_vpu(xn, marks):
        a = [None] * 4
        for hv in range(NVF):
            xh = gate(xn, marks, cfg["beta_f"] * (hv - cfg["lag_f"]) / NVF)
            for g in range(16):
                rows = pl.ds(hv * 128 + g * 8, 8)
                qc = jnp.sum(_lane_blocks_sum(WQT[rows, :] * xh), axis=1, keepdims=True)
                for cb in range(4):
                    t = UTF[rows, pl.ds(cb * 128, 128)] * qc
                    a[cb] = a[cb] + t if g > 0 else t
            for cb in range(4):
                PS[pl.ds((cb * NVF + hv) * SP, 8), :] = a[cb]
        for cb in range(4):
            for hv0 in range(0, NVF, 8):
                n = min(8, NVF - hv0)
                tot = None
                for s_ in range(8):
                    t = PS[pl.ds((cb * NVF + hv0) * SP + s_, n, stride=SP), :]
                    tot = t if tot is None else tot + t
                QAR[pl.ds(cb * H + NMF + hv0, n), :] = tot

    def finish_front(mean, rstd):
        row = lax.broadcasted_iota(jnp.int32, (H, 1), 0)
        mean32 = jnp.concatenate([mean] * 4, axis=0)
        rstd32 = jnp.concatenate([rstd] * 4, axis=0)
        off = jnp.where(row < NMF, mean32, 0.0)
        mul = rstd32 * (D ** -0.5)
        return jnp.concatenate(
            [((QAR[pl.ds(cb * H, H), :] - off * CSA[pl.ds(cb * H, H), :]) * mul).astype(BF)
             for cb in range(4)], axis=1)

    def scores(qa, nb0, nnb):
        return jnp.concatenate(
            [_dot(qa, _bf(CKT[pl.ds(nb * 256, 256), :])) for nb in range(nb0, nb0 + nnb)], axis=1)

    def pv(p, kb0, nkb):
        return jnp.concatenate(
            [_dot(p, _bf(CK[pl.ds(cb * 2048 + kb0 * 64, nkb * 64), :])) for cb in range(4)], axis=1)

    def stage_attn(qa):
        sa = scores(qa, 0, 16)
        sb = scores(qa, 16, 16)
        ma = jnp.max(sa, axis=1, keepdims=True)
        pa = jnp.exp(sa - ma)
        la = jnp.sum(pa, axis=1, keepdims=True)
        ca = pv(pa.astype(BF), 0, 16)
        m = jnp.maximum(ma, jnp.max(sb, axis=1, keepdims=True))
        pb = jnp.exp(sb - m)
        lb = jnp.sum(pb, axis=1, keepdims=True)
        cbv = pv(pb.astype(BF), 16, 16)
        alpha = jnp.exp(ma - m)
        inv = 1.0 / (alpha * la + lb)
        cl = (alpha * ca + cbv) * inv
        bits = pltpu.bitcast(cl.astype(BF).astype(F32), U32)
        dupw = bits | (bits >> 16)
        for cb in range(4):
            CL[pl.ds(cb * H, H), :] = dupw[:, cb * 128:(cb + 1) * 128]
            CLF[pl.ds(cb * H, H), :] = cl[:, cb * 128:(cb + 1) * 128]

    def ctx_mxu(marks):
        for h in range(NMB):
            lhs = jnp.concatenate(
                [_bf(_bcast_row(CL, cb * H + h)) for cb in range(4)], axis=1)
            r = _dot(lhs, _bf(UV[pl.ds(h * SV, 256), :]))[0:8]
            QD[pl.ds(h * 8, 8), :] = _u32(_dup(r))
            marks.append(((marks[-1][0] if marks else 0) + 4, r))

    def out_mxu(h0, nh, acc, first, marks):
        for h in range(h0, h0 + nh):
            if first:
                w = wo_n[h]
                for mb in range(5):
                    WOU[pl.ds((h * 5 + mb) * 64, 64), :] = _u32(w[:, mb * 128:(mb + 1) * 128])
            else:
                w = jnp.concatenate(
                    [_bf(WOU[pl.ds((h * 5 + mb) * 64, 64), :]) for mb in range(5)], axis=1)
            r = _dot(_bf(QD[pl.ds(h * 8, 8), :]), w)[0:8]
            acc = acc + r
            marks.append(((marks[-1][0] if marks else 0) + 5, r[:, 0:128]))
        return acc

    def back_vpu(h0, nh, acc, marks):
        for h in range(h0, h0 + nh):
            hv = h - NMB
            cl = jnp.concatenate(
                [_bcast_row(CLF, cb * H + h) for cb in range(4)], axis=1)
            cl = gate(cl, marks, cfg["beta_b"] * (hv - cfg["lag_b"]) / NVB)
            for g in range(16):
                rows = pl.ds(hv * 128 + g * 8, 8)
                cc = jnp.sum(_lane_blocks_sum(UVT[rows, :] * cl), axis=1, keepdims=True)
                acc = acc + WOF[rows, :] * cc
        return acc

    def gate_up_mxu_raw(xs, marks):
        g, u = [], []
        for nb in range(NFM):
            g.append(_dot2(xs, _bf(GT[pl.ds(nb * 320, 320), :])))
            marks.append(((marks[-1][0] if marks else 0) + 5, g[-1]))
            u.append(_dot2(xs, _bf(UPT[pl.ds(nb * 320, 320), :])))
            marks.append((marks[-1][0] + 5, u[-1]))
        return g, u

    def gate_up_mxu(xs, mean, rstd, marks):
        g, u = gate_up_mxu_raw(xs, marks)
        hd = []
        for nb in range(NFM):
            cols = pl.ds(nb * 128, 128)
            gg = (g[nb] - mean * CSG[:, cols]) * rstd
            uu = (u[nb] - mean * CSU[:, cols]) * rstd
            hd.append(_dup(_swiglu(gg, uu)))
        return hd

    def down_mxu(hd, nb0, nb1, acc, first, marks):
        for nb in range(nb0, nb1):
            if first:
                w = wd_n[pl.ds(nb * 128, 128), :]
                for mb in range(5):
                    WDU[pl.ds((nb * 5 + mb) * 64, 64), :] = _u32(w[:, mb * 128:(mb + 1) * 128])
            else:
                w = jnp.concatenate(
                    [_bf(WDU[pl.ds((nb * 5 + mb) * 64, 64), :]) for mb in range(5)], axis=1)
            r = _dot(hd[nb], w)[0:8]
            acc = acc + r
            marks.append(((marks[-1][0] if marks else 0) + 5, r[:, 0:128]))
        return acc

    def ffn_vpu(x8, rstd, marks, nlate=0):
        acc = None
        xg = x8
        hcols = []
        for g in range(NG):
            if g % cfg["gstep"] == 0:
                xg = gate(x8, marks, cfg["beta_n"] * (g - cfg["lag_n"]) / NG)
            rows = pl.ds(g * 8, 8)
            gc = jnp.sum(_lane_blocks_sum(GF[rows, :] * xg), axis=1, keepdims=True)
            uc = jnp.sum(_lane_blocks_sum(UF[rows, :] * xg), axis=1, keepdims=True)
            hc = _swiglu(gc * rstd, uc * rstd)
            if g >= NG - nlate:
                hcols.append(hc)
            else:
                t = DF[rows, :] * hc
                acc = t if acc is None else acc + t
        return acc, hcols

    def gate_scalar(xn, wr8):
        return jax.nn.sigmoid(jnp.sum(xn * wr8, axis=1, keepdims=True))

    ones_split = jnp.concatenate([jnp.ones((8, M), BF), jnp.zeros((8, M), BF)], axis=0)

    cx.wait()
    chunk_copy(NSEM - 2).start()
    cr.wait()
    chunk_copy(NSEM - 1).start()
    x = jnp.broadcast_to(x_s[0].astype(F32), (8, M))
    wr8 = jnp.broadcast_to(wr_s[...].reshape(1, M).astype(F32), (8, M))

    if not cfg["compute1"]:
        for i in range(NCH):
            wait(i)
        o_ref[0] = x[0:1].astype(BF)
        return

    for k, i in enumerate(idx("wq")):
        wait(i)
        with scope("p_wq"):
            repack(wq_n, WQ, SQ, k * 64, 64)
            vpu_transposes(WQ, SQ, k, WQT, NMF)
    with scope("s1_csq"):
        center_wqt()
        front_mxu_q(ones_split, [])
    for k, i in enumerate(idx("wuk")):
        wait(i)
        with scope("p_wuk"):
            repack(wuk_n, UP, SV, k * 64, 64)
            prep_wuk_transpose(k)
            vpu_transposes(UP, SV, k, UTF, NMF)
    with scope("s1_csa"):
        front_mxu_qabs([])
        for cb in range(4):
            CSA[pl.ds(cb * H, NMF), :] = QAR[pl.ds(cb * H, NMF), :]
            CSA[pl.ds(cb * H + NMF, NVF), :] = jnp.zeros((NVF, 128), F32)
    with scope("s1_front"):
        mean, rstd = _ln_stats(x)
        front_mxu_q(_split(x), [])
        front_mxu_qabs([])
        front_vpu(x, [])
        qa = finish_front(mean, rstd)
    for k, i in enumerate(idx("ckv")):
        wait(i)
        with scope("p_ckv"):
            prep_ckv(k * 8, 8)
    with scope("s1_attn"):
        stage_attn(qa)
    for k, i in enumerate(idx("wuv")):
        wait(i)
        with scope("p_wuv"):
            repack(wuv_n, UV, SV, k * 64, 64)
            vpu_transposes(UV, SV, k, UVT, NMB)
    with scope("s1_ctx"):
        ctx_mxu([])
    acc_v = jnp.zeros((8, M), F32)
    acc_m = jnp.zeros((8, M), F32)
    for i in idx("wo"):
        wait(i)
        h0, nh = CHUNKS[i][1], CHUNKS[i][2]
        with scope("s1_out"):
            if h0 >= NMB:
                unpack_wo(h0, nh)
                acc_v = back_vpu(h0, nh, acc_v, [])
            else:
                acc_m = out_mxu(h0, nh, acc_m, True, [])
    x = x + acc_m + _row_total(acc_v)
    for name, nat, tr, fl in (("wg", wg_n, GT, GF), ("wu", wu_n, UPT, UF)):
        for i in idx(name):
            wait(i)
            r0, n = CHUNKS[i][1], CHUNKS[i][2]
            with scope("p_" + name):
                if r0 >= FM:
                    unpack_rows(nat, r0, n, fl, True)
                else:
                    prep_ffn_mxu(nat, tr, r0, n)
    with scope("s2_cs"):
        g, u = gate_up_mxu_raw(ones_split, [])
        CSG[...] = jnp.concatenate(g, axis=1)
        CSU[...] = jnp.concatenate(u, axis=1)
    wd_idx = idx("wd")
    LATE = cfg["late"]
    wait(wd_idx[0])
    with scope("p_wd"):
        unpack_rows(wd_n, FM, F - FM - LATE, DF, False)
    with scope("s2_gu"):
        mean, rstd = _ln_stats(x)
        xn = (x - mean) * rstd
        hd = gate_up_mxu(_split(x), mean, rstd, [])
        acc_v, hcols = ffn_vpu(x, rstd, [], LATE // 8)
        sg = gate_scalar(xn, wr8)
    acc_m = jnp.zeros((8, M), F32)
    for i in wd_idx[1:]:
        wait(i)
        r0, n = CHUNKS[i][1], CHUNKS[i][2]
        with scope("s2_down"):
            if r0 < FM:
                acc_m = down_mxu(hd, r0 // 128, (r0 + n) // 128, acc_m, True, [])
            else:
                for j in range(n // 16):
                    v = wd_n[pl.ds(r0 + j * 16, 16), :].astype(F32)
                    DF[pl.ds(r0 - FM + j * 16, 16), :] = v
                    acc_v = acc_v + v[0:8] * hcols[2 * j] + v[8:16] * hcols[2 * j + 1]
    acc_m = acc_m + _row_total(acc_v)
    x = x + xn + acc_m * sg

    if cfg["phase2"]:
        with scope("phase2"):
            mean, rstd = _ln_stats(x)
            marks = []
            front_mxu_q(_split(x), marks)
            front_mxu_qabs(marks)
            front_vpu(x, marks if cfg["gate"] else [])
            stage_attn(finish_front(mean, rstd))
            marks = []
            ctx_mxu(marks)
            acc_m = out_mxu(0, NMB, jnp.zeros((8, M), F32), False, marks)
            acc_v = back_vpu(NMB, NVB, jnp.zeros((8, M), F32), marks if cfg["gate"] else [])
            x = x + acc_m + _row_total(acc_v)
            mean, rstd = _ln_stats(x)
            xn = (x - mean) * rstd
            marks = []
            hd = gate_up_mxu(_split(x), mean, rstd, marks)
            y = down_mxu(hd, 0, NFM, jnp.zeros((8, M), F32), False, marks)
            acc_v, _ = ffn_vpu(x, rstd, marks if cfg["gate"] else [])
            sg = gate_scalar(xn, wr8)
            x = x + xn + (y + _row_total(acc_v)) * sg

    o_ref[0] = x[0:1].astype(BF)


def _run(cfg, A_x, A_c_kv, A_w_q, A_w_uk, A_w_uv, A_w_o, B_w_r, B_w_gate, B_w_up, B_w_down):
    any_spec = pl.BlockSpec(memory_space=pl.ANY)
    nmf, nmb = cfg["nmf"], cfg["nmb"]
    nvf, nvb = H - nmf, H - nmb
    fm = cfg["fm"]
    nsem = min(cfg["nsem"], len(_chunks(cfg)))
    scratch = [
        pltpu.VMEM((1, 1, M), BF),
        pltpu.VMEM((M,), BF),
        pltpu.VMEM((M, H, D), BF),
        pltpu.VMEM((DC, H, D), BF),
        pltpu.VMEM((DC, H, D), BF),
        pltpu.VMEM((SK, DC), BF),
        pltpu.VMEM((H, D, M), BF),
        pltpu.VMEM((F, M), BF),
        pltpu.VMEM((F, M), BF),
        pltpu.VMEM((F, M), BF),
        pltpu.VMEM(((H + 2) * SQ, 128), U32),
        pltpu.VMEM(((H + 2) * SV, 128), U32),
        pltpu.VMEM((4 * nmf * 64, 128), U32),
        pltpu.VMEM(((H + 2) * SV, 128), U32),
        pltpu.VMEM((32 * 4 * 64, 128), U32),
        pltpu.VMEM((4 * 2048, 128), U32),
        pltpu.VMEM((fm // 128 * 320, 128), U32),
        pltpu.VMEM((fm // 128 * 320, 128), U32),
        pltpu.VMEM((H * 8, 128), U32),
        pltpu.VMEM((4 * H, 128), U32),
        pltpu.VMEM((nvf * 128, M), F32),
        pltpu.VMEM((nvf * 128, DC), F32),
        pltpu.VMEM((nvb * 128, DC), F32),
        pltpu.VMEM((nvb * 128, M), F32),
        pltpu.VMEM((F - fm, M), F32),
        pltpu.VMEM((F - fm, M), F32),
        pltpu.VMEM((F - fm, M), F32),
        pltpu.VMEM((4 * H, 128), F32),
        pltpu.VMEM((8, fm), F32),
        pltpu.VMEM((8, fm), F32),
        pltpu.VMEM((4 * H, 128), F32),
        pltpu.VMEM((4 * H, 128), F32),
        pltpu.VMEM(((4 * nvf + 2) * SP, 128), F32),
        pltpu.VMEM((nmb * 5 * 64, 128), U32),
        pltpu.VMEM((fm // 128 * 5 * 64, 128), U32),
        pltpu.VMEM((8, 128), jnp.int32),
        pltpu.SemaphoreType.DMA((nsem,)),
    ]
    return pl.pallas_call(
        functools.partial(_kernel, cfg),
        out_shape=jax.ShapeDtypeStruct((1, 1, M), BF),
        in_specs=[any_spec] * 10,
        out_specs=pl.BlockSpec(memory_space=pltpu.VMEM),
        scratch_shapes=scratch,
        compiler_params=pltpu.CompilerParams(vmem_limit_bytes=110 * 1024 * 1024),
    )(A_x, A_c_kv, A_w_q, A_w_uk, A_w_uv, A_w_o, B_w_r, B_w_gate.T, B_w_up.T, B_w_down)


def build(**overrides):
    cfg = dict(DEFAULT_CFG, **overrides)

    @jax.jit
    def fn(A_x, A_c_kv, A_w_q, A_w_uk, A_w_uv, A_w_o, B_x, B_w_r, B_w_gate, B_w_up, B_w_down):
        return _run(cfg, A_x, A_c_kv, A_w_q, A_w_uk, A_w_uv, A_w_o, B_w_r, B_w_gate, B_w_up, B_w_down)
    return fn


@jax.jit
def pallas_interleave_layers__compressed_kv_cla__moe_arch_mod__decode_kernel(
    A_x: jax.Array,
    A_c_kv: jax.Array,
    A_w_q: jax.Array,
    A_w_uk: jax.Array,
    A_w_uv: jax.Array,
    A_w_o: jax.Array,
    B_x: jax.Array,
    B_w_r: jax.Array,
    B_w_gate: jax.Array,
    B_w_up: jax.Array,
    B_w_down: jax.Array,
):
    del B_x
    return _run(DEFAULT_CFG, A_x, A_c_kv, A_w_q, A_w_uk, A_w_uv, A_w_o, B_w_r, B_w_gate, B_w_up,
                B_w_down)
```

```python
import functools

import jax
import jax.numpy as jnp
from jax import lax
from jax.experimental import pallas as pl
from jax.experimental.pallas import tpu as pltpu

M = 640
H = 32
D = 128
DC = 512
SK = 4096
F = 1728
EPS = 1e-5

SQ = 322
SP = 9
SV = 258

BF = jnp.bfloat16
F32 = jnp.float32
U32 = jnp.uint32


def _bf(u32_val):
    return pltpu.bitcast(u32_val, BF)


def _u32(bf_val):
    return pltpu.bitcast(bf_val, U32)


def _dup(v8):
    return jnp.concatenate([v8, v8], axis=0).astype(BF)


def _dot(a, b):
    return jnp.dot(a, b, preferred_element_type=F32)


def _dot_nt(a, b):
    return lax.dot_general(a, b, (((1,), (1,)), ((), ())), preferred_element_type=F32)


def _split(v8):
    hi = pltpu.bitcast(pltpu.bitcast(v8, U32) & jnp.uint32(0xFFFF0000), F32)
    return jnp.concatenate([hi, v8 - hi], axis=0).astype(BF)


def _dot2(a16, b):
    r = _dot(a16, b)
    return r[0:8] + r[8:16]


def _ln_stats(x8):
    s1 = jnp.sum(x8, axis=1, keepdims=True)
    s2 = jnp.sum(x8 * x8, axis=1, keepdims=True)
    mean = s1 * (1.0 / M)
    var = jnp.maximum(s2 * (1.0 / M) - mean * mean, 0.0)
    return mean, lax.rsqrt(var + EPS)


def _swiglu(g, u):
    a = 0.5 * g
    b = a * u
    return b * jnp.tanh(a) + b


def _bcast_row(ref, row):
    return jnp.broadcast_to(ref[pl.ds(row, 1), :], (8, 128))


def _lane_blocks_sum(p):
    n = p.shape[1] // 128
    acc = p[:, 0:128]
    for i in range(1, n):
        acc = acc + p[:, i * 128:(i + 1) * 128]
    return acc


def _row_total(a8):
    return jnp.broadcast_to(jnp.sum(a8, axis=0, keepdims=True), a8.shape)


def _eye():
    r = lax.broadcasted_iota(jnp.int32, (128, 128), 0)
    c = lax.broadcasted_iota(jnp.int32, (128, 128), 1)
    return jnp.where(r == c, 1.0, 0.0).astype(BF)


def _transpose_tile(eye, tile):
    return _u32(_dot_nt(eye, tile).astype(BF))


def _chunks(cfg):
    fm = cfg["fm"]
    nm = cfg["nmb"]
    ch = []
    ch += [("wq", i * 128, 128) for i in range(5)]
    ch += [("wuk", i * 128, 128) for i in range(4)]
    ch += [("ckv", i * 1024, 1024) for i in range(4)]
    ch += [("wuv", i * 128, 128) for i in range(4)]
    ch += [("wo", h0, min(8, H - h0)) for h0 in range(nm, H, 8)]
    ch += [("wo", h0, min(8, nm - h0)) for h0 in range(0, nm, 8)]
    for name in ("wg", "wu"):
        ch += [(name, fm, F - fm)]
        ch += [(name, r0, min(512, fm - r0)) for r0 in range(0, fm, 512)]
    late = cfg["late"]
    ch += [("wd", fm, F - fm - late)]
    r0 = 0
    while r0 < fm - 128:
        n = min(512, fm - 128 - r0)
        ch.append(("wd", r0, n))
        r0 += n
    ch.append(("wd", fm - 128, 128))
    if late:
        ch.append(("wd", F - late, late))
    return ch


DEFAULT_CFG = dict(phase2=True, compute1=True, scopes=False, u_uk=16, u_ckv=4, u_rp=4,
                   nmf=18, nmb=16, fm=1024, gate=True, nsem=5,
                   lag_f=2, beta_f=1.0, lag_b=2, beta_b=1.0, lag_n=8, beta_n=1.0, gstep=8, late=128, small_after=0, hmajor=True)


class _NoScope:
    def __enter__(self):
        return self

    def __exit__(self, *a):
        return False


def _kernel(cfg, x_hbm, ckv_hbm, wq_hbm, wuk_hbm, wuv_hbm, wo_hbm, wr_hbm, wg_hbm, wu_hbm, wd_hbm,
            o_ref,
            x_s, wr_s, wq_n, wuk_n, wuv_n, ckv_n, wo_n, wg_n, wu_n, wd_n,
            WQ, UP, UT, UV, CKT, CK, GT, UPT, QD, CL,
            WQT, UTF, UVT, WOF, GF, UF, DF, CSA, CSG, CSU, CLF, QAR, PS, WOU, WDU, FLAG,
            sems):
    NMF = cfg["nmf"]
    NVF = H - NMF
    NMB = cfg["nmb"]
    NVB = H - NMB
    FM = cfg["fm"]
    NFM = FM // 128
    NG = (F - FM) // 8
    CHUNKS = _chunks(cfg)
    NCH = len(CHUNKS)
    NSEM = min(cfg["nsem"], NCH)

    hbm = dict(wq=wq_hbm, wuk=wuk_hbm, wuv=wuv_hbm, wo=wo_hbm, wg=wg_hbm, wu=wu_hbm, wd=wd_hbm,
               ckv=ckv_hbm.at[0])
    vm = dict(wq=wq_n, wuk=wuk_n, wuv=wuv_n, wo=wo_n, wg=wg_n, wu=wu_n, wd=wd_n, ckv=ckv_n)

    def chunk_copy(i):
        name, r0, n = CHUNKS[i]
        return pltpu.make_async_copy(hbm[name].at[pl.ds(r0, n)], vm[name].at[pl.ds(r0, n)],
                                     sems.at[(i + 2) % NSEM])

    def scope(name):
        return jax.named_scope(name) if cfg["scopes"] else _NoScope()

    def wait(i):
        with scope("wait%02d_%s" % (i, CHUNKS[i][0])):
            chunk_copy(i).wait()
        if i + NSEM < NCH:
            chunk_copy(i + NSEM).start()

    def idx(name):
        return [i for i, c in enumerate(CHUNKS) if c[0] == name]

    cx = pltpu.make_async_copy(x_hbm, x_s, sems.at[0])
    cr = pltpu.make_async_copy(wr_hbm, wr_s, sems.at[1])
    for i in range(NSEM - 2):
        if i == cfg["small_after"]:
            cx.start()
            cr.start()
        chunk_copy(i).start()

    FLAG[...] = jnp.ones((8, 128), jnp.int32)

    def repack(src_n, dst, stride, j0, nj):
        def body(j, c):
            a = _u32(src_n[2 * j])
            b = _u32(src_n[2 * j + 1])
            lo = (a & jnp.uint32(0xFFFF)) | (b << 16)
            hi = (a >> 16) | (b & jnp.uint32(0xFFFF0000))
            dst[pl.ds(j, 16, stride=2 * stride), :] = lo
            dst[pl.ds(stride + j, 16, stride=2 * stride), :] = hi
            return c
        lax.fori_loop(j0, j0 + nj, body, 0, unroll=cfg["u_rp"])

    def vpu_transposes(src, stride, kb, dst, NM):
        eye = _eye()

        def body(hv, c):
            tile = _bf(src[pl.ds((NM + hv) * stride + kb * 64, 64), :])
            row = pl.multiple_of(hv * 128, 128)
            dst[pl.ds(row, 128), pl.ds(kb * 128, 128)] = _dot_nt(eye, tile)
            return c
        lax.fori_loop(0, H - NM, body, 0, unroll=True)

    def prep_wuk_transpose(cb):
        eye = _eye()

        def body(h, c):
            tile = _bf(UP[pl.ds(h * SV + cb * 64, 64), :])
            UT[pl.ds((cb * NMF + h) * 64, 64), :] = _transpose_tile(eye, tile)
            return c
        lax.fori_loop(0, NMF, body, 0, unroll=True)

    def prep_ckv(kb0, nkb):
        eye = _eye()

        def body(kb, c):
            r0 = pl.multiple_of(kb * 128, 128)
            for cb in range(4):
                tile = ckv_n[pl.ds(r0, 128), pl.ds(cb * 128, 128)]
                CK[pl.ds(cb * 2048 + kb * 64, 64), :] = _u32(tile)
                CKT[pl.ds((kb * 4 + cb) * 64, 64), :] = _transpose_tile(eye, tile)
            return c
        lax.fori_loop(kb0, kb0 + nkb, body, 0, unroll=cfg["u_ckv"])

    def prep_ffn_mxu(src_n, dst, r0, n):
        eye = _eye()

        def body(nb, c):
            row = pl.multiple_of(nb * 128, 128)
            for kb in range(5):
                tile = src_n[pl.ds(row, 128), pl.ds(kb * 128, 128)]
                dst[pl.ds((nb * 5 + kb) * 64, 64), :] = _transpose_tile(eye, tile)
            return c
        lax.fori_loop(r0 // 128, (r0 + n) // 128, body, 0, unroll=True)

    def centered(v):
        return v - jnp.sum(v, axis=1, keepdims=True) * (1.0 / M)

    def unpack_rows(src, r0, n, dst, center):
        step = 16
        nit = n // step
        unroll = max(u for u in range(1, 13) if nit % u == 0)

        def body(i, c):
            r = pl.multiple_of(i * step, step)
            v = src[pl.ds(r0 + r, step), :].astype(F32)
            dst[pl.ds(r, step), :] = centered(v) if center else v
            return c
        lax.fori_loop(0, nit, body, 0, unroll=unroll)

    def center_wqt():
        for i in range(NVF * 8):
            rows = pl.ds(i * 16, 16)
            WQT[rows, :] = centered(WQT[rows, :])

    def unpack_wo(h0, nh):
        def body(h, c):
            row = pl.multiple_of((h - NMB) * 128, 128)
            WOF[pl.ds(row, 128), :] = wo_n[h].astype(F32)
            return c
        lax.fori_loop(h0, h0 + nh, body, 0)

    def gate(v, marks, frac):
        if not marks or frac <= 0.0:
            return v
        total = marks[-1][0]
        pick = None
        for done, val in marks:
            if done <= frac * total:
                pick = val
        if pick is None:
            return v
        always = FLAG[...] != 0
        return jnp.concatenate(
            [jnp.where(always, v[:, i * 128:(i + 1) * 128], pick) for i in range(v.shape[1] // 128)],
            axis=1)

    def front_mxu_q(xs, marks):
        qs = []
        for h in range(NMF):
            r = _dot2(xs, _bf(WQ[pl.ds(h * SQ, 320), :]))
            qs.append(_split(r))
            marks.append(((marks[-1][0] if marks else 0) + 5, r))
        return qs

    def front_mxu_qabs(qs, marks):
        order = ([(h, cb) for h in range(NMF) for cb in range(4)] if cfg["hmajor"] else
                 [(h, cb) for cb in range(4) for h in range(NMF)])
        for h, cb in order:
            r = _dot2(qs[h], _bf(UT[pl.ds((cb * NMF + h) * 64, 64), :]))
            QAR[pl.ds(cb * H + h, 1), :] = r[0:1]
            marks.append(((marks[-1][0] if marks else 0) + 1, r))

    def front_vpu(xn, marks):
        a = [None] * 4
        for hv in range(NVF):
            xh = gate(xn, marks, cfg["beta_f"] * (hv - cfg["lag_f"]) / NVF)
            for g in range(16):
                rows = pl.ds(hv * 128 + g * 8, 8)
                qc = jnp.sum(_lane_blocks_sum(WQT[rows, :] * xh), axis=1, keepdims=True)
                for cb in range(4):
                    t = UTF[rows, pl.ds(cb * 128, 128)] * qc
                    a[cb] = a[cb] + t if g > 0 else t
            for cb in range(4):
                PS[pl.ds((cb * NVF + hv) * SP, 8), :] = a[cb]
        for cb in range(4):
            for hv0 in range(0, NVF, 8):
                n = min(8, NVF - hv0)
                tot = None
                for s_ in range(8):
                    t = PS[pl.ds((cb * NVF + hv0) * SP + s_, n, stride=SP), :]
                    tot = t if tot is None else tot + t
                QAR[pl.ds(cb * H + NMF + hv0, n), :] = tot

    def finish_front(mean, rstd):
        row = lax.broadcasted_iota(jnp.int32, (H, 1), 0)
        mean32 = jnp.concatenate([mean] * 4, axis=0)
        rstd32 = jnp.concatenate([rstd] * 4, axis=0)
        off = jnp.where(row < NMF, mean32, 0.0)
        mul = rstd32 * (D ** -0.5)
        return jnp.concatenate(
            [((QAR[pl.ds(cb * H, H), :] - off * CSA[pl.ds(cb * H, H), :]) * mul).astype(BF)
             for cb in range(4)], axis=1)

    def scores(qa, nb0, nnb):
        return jnp.concatenate(
            [_dot(qa, _bf(CKT[pl.ds(nb * 256, 256), :])) for nb in range(nb0, nb0 + nnb)], axis=1)

    def pv(p, kb0, nkb):
        return jnp.concatenate(
            [_dot(p, _bf(CK[pl.ds(cb * 2048 + kb0 * 64, nkb * 64), :])) for cb in range(4)], axis=1)

    def stage_attn(qa):
        sa = scores(qa, 0, 16)
        sb = scores(qa, 16, 16)
        ma = jnp.max(sa, axis=1, keepdims=True)
        pa = jnp.exp(sa - ma)
        la = jnp.sum(pa, axis=1, keepdims=True)
        ca = pv(pa.astype(BF), 0, 16)
        m = jnp.maximum(ma, jnp.max(sb, axis=1, keepdims=True))
        pb = jnp.exp(sb - m)
        lb = jnp.sum(pb, axis=1, keepdims=True)
        cbv = pv(pb.astype(BF), 16, 16)
        alpha = jnp.exp(ma - m)
        inv = 1.0 / (alpha * la + lb)
        cl = (alpha * ca + cbv) * inv
        nm8 = -(-NMB // 8) * 8
        nv0 = NMB // 8 * 8
        bits = pltpu.bitcast(cl[0:nm8].astype(BF).astype(F32), U32)
        dupw = bits | (bits >> 16)
        for cb in range(4):
            CL[pl.ds(cb * H, nm8), :] = dupw[:, cb * 128:(cb + 1) * 128]
            CLF[pl.ds(cb * H + nv0, H - nv0), :] = cl[nv0:H, cb * 128:(cb + 1) * 128]

    def ctx_mxu(marks):
        for h in range(NMB):
            lhs = jnp.concatenate(
                [_bf(_bcast_row(CL, cb * H + h)) for cb in range(4)], axis=1)
            r = _dot(lhs, _bf(UV[pl.ds(h * SV, 256), :]))[0:8]
            QD[pl.ds(h * 8, 8), :] = _u32(_dup(r))
            marks.append(((marks[-1][0] if marks else 0) + 4, r))

    def out_mxu(h0, nh, acc, first, marks):
        for h in range(h0, h0 + nh):
            if first:
                w = wo_n[h]
                for mb in range(5):
                    WOU[pl.ds((h * 5 + mb) * 64, 64), :] = _u32(w[:, mb * 128:(mb + 1) * 128])
            else:
                w = jnp.concatenate(
                    [_bf(WOU[pl.ds((h * 5 + mb) * 64, 64), :]) for mb in range(5)], axis=1)
            r = _dot(_bf(QD[pl.ds(h * 8, 8), :]), w)[0:8]
            acc = acc + r
            marks.append(((marks[-1][0] if marks else 0) + 5, r[:, 0:128]))
        return acc

    def back_vpu(h0, nh, acc, marks):
        for h in range(h0, h0 + nh):
            hv = h - NMB
            cl = jnp.concatenate(
                [_bcast_row(CLF, cb * H + h) for cb in range(4)], axis=1)
            cl = gate(cl, marks, cfg["beta_b"] * (hv - cfg["lag_b"]) / NVB)
            for g in range(16):
                rows = pl.ds(hv * 128 + g * 8, 8)
                cc = jnp.sum(_lane_blocks_sum(UVT[rows, :] * cl), axis=1, keepdims=True)
                acc = acc + WOF[rows, :] * cc
        return acc

    def gate_up_mxu_raw(xs, marks):
        g, u = [], []
        for nb in range(NFM):
            g.append(_dot2(xs, _bf(GT[pl.ds(nb * 320, 320), :])))
            marks.append(((marks[-1][0] if marks else 0) + 5, g[-1]))
            u.append(_dot2(xs, _bf(UPT[pl.ds(nb * 320, 320), :])))
            marks.append((marks[-1][0] + 5, u[-1]))
        return g, u

    def gate_up_mxu(xs, mean, rstd, marks):
        g, u = gate_up_mxu_raw(xs, marks)
        hd = []
        for nb in range(NFM):
            cols = pl.ds(nb * 128, 128)
            gg = (g[nb] - mean * CSG[:, cols]) * rstd
            uu = (u[nb] - mean * CSU[:, cols]) * rstd
            hd.append(_dup(_swiglu(gg, uu)))
        return hd

    def down_mxu(hd, nb0, nb1, acc, first, marks):
        for nb in range(nb0, nb1):
            if first:
                w = wd_n[pl.ds(nb * 128, 128), :]
                for mb in range(5):
                    WDU[pl.ds((nb * 5 + mb) * 64, 64), :] = _u32(w[:, mb * 128:(mb + 1) * 128])
            else:
                w = jnp.concatenate(
                    [_bf(WDU[pl.ds((nb * 5 + mb) * 64, 64), :]) for mb in range(5)], axis=1)
            r = _dot(hd[nb], w)[0:8]
            acc = acc + r
            marks.append(((marks[-1][0] if marks else 0) + 5, r[:, 0:128]))
        return acc

    def ffn_vpu(x8, rstd, marks, nlate=0):
        acc = None
        xg = x8
        hcols = []
        half_rstd = 0.5 * rstd
        for g in range(NG):
            if g % cfg["gstep"] == 0:
                xg = gate(x8, marks, cfg["beta_n"] * (g - cfg["lag_n"]) / NG)
            rows = pl.ds(g * 8, 8)
            gc = jnp.sum(_lane_blocks_sum(GF[rows, :] * xg), axis=1, keepdims=True)
            uc = jnp.sum(_lane_blocks_sum(UF[rows, :] * xg), axis=1, keepdims=True)
            a = gc * half_rstd
            b = a * uc
            hc = b * jnp.tanh(a) + b
            if g >= NG - nlate:
                hcols.append(hc)
            else:
                t = DF[rows, :] * hc
                acc = t if acc is None else acc + t
        return acc, hcols

    def gate_scalar(xn, wr8):
        return jax.nn.sigmoid(jnp.sum(xn * wr8, axis=1, keepdims=True))

    ones_split = jnp.concatenate([jnp.ones((8, M), BF), jnp.zeros((8, M), BF)], axis=0)

    cx.wait()
    chunk_copy(NSEM - 2).start()
    cr.wait()
    chunk_copy(NSEM - 1).start()
    x = jnp.broadcast_to(x_s[0].astype(F32), (8, M))
    wr8 = jnp.broadcast_to(wr_s[...].reshape(1, M).astype(F32), (8, M))

    if not cfg["compute1"]:
        for i in range(NCH):
            wait(i)
        o_ref[0] = x[0:1].astype(BF)
        return

    for k, i in enumerate(idx("wq")):
        wait(i)
        with scope("p_wq"):
            repack(wq_n, WQ, SQ, k * 64, 64)
            vpu_transposes(WQ, SQ, k, WQT, NMF)
    with scope("s1_csq"):
        center_wqt()
    for k, i in enumerate(idx("wuk")):
        wait(i)
        with scope("p_wuk"):
            repack(wuk_n, UP, SV, k * 64, 64)
            prep_wuk_transpose(k)
            vpu_transposes(UP, SV, k, UTF, NMF)
    with scope("s1_csa"):
        front_mxu_qabs(front_mxu_q(ones_split, []), [])
        for cb in range(4):
            CSA[pl.ds(cb * H, NMF), :] = QAR[pl.ds(cb * H, NMF), :]
            CSA[pl.ds(cb * H + NMF, NVF), :] = jnp.zeros((NVF, 128), F32)
    with scope("s1_front"):
        mean, rstd = _ln_stats(x)
        front_mxu_qabs(front_mxu_q(_split(x), []), [])
        front_vpu(x, [])
        qa = finish_front(mean, rstd)
    for k, i in enumerate(idx("ckv")):
        wait(i)
        with scope("p_ckv"):
            prep_ckv(k * 8, 8)
    with scope("s1_attn"):
        stage_attn(qa)
    for k, i in enumerate(idx("wuv")):
        wait(i)
        with scope("p_wuv"):
            repack(wuv_n, UV, SV, k * 64, 64)
            vpu_transposes(UV, SV, k, UVT, NMB)
    with scope("s1_ctx"):
        ctx_mxu([])
    acc_v = jnp.zeros((8, M), F32)
    acc_m = jnp.zeros((8, M), F32)
    for i in idx("wo"):
        wait(i)
        h0, nh = CHUNKS[i][1], CHUNKS[i][2]
        with scope("s1_out"):
            if h0 >= NMB:
                unpack_wo(h0, nh)
                acc_v = back_vpu(h0, nh, acc_v, [])
            else:
                acc_m = out_mxu(h0, nh, acc_m, True, [])
    x = x + acc_m + _row_total(acc_v)
    for name, nat, tr, fl in (("wg", wg_n, GT, GF), ("wu", wu_n, UPT, UF)):
        for i in idx(name):
            wait(i)
            r0, n = CHUNKS[i][1], CHUNKS[i][2]
            with scope("p_" + name):
                if r0 >= FM:
                    unpack_rows(nat, r0, n, fl, True)
                else:
                    prep_ffn_mxu(nat, tr, r0, n)
    with scope("s2_cs"):
        g, u = gate_up_mxu_raw(ones_split, [])
        CSG[...] = jnp.concatenate(g, axis=1)
        CSU[...] = jnp.concatenate(u, axis=1)
    wd_idx = idx("wd")
    LATE = cfg["late"]
    wait(wd_idx[0])
    with scope("p_wd"):
        unpack_rows(wd_n, FM, F - FM - LATE, DF, False)
    with scope("s2_gu"):
        mean, rstd = _ln_stats(x)
        xn = (x - mean) * rstd
        hd = gate_up_mxu(_split(x), mean, rstd, [])
        acc_v, hcols = ffn_vpu(x, rstd, [], LATE // 8)
        sg = gate_scalar(xn, wr8)
    acc_m = jnp.zeros((8, M), F32)
    for i in wd_idx[1:]:
        wait(i)
        r0, n = CHUNKS[i][1], CHUNKS[i][2]
        with scope("s2_down"):
            if r0 < FM:
                acc_m = down_mxu(hd, r0 // 128, (r0 + n) // 128, acc_m, True, [])
            else:
                for j in range(n // 16):
                    v = wd_n[pl.ds(r0 + j * 16, 16), :].astype(F32)
                    DF[pl.ds(r0 - FM + j * 16, 16), :] = v
                    acc_v = acc_v + v[0:8] * hcols[2 * j] + v[8:16] * hcols[2 * j + 1]
    acc_m = acc_m + _row_total(acc_v) * rstd
    x = x + xn + acc_m * sg

    if cfg["phase2"]:
        with scope("phase2"):
            mean, rstd = _ln_stats(x)
            marks = []
            front_mxu_qabs(front_mxu_q(_split(x), marks), marks)
            front_vpu(x, marks if cfg["gate"] else [])
            stage_attn(finish_front(mean, rstd))
            marks = []
            ctx_mxu(marks)
            acc_m = out_mxu(0, NMB, jnp.zeros((8, M), F32), False, marks)
            acc_v = back_vpu(NMB, NVB, jnp.zeros((8, M), F32), marks if cfg["gate"] else [])
            x = x + acc_m + _row_total(acc_v)
            mean, rstd = _ln_stats(x)
            xn = (x - mean) * rstd
            marks = []
            hd = gate_up_mxu(_split(x), mean, rstd, marks)
            y = down_mxu(hd, 0, NFM, jnp.zeros((8, M), F32), False, marks)
            acc_v, _ = ffn_vpu(x, rstd, marks if cfg["gate"] else [])
            sg = gate_scalar(xn, wr8)
            x = x + xn + (y + _row_total(acc_v) * rstd) * sg

    o_ref[0] = x[0:1].astype(BF)


def _run(cfg, A_x, A_c_kv, A_w_q, A_w_uk, A_w_uv, A_w_o, B_w_r, B_w_gate, B_w_up, B_w_down):
    any_spec = pl.BlockSpec(memory_space=pl.ANY)
    nmf, nmb = cfg["nmf"], cfg["nmb"]
    nvf, nvb = H - nmf, H - nmb
    fm = cfg["fm"]
    nsem = min(cfg["nsem"], len(_chunks(cfg)))
    scratch = [
        pltpu.VMEM((1, 1, M), BF),
        pltpu.VMEM((M,), BF),
        pltpu.VMEM((M, H, D), BF),
        pltpu.VMEM((DC, H, D), BF),
        pltpu.VMEM((DC, H, D), BF),
        pltpu.VMEM((SK, DC), BF),
        pltpu.VMEM((H, D, M), BF),
        pltpu.VMEM((F, M), BF),
        pltpu.VMEM((F, M), BF),
        pltpu.VMEM((F, M), BF),
        pltpu.VMEM(((H + 2) * SQ, 128), U32),
        pltpu.VMEM(((H + 2) * SV, 128), U32),
        pltpu.VMEM((4 * nmf * 64, 128), U32),
        pltpu.VMEM(((H + 2) * SV, 128), U32),
        pltpu.VMEM((32 * 4 * 64, 128), U32),
        pltpu.VMEM((4 * 2048, 128), U32),
        pltpu.VMEM((fm // 128 * 320, 128), U32),
        pltpu.VMEM((fm // 128 * 320, 128), U32),
        pltpu.VMEM((H * 8, 128), U32),
        pltpu.VMEM((4 * H, 128), U32),
        pltpu.VMEM((nvf * 128, M), F32),
        pltpu.VMEM((nvf * 128, DC), F32),
        pltpu.VMEM((nvb * 128, DC), F32),
        pltpu.VMEM((nvb * 128, M), F32),
        pltpu.VMEM((F - fm, M), F32),
        pltpu.VMEM((F - fm, M), F32),
        pltpu.VMEM((F - fm, M), F32),
        pltpu.VMEM((4 * H, 128), F32),
        pltpu.VMEM((8, fm), F32),
        pltpu.VMEM((8, fm), F32),
        pltpu.VMEM((4 * H, 128), F32),
        pltpu.VMEM((4 * H, 128), F32),
        pltpu.VMEM(((4 * nvf + 2) * SP, 128), F32),
        pltpu.VMEM((nmb * 5 * 64, 128), U32),
        pltpu.VMEM((fm // 128 * 5 * 64, 128), U32),
        pltpu.VMEM((8, 128), jnp.int32),
        pltpu.SemaphoreType.DMA((nsem,)),
    ]
    return pl.pallas_call(
        functools.partial(_kernel, cfg),
        out_shape=jax.ShapeDtypeStruct((1, 1, M), BF),
        in_specs=[any_spec] * 10,
        out_specs=pl.BlockSpec(memory_space=pltpu.VMEM),
        scratch_shapes=scratch,
        compiler_params=pltpu.CompilerParams(vmem_limit_bytes=110 * 1024 * 1024),
    )(A_x, A_c_kv, A_w_q, A_w_uk, A_w_uv, A_w_o, B_w_r, B_w_gate.T, B_w_up.T, B_w_down)


def build(**overrides):
    cfg = dict(DEFAULT_CFG, **overrides)

    @jax.jit
    def fn(A_x, A_c_kv, A_w_q, A_w_uk, A_w_uv, A_w_o, B_x, B_w_r, B_w_gate, B_w_up, B_w_down):
        return _run(cfg, A_x, A_c_kv, A_w_q, A_w_uk, A_w_uv, A_w_o, B_w_r, B_w_gate, B_w_up, B_w_down)
    return fn


@jax.jit
def pallas_interleave_layers__compressed_kv_cla__moe_arch_mod__decode_kernel(
    A_x: jax.Array,
    A_c_kv: jax.Array,
    A_w_q: jax.Array,
    A_w_uk: jax.Array,
    A_w_uv: jax.Array,
    A_w_o: jax.Array,
    B_x: jax.Array,
    B_w_r: jax.Array,
    B_w_gate: jax.Array,
    B_w_up: jax.Array,
    B_w_down: jax.Array,
):
    del B_x
    return _run(DEFAULT_CFG, A_x, A_c_kv, A_w_q, A_w_uk, A_w_uv, A_w_o, B_w_r, B_w_gate, B_w_up,
                B_w_down)
```

```python
import functools

import jax
import jax.numpy as jnp
from jax import lax
from jax.experimental import pallas as pl
from jax.experimental.pallas import tpu as pltpu

M = 640
H = 32
D = 128
DC = 512
SK = 4096
F = 1728
EPS = 1e-5

SQ = 322
SP = 9
SV = 258

BF = jnp.bfloat16
F32 = jnp.float32
U32 = jnp.uint32


def _bf(u32_val):
    return pltpu.bitcast(u32_val, BF)


def _u32(bf_val):
    return pltpu.bitcast(bf_val, U32)


def _dup(v8):
    return jnp.concatenate([v8, v8], axis=0).astype(BF)


def _dot(a, b):
    return jnp.dot(a, b, preferred_element_type=F32)


def _dot_nt(a, b):
    return lax.dot_general(a, b, (((1,), (1,)), ((), ())), preferred_element_type=F32)


def _split(v8):
    hi = pltpu.bitcast(pltpu.bitcast(v8, U32) & jnp.uint32(0xFFFF0000), F32)
    return jnp.concatenate([hi, v8 - hi], axis=0).astype(BF)


def _dot2(a16, b):
    r = _dot(a16, b)
    return r[0:8] + r[8:16]


def _ln_stats(x8):
    s1 = jnp.sum(x8, axis=1, keepdims=True)
    s2 = jnp.sum(x8 * x8, axis=1, keepdims=True)
    mean = s1 * (1.0 / M)
    var = jnp.maximum(s2 * (1.0 / M) - mean * mean, 0.0)
    return mean, lax.rsqrt(var + EPS)


def _swiglu(g, u):
    a = 0.5 * g
    b = a * u
    return b * jnp.tanh(a) + b


def _bcast_row(ref, row):
    return jnp.broadcast_to(ref[pl.ds(row, 1), :], (8, 128))


def _lane_blocks_sum(p):
    n = p.shape[1] // 128
    acc = p[:, 0:128]
    for i in range(1, n):
        acc = acc + p[:, i * 128:(i + 1) * 128]
    return acc


def _row_total(a8):
    return jnp.broadcast_to(jnp.sum(a8, axis=0, keepdims=True), a8.shape)


def _eye():
    r = lax.broadcasted_iota(jnp.int32, (128, 128), 0)
    c = lax.broadcasted_iota(jnp.int32, (128, 128), 1)
    return jnp.where(r == c, 1.0, 0.0).astype(BF)


def _transpose_tile(eye, tile):
    return _u32(_dot_nt(eye, tile).astype(BF))


def _chunks(cfg):
    fm = cfg["fm"]
    nm = cfg["nmb"]
    ch = []
    ch += [("wq", i * 128, 128) for i in range(5)]
    ch += [("wuk", i * 128, 128) for i in range(4)]
    ch += [("ckv", i * 1024, 1024) for i in range(4)]
    ch += [("wuv", i * 128, 128) for i in range(4)]
    ch += [("wo", h0, min(8, H - h0)) for h0 in range(nm, H, 8)]
    ch += [("wo", h0, min(8, nm - h0)) for h0 in range(0, nm, 8)]
    for name in ("wg", "wu"):
        ch += [(name, fm, F - fm)]
        ch += [(name, r0, min(512, fm - r0)) for r0 in range(0, fm, 512)]
    late = cfg["late"]
    ch += [("wd", fm, F - fm - late)]
    r0 = 0
    while r0 < fm - 128:
        n = min(512, fm - 128 - r0)
        ch.append(("wd", r0, n))
        r0 += n
    ch.append(("wd", fm - 128, 128))
    if late:
        ch.append(("wd", F - late, late))
    return ch


DEFAULT_CFG = dict(phase2=True, compute1=True, scopes=False, u_uk=16, u_ckv=4, u_rp=4,
                   nmf=18, nmb=16, fm=1024, gate=True, nsem=5,
                   lag_f=2, beta_f=1.0, lag_b=1, beta_b=1.0, lag_n=8, beta_n=1.0, gstep=8, late=128, small_after=0, hmajor=True)


class _NoScope:
    def __enter__(self):
        return self

    def __exit__(self, *a):
        return False


def _kernel(cfg, x_hbm, ckv_hbm, wq_hbm, wuk_hbm, wuv_hbm, wo_hbm, wr_hbm, wg_hbm, wu_hbm, wd_hbm,
            o_ref,
            x_s, wr_s, wq_n, wuk_n, wuv_n, ckv_n, wo_n, wg_n, wu_n, wd_n,
            WQ, UP, UT, UV, CKT, CK, GT, UPT, QD, CL,
            WQT, UTF, UVT, WOF, GF, UF, DF, CSA, CSG, CSU, CLF, QAR, PS, WOU, WDU, FLAG,
            sems):
    NMF = cfg["nmf"]
    NVF = H - NMF
    NMB = cfg["nmb"]
    NVB = H - NMB
    FM = cfg["fm"]
    NFM = FM // 128
    NG = (F - FM) // 8
    CHUNKS = _chunks(cfg)
    NCH = len(CHUNKS)
    NSEM = min(cfg["nsem"], NCH)

    hbm = dict(wq=wq_hbm, wuk=wuk_hbm, wuv=wuv_hbm, wo=wo_hbm, wg=wg_hbm, wu=wu_hbm, wd=wd_hbm,
               ckv=ckv_hbm.at[0])
    vm = dict(wq=wq_n, wuk=wuk_n, wuv=wuv_n, wo=wo_n, wg=wg_n, wu=wu_n, wd=wd_n, ckv=ckv_n)

    def chunk_copy(i):
        name, r0, n = CHUNKS[i]
        return pltpu.make_async_copy(hbm[name].at[pl.ds(r0, n)], vm[name].at[pl.ds(r0, n)],
                                     sems.at[(i + 2) % NSEM])

    def scope(name):
        return jax.named_scope(name) if cfg["scopes"] else _NoScope()

    def wait(i):
        with scope("wait%02d_%s" % (i, CHUNKS[i][0])):
            chunk_copy(i).wait()
        if i + NSEM < NCH:
            chunk_copy(i + NSEM).start()

    def idx(name):
        return [i for i, c in enumerate(CHUNKS) if c[0] == name]

    cx = pltpu.make_async_copy(x_hbm, x_s, sems.at[0])
    cr = pltpu.make_async_copy(wr_hbm, wr_s, sems.at[1])
    for i in range(NSEM - 2):
        if i == cfg["small_after"]:
            cx.start()
            cr.start()
        chunk_copy(i).start()

    FLAG[...] = jnp.ones((8, 128), jnp.int32)

    def repack(src_n, dst, stride, j0, nj):
        def body(j, c):
            a = _u32(src_n[2 * j])
            b = _u32(src_n[2 * j + 1])
            lo = (a & jnp.uint32(0xFFFF)) | (b << 16)
            hi = (a >> 16) | (b & jnp.uint32(0xFFFF0000))
            dst[pl.ds(j, 16, stride=2 * stride), :] = lo
            dst[pl.ds(stride + j, 16, stride=2 * stride), :] = hi
            return c
        lax.fori_loop(j0, j0 + nj, body, 0, unroll=cfg["u_rp"])

    def vpu_transposes(src, stride, kb, dst, NM):
        eye = _eye()

        def body(hv, c):
            tile = _bf(src[pl.ds((NM + hv) * stride + kb * 64, 64), :])
            row = pl.multiple_of(hv * 128, 128)
            dst[pl.ds(row, 128), pl.ds(kb * 128, 128)] = _dot_nt(eye, tile)
            return c
        lax.fori_loop(0, H - NM, body, 0, unroll=True)

    def prep_wuk_transpose(cb):
        eye = _eye()

        def body(h, c):
            tile = _bf(UP[pl.ds(h * SV + cb * 64, 64), :])
            UT[pl.ds((cb * NMF + h) * 64, 64), :] = _transpose_tile(eye, tile)
            return c
        lax.fori_loop(0, NMF, body, 0, unroll=True)

    def prep_ckv(kb0, nkb):
        eye = _eye()

        def body(kb, c):
            r0 = pl.multiple_of(kb * 128, 128)
            for cb in range(4):
                tile = ckv_n[pl.ds(r0, 128), pl.ds(cb * 128, 128)]
                CK[pl.ds(cb * 2048 + kb * 64, 64), :] = _u32(tile)
                CKT[pl.ds((kb * 4 + cb) * 64, 64), :] = _transpose_tile(eye, tile)
            return c
        lax.fori_loop(kb0, kb0 + nkb, body, 0, unroll=cfg["u_ckv"])

    def prep_ffn_mxu(src_n, dst, r0, n):
        eye = _eye()

        def body(nb, c):
            row = pl.multiple_of(nb * 128, 128)
            for kb in range(5):
                tile = src_n[pl.ds(row, 128), pl.ds(kb * 128, 128)]
                dst[pl.ds((nb * 5 + kb) * 64, 64), :] = _transpose_tile(eye, tile)
            return c
        lax.fori_loop(r0 // 128, (r0 + n) // 128, body, 0, unroll=True)

    def centered(v):
        return v - jnp.sum(v, axis=1, keepdims=True) * (1.0 / M)

    def unpack_rows(src, r0, n, dst, center):
        step = 16
        nit = n // step
        unroll = max(u for u in range(1, 13) if nit % u == 0)

        def body(i, c):
            r = pl.multiple_of(i * step, step)
            v = src[pl.ds(r0 + r, step), :].astype(F32)
            dst[pl.ds(r, step), :] = centered(v) if center else v
            return c
        lax.fori_loop(0, nit, body, 0, unroll=unroll)

    def center_wqt():
        for i in range(NVF * 8):
            rows = pl.ds(i * 16, 16)
            WQT[rows, :] = centered(WQT[rows, :])

    def unpack_wo(h0, nh):
        def body(h, c):
            row = pl.multiple_of((h - NMB) * 128, 128)
            WOF[pl.ds(row, 128), :] = wo_n[h].astype(F32)
            return c
        lax.fori_loop(h0, h0 + nh, body, 0)

    def gate(v, marks, frac):
        if not marks or frac <= 0.0:
            return v
        total = marks[-1][0]
        pick = None
        for done, val in marks:
            if done <= frac * total:
                pick = val
        if pick is None:
            return v
        always = FLAG[...] != 0
        return jnp.concatenate(
            [jnp.where(always, v[:, i * 128:(i + 1) * 128], pick) for i in range(v.shape[1] // 128)],
            axis=1)

    def front_mxu_q(xs, marks):
        qs = []
        for h in range(NMF):
            r = _dot2(xs, _bf(WQ[pl.ds(h * SQ, 320), :]))
            qs.append(_split(r))
            marks.append(((marks[-1][0] if marks else 0) + 5, r))
        return qs

    def front_mxu_qabs(qs, marks):
        order = ([(h, cb) for h in range(NMF) for cb in range(4)] if cfg["hmajor"] else
                 [(h, cb) for cb in range(4) for h in range(NMF)])
        for h, cb in order:
            r = _dot2(qs[h], _bf(UT[pl.ds((cb * NMF + h) * 64, 64), :]))
            QAR[pl.ds(cb * H + h, 1), :] = r[0:1]
            marks.append(((marks[-1][0] if marks else 0) + 1, r))

    def front_vpu(xn, marks):
        a = [None] * 4
        for hv in range(NVF):
            xh = gate(xn, marks, cfg["beta_f"] * (hv - cfg["lag_f"]) / NVF)
            for g in range(16):
                rows = pl.ds(hv * 128 + g * 8, 8)
                qc = jnp.sum(_lane_blocks_sum(WQT[rows, :] * xh), axis=1, keepdims=True)
                for cb in range(4):
                    t = UTF[rows, pl.ds(cb * 128, 128)] * qc
                    a[cb] = a[cb] + t if g > 0 else t
            for cb in range(4):
                PS[pl.ds((cb * NVF + hv) * SP, 8), :] = a[cb]
        for cb in range(4):
            for hv0 in range(0, NVF, 8):
                n = min(8, NVF - hv0)
                tot = None
                for s_ in range(8):
                    t = PS[pl.ds((cb * NVF + hv0) * SP + s_, n, stride=SP), :]
                    tot = t if tot is None else tot + t
                QAR[pl.ds(cb * H + NMF + hv0, n), :] = tot

    def finish_front(mean, rstd):
        row = lax.broadcasted_iota(jnp.int32, (H, 1), 0)
        mean32 = jnp.concatenate([mean] * 4, axis=0)
        rstd32 = jnp.concatenate([rstd] * 4, axis=0)
        off = jnp.where(row < NMF, mean32, 0.0)
        mul = rstd32 * (D ** -0.5)
        return jnp.concatenate(
            [((QAR[pl.ds(cb * H, H), :] - off * CSA[pl.ds(cb * H, H), :]) * mul).astype(BF)
             for cb in range(4)], axis=1)

    def scores(qa, nb0, nnb):
        return jnp.concatenate(
            [_dot(qa, _bf(CKT[pl.ds(nb * 256, 256), :])) for nb in range(nb0, nb0 + nnb)], axis=1)

    def pv(p, kb0, nkb):
        return jnp.concatenate(
            [_dot(p, _bf(CK[pl.ds(cb * 2048 + kb0 * 64, nkb * 64), :])) for cb in range(4)], axis=1)

    def stage_attn(qa):
        sa = scores(qa, 0, 16)
        sb = scores(qa, 16, 16)
        ma = jnp.max(sa, axis=1, keepdims=True)
        pa = jnp.exp(sa - ma)
        la = jnp.sum(pa, axis=1, keepdims=True)
        ca = pv(pa.astype(BF), 0, 16)
        m = jnp.maximum(ma, jnp.max(sb, axis=1, keepdims=True))
        pb = jnp.exp(sb - m)
        lb = jnp.sum(pb, axis=1, keepdims=True)
        cbv = pv(pb.astype(BF), 16, 16)
        alpha = jnp.exp(ma - m)
        inv = 1.0 / (alpha * la + lb)
        cl = (alpha * ca + cbv) * inv
        nm8 = -(-NMB // 8) * 8
        nv0 = NMB // 8 * 8
        bits = pltpu.bitcast(cl[0:nm8].astype(BF).astype(F32), U32)
        dupw = bits | (bits >> 16)
        for cb in range(4):
            CL[pl.ds(cb * H, nm8), :] = dupw[:, cb * 128:(cb + 1) * 128]
            CLF[pl.ds(cb * H + nv0, H - nv0), :] = cl[nv0:H, cb * 128:(cb + 1) * 128]

    def ctx_mxu(marks):
        r = [None] * NMB
        for cb in range(4):
            for h in range(NMB):
                lhs = _bf(_bcast_row(CL, cb * H + h))
                t = _dot(lhs, _bf(UV[pl.ds(h * SV + cb * 64, 64), :]))[0:8]
                r[h] = t if cb == 0 else r[h] + t
                marks.append(((marks[-1][0] if marks else 0) + 1, t))
        for h in range(NMB):
            QD[pl.ds(h * 8, 8), :] = _u32(_dup(r[h]))

    def out_mxu(h0, nh, acc, first, marks):
        for h in range(h0, h0 + nh):
            if first:
                w = wo_n[h]
                for mb in range(5):
                    WOU[pl.ds((h * 5 + mb) * 64, 64), :] = _u32(w[:, mb * 128:(mb + 1) * 128])
            else:
                w = jnp.concatenate(
                    [_bf(WOU[pl.ds((h * 5 + mb) * 64, 64), :]) for mb in range(5)], axis=1)
            r = _dot(_bf(QD[pl.ds(h * 8, 8), :]), w)[0:8]
            acc = acc + r
            marks.append(((marks[-1][0] if marks else 0) + 5, r[:, 0:128]))
        return acc

    def back_vpu(h0, nh, acc, marks):
        for h in range(h0, h0 + nh):
            hv = h - NMB
            cl = jnp.concatenate(
                [_bcast_row(CLF, cb * H + h) for cb in range(4)], axis=1)
            cl = gate(cl, marks, cfg["beta_b"] * (hv - cfg["lag_b"]) / NVB)
            for g in range(16):
                rows = pl.ds(hv * 128 + g * 8, 8)
                cc = jnp.sum(_lane_blocks_sum(UVT[rows, :] * cl), axis=1, keepdims=True)
                acc = acc + WOF[rows, :] * cc
        return acc

    def gate_up_mxu_raw(xs, marks):
        g, u = [], []
        for nb in range(NFM):
            g.append(_dot2(xs, _bf(GT[pl.ds(nb * 320, 320), :])))
            marks.append(((marks[-1][0] if marks else 0) + 5, g[-1]))
            u.append(_dot2(xs, _bf(UPT[pl.ds(nb * 320, 320), :])))
            marks.append((marks[-1][0] + 5, u[-1]))
        return g, u

    def gate_up_mxu(xs, mean, rstd, marks):
        g, u = gate_up_mxu_raw(xs, marks)
        hd = []
        for nb in range(NFM):
            cols = pl.ds(nb * 128, 128)
            gg = (g[nb] - mean * CSG[:, cols]) * rstd
            uu = (u[nb] - mean * CSU[:, cols]) * rstd
            hd.append(_dup(_swiglu(gg, uu)))
        return hd

    def down_mxu(hd, nb0, nb1, acc, first, marks):
        for nb in range(nb0, nb1):
            if first:
                w = wd_n[pl.ds(nb * 128, 128), :]
                for mb in range(5):
                    WDU[pl.ds((nb * 5 + mb) * 64, 64), :] = _u32(w[:, mb * 128:(mb + 1) * 128])
            else:
                w = jnp.concatenate(
                    [_bf(WDU[pl.ds((nb * 5 + mb) * 64, 64), :]) for mb in range(5)], axis=1)
            r = _dot(hd[nb], w)[0:8]
            acc = acc + r
            marks.append(((marks[-1][0] if marks else 0) + 5, r[:, 0:128]))
        return acc

    def ffn_vpu(x8, rstd, marks, nlate=0):
        acc = None
        xg = x8
        hcols = []
        half_rstd = 0.5 * rstd
        for g in range(NG):
            if g % cfg["gstep"] == 0:
                xg = gate(x8, marks, cfg["beta_n"] * (g - cfg["lag_n"]) / NG)
            rows = pl.ds(g * 8, 8)
            gc = jnp.sum(_lane_blocks_sum(GF[rows, :] * xg), axis=1, keepdims=True)
            uc = jnp.sum(_lane_blocks_sum(UF[rows, :] * xg), axis=1, keepdims=True)
            a = gc * half_rstd
            b = a * uc
            hc = b * jnp.tanh(a) + b
            if g >= NG - nlate:
                hcols.append(hc)
            else:
                t = DF[rows, :] * hc
                acc = t if acc is None else acc + t
        return acc, hcols

    def gate_scalar(xn, wr8):
        return jax.nn.sigmoid(jnp.sum(xn * wr8, axis=1, keepdims=True))

    ones_split = jnp.concatenate([jnp.ones((8, M), BF), jnp.zeros((8, M), BF)], axis=0)

    cx.wait()
    chunk_copy(NSEM - 2).start()
    cr.wait()
    chunk_copy(NSEM - 1).start()
    x = jnp.broadcast_to(x_s[0].astype(F32), (8, M))
    wr8 = jnp.broadcast_to(wr_s[...].reshape(1, M).astype(F32), (8, M))

    if not cfg["compute1"]:
        for i in range(NCH):
            wait(i)
        o_ref[0] = x[0:1].astype(BF)
        return

    for k, i in enumerate(idx("wq")):
        wait(i)
        with scope("p_wq"):
            repack(wq_n, WQ, SQ, k * 64, 64)
            vpu_transposes(WQ, SQ, k, WQT, NMF)
    with scope("s1_csq"):
        center_wqt()
    for k, i in enumerate(idx("wuk")):
        wait(i)
        with scope("p_wuk"):
            repack(wuk_n, UP, SV, k * 64, 64)
            prep_wuk_transpose(k)
            vpu_transposes(UP, SV, k, UTF, NMF)
    with scope("s1_csa"):
        front_mxu_qabs(front_mxu_q(ones_split, []), [])
        for cb in range(4):
            CSA[pl.ds(cb * H, NMF), :] = QAR[pl.ds(cb * H, NMF), :]
            CSA[pl.ds(cb * H + NMF, NVF), :] = jnp.zeros((NVF, 128), F32)
    with scope("s1_front"):
        mean, rstd = _ln_stats(x)
        front_mxu_qabs(front_mxu_q(_split(x), []), [])
        front_vpu(x, [])
        qa = finish_front(mean, rstd)
    for k, i in enumerate(idx("ckv")):
        wait(i)
        with scope("p_ckv"):
            prep_ckv(k * 8, 8)
    with scope("s1_attn"):
        stage_attn(qa)
    for k, i in enumerate(idx("wuv")):
        wait(i)
        with scope("p_wuv"):
            repack(wuv_n, UV, SV, k * 64, 64)
            vpu_transposes(UV, SV, k, UVT, NMB)
    with scope("s1_ctx"):
        ctx_mxu([])
    acc_v = jnp.zeros((8, M), F32)
    acc_m = jnp.zeros((8, M), F32)
    for i in idx("wo"):
        wait(i)
        h0, nh = CHUNKS[i][1], CHUNKS[i][2]
        with scope("s1_out"):
            if h0 >= NMB:
                unpack_wo(h0, nh)
                acc_v = back_vpu(h0, nh, acc_v, [])
            else:
                acc_m = out_mxu(h0, nh, acc_m, True, [])
    x = x + acc_m + _row_total(acc_v)
    for name, nat, tr, fl in (("wg", wg_n, GT, GF), ("wu", wu_n, UPT, UF)):
        for i in idx(name):
            wait(i)
            r0, n = CHUNKS[i][1], CHUNKS[i][2]
            with scope("p_" + name):
                if r0 >= FM:
                    unpack_rows(nat, r0, n, fl, True)
                else:
                    prep_ffn_mxu(nat, tr, r0, n)
    with scope("s2_cs"):
        g, u = gate_up_mxu_raw(ones_split, [])
        CSG[...] = jnp.concatenate(g, axis=1)
        CSU[...] = jnp.concatenate(u, axis=1)
    wd_idx = idx("wd")
    LATE = cfg["late"]
    wait(wd_idx[0])
    with scope("p_wd"):
        unpack_rows(wd_n, FM, F - FM - LATE, DF, False)
    with scope("s2_gu"):
        mean, rstd = _ln_stats(x)
        xn = (x - mean) * rstd
        hd = gate_up_mxu(_split(x), mean, rstd, [])
        acc_v, hcols = ffn_vpu(x, rstd, [], LATE // 8)
        sg = gate_scalar(xn, wr8)
    acc_m = jnp.zeros((8, M), F32)
    for i in wd_idx[1:]:
        wait(i)
        r0, n = CHUNKS[i][1], CHUNKS[i][2]
        with scope("s2_down"):
            if r0 < FM:
                acc_m = down_mxu(hd, r0 // 128, (r0 + n) // 128, acc_m, True, [])
            else:
                for j in range(n // 16):
                    v = wd_n[pl.ds(r0 + j * 16, 16), :].astype(F32)
                    DF[pl.ds(r0 - FM + j * 16, 16), :] = v
                    acc_v = acc_v + v[0:8] * hcols[2 * j] + v[8:16] * hcols[2 * j + 1]
    acc_m = acc_m + _row_total(acc_v) * rstd
    x = x + xn + acc_m * sg

    if cfg["phase2"]:
        with scope("phase2"):
            mean, rstd = _ln_stats(x)
            marks = []
            front_mxu_qabs(front_mxu_q(_split(x), marks), marks)
            front_vpu(x, marks if cfg["gate"] else [])
            stage_attn(finish_front(mean, rstd))
            marks = []
            ctx_mxu(marks)
            acc_m = out_mxu(0, NMB, jnp.zeros((8, M), F32), False, marks)
            acc_v = back_vpu(NMB, NVB, jnp.zeros((8, M), F32), marks if cfg["gate"] else [])
            x = x + acc_m + _row_total(acc_v)
            mean, rstd = _ln_stats(x)
            xn = (x - mean) * rstd
            marks = []
            hd = gate_up_mxu(_split(x), mean, rstd, marks)
            y = down_mxu(hd, 0, NFM, jnp.zeros((8, M), F32), False, marks)
            acc_v, _ = ffn_vpu(x, rstd, marks if cfg["gate"] else [])
            sg = gate_scalar(xn, wr8)
            x = x + xn + (y + _row_total(acc_v) * rstd) * sg

    o_ref[0] = x[0:1].astype(BF)


def _run(cfg, A_x, A_c_kv, A_w_q, A_w_uk, A_w_uv, A_w_o, B_w_r, B_w_gate, B_w_up, B_w_down):
    any_spec = pl.BlockSpec(memory_space=pl.ANY)
    nmf, nmb = cfg["nmf"], cfg["nmb"]
    nvf, nvb = H - nmf, H - nmb
    fm = cfg["fm"]
    nsem = min(cfg["nsem"], len(_chunks(cfg)))
    scratch = [
        pltpu.VMEM((1, 1, M), BF),
        pltpu.VMEM((M,), BF),
        pltpu.VMEM((M, H, D), BF),
        pltpu.VMEM((DC, H, D), BF),
        pltpu.VMEM((DC, H, D), BF),
        pltpu.VMEM((SK, DC), BF),
        pltpu.VMEM((H, D, M), BF),
        pltpu.VMEM((F, M), BF),
        pltpu.VMEM((F, M), BF),
        pltpu.VMEM((F, M), BF),
        pltpu.VMEM(((H + 2) * SQ, 128), U32),
        pltpu.VMEM(((H + 2) * SV, 128), U32),
        pltpu.VMEM((4 * nmf * 64, 128), U32),
        pltpu.VMEM(((H + 2) * SV, 128), U32),
        pltpu.VMEM((32 * 4 * 64, 128), U32),
        pltpu.VMEM((4 * 2048, 128), U32),
        pltpu.VMEM((fm // 128 * 320, 128), U32),
        pltpu.VMEM((fm // 128 * 320, 128), U32),
        pltpu.VMEM((H * 8, 128), U32),
        pltpu.VMEM((4 * H, 128), U32),
        pltpu.VMEM((nvf * 128, M), F32),
        pltpu.VMEM((nvf * 128, DC), F32),
        pltpu.VMEM((nvb * 128, DC), F32),
        pltpu.VMEM((nvb * 128, M), F32),
        pltpu.VMEM((F - fm, M), F32),
        pltpu.VMEM((F - fm, M), F32),
        pltpu.VMEM((F - fm, M), F32),
        pltpu.VMEM((4 * H, 128), F32),
        pltpu.VMEM((8, fm), F32),
        pltpu.VMEM((8, fm), F32),
        pltpu.VMEM((4 * H, 128), F32),
        pltpu.VMEM((4 * H, 128), F32),
        pltpu.VMEM(((4 * nvf + 2) * SP, 128), F32),
        pltpu.VMEM((nmb * 5 * 64, 128), U32),
        pltpu.VMEM((fm // 128 * 5 * 64, 128), U32),
        pltpu.VMEM((8, 128), jnp.int32),
        pltpu.SemaphoreType.DMA((nsem,)),
    ]
    return pl.pallas_call(
        functools.partial(_kernel, cfg),
        out_shape=jax.ShapeDtypeStruct((1, 1, M), BF),
        in_specs=[any_spec] * 10,
        out_specs=pl.BlockSpec(memory_space=pltpu.VMEM),
        scratch_shapes=scratch,
        compiler_params=pltpu.CompilerParams(vmem_limit_bytes=110 * 1024 * 1024),
    )(A_x, A_c_kv, A_w_q, A_w_uk, A_w_uv, A_w_o, B_w_r, B_w_gate.T, B_w_up.T, B_w_down)


def build(**overrides):
    cfg = dict(DEFAULT_CFG, **overrides)

    @jax.jit
    def fn(A_x, A_c_kv, A_w_q, A_w_uk, A_w_uv, A_w_o, B_x, B_w_r, B_w_gate, B_w_up, B_w_down):
        return _run(cfg, A_x, A_c_kv, A_w_q, A_w_uk, A_w_uv, A_w_o, B_w_r, B_w_gate, B_w_up, B_w_down)
    return fn


@jax.jit
def pallas_interleave_layers__compressed_kv_cla__moe_arch_mod__decode_kernel(
    A_x: jax.Array,
    A_c_kv: jax.Array,
    A_w_q: jax.Array,
    A_w_uk: jax.Array,
    A_w_uv: jax.Array,
    A_w_o: jax.Array,
    B_x: jax.Array,
    B_w_r: jax.Array,
    B_w_gate: jax.Array,
    B_w_up: jax.Array,
    B_w_down: jax.Array,
):
    del B_x
    return _run(DEFAULT_CFG, A_x, A_c_kv, A_w_q, A_w_uk, A_w_uv, A_w_o, B_w_r, B_w_gate, B_w_up,
                B_w_down)
```

```python
import functools

import jax
import jax.numpy as jnp
from jax import lax
from jax.experimental import pallas as pl
from jax.experimental.pallas import tpu as pltpu

M = 640
H = 32
D = 128
DC = 512
SK = 4096
F = 1728
EPS = 1e-5

SQ = 322
SP = 9
SV = 258

BF = jnp.bfloat16
F32 = jnp.float32
U32 = jnp.uint32


def _bf(u32_val):
    return pltpu.bitcast(u32_val, BF)


def _u32(bf_val):
    return pltpu.bitcast(bf_val, U32)


def _dup(v8):
    return jnp.concatenate([v8, v8], axis=0).astype(BF)


def _dot(a, b):
    return jnp.dot(a, b, preferred_element_type=F32)


def _dot_nt(a, b):
    return lax.dot_general(a, b, (((1,), (1,)), ((), ())), preferred_element_type=F32)


def _split(v8):
    hi = pltpu.bitcast(pltpu.bitcast(v8, U32) & jnp.uint32(0xFFFF0000), F32)
    return jnp.concatenate([hi, v8 - hi], axis=0).astype(BF)


def _dot2(a16, b):
    r = _dot(a16, b)
    return r[0:8] + r[8:16]


def _ln_stats(x8):
    s1 = jnp.sum(x8, axis=1, keepdims=True)
    s2 = jnp.sum(x8 * x8, axis=1, keepdims=True)
    mean = s1 * (1.0 / M)
    var = jnp.maximum(s2 * (1.0 / M) - mean * mean, 0.0)
    return mean, lax.rsqrt(var + EPS)


def _swiglu(g, u):
    a = 0.5 * g
    b = a * u
    return b * jnp.tanh(a) + b


def _bcast_row(ref, row):
    return jnp.broadcast_to(ref[pl.ds(row, 1), :], (8, 128))


def _lane_blocks_sum(p):
    n = p.shape[1] // 128
    acc = p[:, 0:128]
    for i in range(1, n):
        acc = acc + p[:, i * 128:(i + 1) * 128]
    return acc


def _row_total(a8):
    return jnp.broadcast_to(jnp.sum(a8, axis=0, keepdims=True), a8.shape)


def _eye():
    r = lax.broadcasted_iota(jnp.int32, (128, 128), 0)
    c = lax.broadcasted_iota(jnp.int32, (128, 128), 1)
    return jnp.where(r == c, 1.0, 0.0).astype(BF)


def _transpose_tile(eye, tile):
    return _u32(_dot_nt(eye, tile).astype(BF))


def _chunks(cfg):
    fm = cfg["fm"]
    nm = cfg["nmb"]
    ch = []
    ch += [("wq", i * 128, 128) for i in range(5)]
    ch += [("wuk", i * 128, 128) for i in range(4)]
    ch += [("ckv", i * 1024, 1024) for i in range(4)]
    ch += [("wuv", i * 128, 128) for i in range(4)]
    ch += [("wo", h0, min(8, H - h0)) for h0 in range(nm, H, 8)]
    ch += [("wo", h0, min(8, nm - h0)) for h0 in range(0, nm, 8)]
    for name in ("wg", "wu"):
        ch += [(name, fm, F - fm)]
        ch += [(name, r0, min(512, fm - r0)) for r0 in range(0, fm, 512)]
    late = cfg["late"]
    ch += [("wd", fm, F - fm - late)]
    r0 = 0
    while r0 < fm - 128:
        n = min(512, fm - 128 - r0)
        ch.append(("wd", r0, n))
        r0 += n
    ch.append(("wd", fm - 128, 128))
    if late:
        ch.append(("wd", F - late, late))
    return ch


DEFAULT_CFG = dict(
    phase2=True, compute1=True, scopes=False,
    u_ckv=4, u_rp=4,
    nmf=18, nmb=16, fm=1024,
    nsem=5, late=128, small_after=0,
    gate=True, lag_f=2, beta_f=1.0, lag_b=1, beta_b=1.0, lag_n=8, beta_n=1.0, gstep=8,
    hmajor=True)


class _NoScope:
    def __enter__(self):
        return self

    def __exit__(self, *a):
        return False


def _kernel(cfg, x_hbm, ckv_hbm, wq_hbm, wuk_hbm, wuv_hbm, wo_hbm, wr_hbm, wg_hbm, wu_hbm, wd_hbm,
            o_ref,
            x_s, wr_s, wq_n, wuk_n, wuv_n, ckv_n, wo_n, wg_n, wu_n, wd_n,
            WQ, UP, UT, UV, CKT, CK, GT, UPT, QD, CL,
            WQT, UTF, UVT, WOF, GF, UF, DF, CSA, CSG, CSU, CLF, QAR, PS, WOU, WDU, FLAG,
            sems):
    NMF = cfg["nmf"]
    NVF = H - NMF
    NMB = cfg["nmb"]
    NVB = H - NMB
    FM = cfg["fm"]
    NFM = FM // 128
    NG = (F - FM) // 8
    CHUNKS = _chunks(cfg)
    NCH = len(CHUNKS)
    NSEM = min(cfg["nsem"], NCH)

    hbm = dict(wq=wq_hbm, wuk=wuk_hbm, wuv=wuv_hbm, wo=wo_hbm, wg=wg_hbm, wu=wu_hbm, wd=wd_hbm,
               ckv=ckv_hbm.at[0])
    vm = dict(wq=wq_n, wuk=wuk_n, wuv=wuv_n, wo=wo_n, wg=wg_n, wu=wu_n, wd=wd_n, ckv=ckv_n)

    def chunk_copy(i):
        name, r0, n = CHUNKS[i]
        return pltpu.make_async_copy(hbm[name].at[pl.ds(r0, n)], vm[name].at[pl.ds(r0, n)],
                                     sems.at[(i + 2) % NSEM])

    def scope(name):
        return jax.named_scope(name) if cfg["scopes"] else _NoScope()

    def wait(i):
        with scope("wait%02d_%s" % (i, CHUNKS[i][0])):
            chunk_copy(i).wait()
        if i + NSEM < NCH:
            chunk_copy(i + NSEM).start()

    def idx(name):
        return [i for i, c in enumerate(CHUNKS) if c[0] == name]

    cx = pltpu.make_async_copy(x_hbm, x_s, sems.at[0])
    cr = pltpu.make_async_copy(wr_hbm, wr_s, sems.at[1])
    for i in range(NSEM - 2):
        if i == cfg["small_after"]:
            cx.start()
            cr.start()
        chunk_copy(i).start()

    FLAG[...] = jnp.ones((8, 128), jnp.int32)

    def repack(src_n, dst, stride, j0, nj):
        def body(j, c):
            a = _u32(src_n[2 * j])
            b = _u32(src_n[2 * j + 1])
            lo = (a & jnp.uint32(0xFFFF)) | (b << 16)
            hi = (a >> 16) | (b & jnp.uint32(0xFFFF0000))
            dst[pl.ds(j, 16, stride=2 * stride), :] = lo
            dst[pl.ds(stride + j, 16, stride=2 * stride), :] = hi
            return c
        lax.fori_loop(j0, j0 + nj, body, 0, unroll=cfg["u_rp"])

    def vpu_transposes(src, stride, kb, dst, NM):
        eye = _eye()

        def body(hv, c):
            tile = _bf(src[pl.ds((NM + hv) * stride + kb * 64, 64), :])
            row = pl.multiple_of(hv * 128, 128)
            dst[pl.ds(row, 128), pl.ds(kb * 128, 128)] = _dot_nt(eye, tile)
            return c
        lax.fori_loop(0, H - NM, body, 0, unroll=True)

    def prep_wuk_transpose(cb):
        eye = _eye()

        def body(h, c):
            tile = _bf(UP[pl.ds(h * SV + cb * 64, 64), :])
            UT[pl.ds((cb * NMF + h) * 64, 64), :] = _transpose_tile(eye, tile)
            return c
        lax.fori_loop(0, NMF, body, 0, unroll=True)

    def prep_ckv(kb0, nkb):
        eye = _eye()

        def body(kb, c):
            r0 = pl.multiple_of(kb * 128, 128)
            for cb in range(4):
                tile = ckv_n[pl.ds(r0, 128), pl.ds(cb * 128, 128)]
                CK[pl.ds(cb * 2048 + kb * 64, 64), :] = _u32(tile)
                CKT[pl.ds((kb * 4 + cb) * 64, 64), :] = _transpose_tile(eye, tile)
            return c
        lax.fori_loop(kb0, kb0 + nkb, body, 0, unroll=cfg["u_ckv"])

    def prep_ffn_mxu(src_n, dst, r0, n):
        eye = _eye()

        def body(nb, c):
            row = pl.multiple_of(nb * 128, 128)
            for kb in range(5):
                tile = src_n[pl.ds(row, 128), pl.ds(kb * 128, 128)]
                dst[pl.ds((nb * 5 + kb) * 64, 64), :] = _transpose_tile(eye, tile)
            return c
        lax.fori_loop(r0 // 128, (r0 + n) // 128, body, 0, unroll=True)

    def centered(v):
        return v - jnp.sum(v, axis=1, keepdims=True) * (1.0 / M)

    def unpack_rows(src, r0, n, dst, center):
        step = 16
        nit = n // step
        unroll = max(u for u in range(1, 13) if nit % u == 0)

        def body(i, c):
            r = pl.multiple_of(i * step, step)
            v = src[pl.ds(r0 + r, step), :].astype(F32)
            dst[pl.ds(r, step), :] = centered(v) if center else v
            return c
        lax.fori_loop(0, nit, body, 0, unroll=unroll)

    def center_wqt():
        for i in range(NVF * 8):
            rows = pl.ds(i * 16, 16)
            WQT[rows, :] = centered(WQT[rows, :])

    def unpack_wo(h0, nh):
        def body(h, c):
            row = pl.multiple_of((h - NMB) * 128, 128)
            WOF[pl.ds(row, 128), :] = wo_n[h].astype(F32)
            return c
        lax.fori_loop(h0, h0 + nh, body, 0)

    def gate(v, marks, frac):
        if not marks or frac <= 0.0:
            return v
        total = marks[-1][0]
        pick = None
        for done, val in marks:
            if done <= frac * total:
                pick = val
        if pick is None:
            return v
        always = FLAG[...] != 0
        return jnp.concatenate(
            [jnp.where(always, v[:, i * 128:(i + 1) * 128], pick) for i in range(v.shape[1] // 128)],
            axis=1)

    def front_mxu_q(xs, marks):
        qs = []
        for h in range(NMF):
            r = _dot2(xs, _bf(WQ[pl.ds(h * SQ, 320), :]))
            qs.append(_split(r))
            marks.append(((marks[-1][0] if marks else 0) + 5, r))
        return qs

    def front_mxu_qabs(qs, marks):
        order = ([(h, cb) for h in range(NMF) for cb in range(4)] if cfg["hmajor"] else
                 [(h, cb) for cb in range(4) for h in range(NMF)])
        for h, cb in order:
            r = _dot2(qs[h], _bf(UT[pl.ds((cb * NMF + h) * 64, 64), :]))
            QAR[pl.ds(cb * H + h, 1), :] = r[0:1]
            marks.append(((marks[-1][0] if marks else 0) + 1, r))

    def front_vpu(xn, marks):
        a = [None] * 4
        for hv in range(NVF):
            xh = gate(xn, marks, cfg["beta_f"] * (hv - cfg["lag_f"]) / NVF)
            for g in range(16):
                rows = pl.ds(hv * 128 + g * 8, 8)
                qc = jnp.sum(_lane_blocks_sum(WQT[rows, :] * xh), axis=1, keepdims=True)
                for cb in range(4):
                    t = UTF[rows, pl.ds(cb * 128, 128)] * qc
                    a[cb] = a[cb] + t if g > 0 else t
            for cb in range(4):
                PS[pl.ds((cb * NVF + hv) * SP, 8), :] = a[cb]
        for cb in range(4):
            for hv0 in range(0, NVF, 8):
                n = min(8, NVF - hv0)
                tot = None
                for s_ in range(8):
                    t = PS[pl.ds((cb * NVF + hv0) * SP + s_, n, stride=SP), :]
                    tot = t if tot is None else tot + t
                QAR[pl.ds(cb * H + NMF + hv0, n), :] = tot

    def finish_front(mean, rstd):
        row = lax.broadcasted_iota(jnp.int32, (H, 1), 0)
        mean32 = jnp.concatenate([mean] * 4, axis=0)
        rstd32 = jnp.concatenate([rstd] * 4, axis=0)
        off = jnp.where(row < NMF, mean32, 0.0)
        mul = rstd32 * (D ** -0.5)
        return jnp.concatenate(
            [((QAR[pl.ds(cb * H, H), :] - off * CSA[pl.ds(cb * H, H), :]) * mul).astype(BF)
             for cb in range(4)], axis=1)

    def scores(qa, nb0, nnb):
        return jnp.concatenate(
            [_dot(qa, _bf(CKT[pl.ds(nb * 256, 256), :])) for nb in range(nb0, nb0 + nnb)], axis=1)

    def pv(p, kb0, nkb):
        return jnp.concatenate(
            [_dot(p, _bf(CK[pl.ds(cb * 2048 + kb0 * 64, nkb * 64), :])) for cb in range(4)], axis=1)

    def stage_attn(qa):
        sa = scores(qa, 0, 16)
        sb = scores(qa, 16, 16)
        ma = jnp.max(sa, axis=1, keepdims=True)
        pa = jnp.exp(sa - ma)
        la = jnp.sum(pa, axis=1, keepdims=True)
        ca = pv(pa.astype(BF), 0, 16)
        m = jnp.maximum(ma, jnp.max(sb, axis=1, keepdims=True))
        pb = jnp.exp(sb - m)
        lb = jnp.sum(pb, axis=1, keepdims=True)
        cbv = pv(pb.astype(BF), 16, 16)
        alpha = jnp.exp(ma - m)
        inv = 1.0 / (alpha * la + lb)
        cl = (alpha * ca + cbv) * inv
        nm8 = -(-NMB // 8) * 8
        nv0 = NMB // 8 * 8
        bits = pltpu.bitcast(cl[0:nm8].astype(BF).astype(F32), U32)
        dupw = bits | (bits >> 16)
        for cb in range(4):
            CL[pl.ds(cb * H, nm8), :] = dupw[:, cb * 128:(cb + 1) * 128]
            CLF[pl.ds(cb * H + nv0, H - nv0), :] = cl[nv0:H, cb * 128:(cb + 1) * 128]

    def ctx_mxu(marks):
        r = [None] * NMB
        for cb in range(4):
            for h in range(NMB):
                lhs = _bf(_bcast_row(CL, cb * H + h))
                t = _dot(lhs, _bf(UV[pl.ds(h * SV + cb * 64, 64), :]))[0:8]
                r[h] = t if cb == 0 else r[h] + t
                marks.append(((marks[-1][0] if marks else 0) + 1, t))
        for h in range(NMB):
            QD[pl.ds(h * 8, 8), :] = _u32(_dup(r[h]))

    def out_mxu(h0, nh, acc, first, marks):
        for h in range(h0, h0 + nh):
            if first:
                w = wo_n[h]
                for mb in range(5):
                    WOU[pl.ds((h * 5 + mb) * 64, 64), :] = _u32(w[:, mb * 128:(mb + 1) * 128])
            else:
                w = jnp.concatenate(
                    [_bf(WOU[pl.ds((h * 5 + mb) * 64, 64), :]) for mb in range(5)], axis=1)
            r = _dot(_bf(QD[pl.ds(h * 8, 8), :]), w)[0:8]
            acc = acc + r
            marks.append(((marks[-1][0] if marks else 0) + 5, r[:, 0:128]))
        return acc

    def back_vpu(h0, nh, acc, marks):
        for h in range(h0, h0 + nh):
            hv = h - NMB
            cl = jnp.concatenate(
                [_bcast_row(CLF, cb * H + h) for cb in range(4)], axis=1)
            cl = gate(cl, marks, cfg["beta_b"] * (hv - cfg["lag_b"]) / NVB)
            for g in range(16):
                rows = pl.ds(hv * 128 + g * 8, 8)
                cc = jnp.sum(_lane_blocks_sum(UVT[rows, :] * cl), axis=1, keepdims=True)
                acc = acc + WOF[rows, :] * cc
        return acc

    def gate_up_mxu_raw(xs, marks):
        g, u = [], []
        for nb in range(NFM):
            g.append(_dot2(xs, _bf(GT[pl.ds(nb * 320, 320), :])))
            marks.append(((marks[-1][0] if marks else 0) + 5, g[-1]))
            u.append(_dot2(xs, _bf(UPT[pl.ds(nb * 320, 320), :])))
            marks.append((marks[-1][0] + 5, u[-1]))
        return g, u

    def gate_up_mxu(xs, mean, rstd, marks):
        g, u = gate_up_mxu_raw(xs, marks)
        hd = []
        for nb in range(NFM):
            cols = pl.ds(nb * 128, 128)
            gg = (g[nb] - mean * CSG[:, cols]) * rstd
            uu = (u[nb] - mean * CSU[:, cols]) * rstd
            hd.append(_dup(_swiglu(gg, uu)))
        return hd

    def down_mxu(hd, nb0, nb1, acc, first, marks):
        for nb in range(nb0, nb1):
            if first:
                w = wd_n[pl.ds(nb * 128, 128), :]
                for mb in range(5):
                    WDU[pl.ds((nb * 5 + mb) * 64, 64), :] = _u32(w[:, mb * 128:(mb + 1) * 128])
            else:
                w = jnp.concatenate(
                    [_bf(WDU[pl.ds((nb * 5 + mb) * 64, 64), :]) for mb in range(5)], axis=1)
            r = _dot(hd[nb], w)[0:8]
            acc = acc + r
            marks.append(((marks[-1][0] if marks else 0) + 5, r[:, 0:128]))
        return acc

    def ffn_vpu(x8, rstd, marks, nlate=0):
        acc = None
        xg = x8
        hcols = []
        half_rstd = 0.5 * rstd
        for g in range(NG):
            if g % cfg["gstep"] == 0:
                xg = gate(x8, marks, cfg["beta_n"] * (g - cfg["lag_n"]) / NG)
            rows = pl.ds(g * 8, 8)
            gc = jnp.sum(_lane_blocks_sum(GF[rows, :] * xg), axis=1, keepdims=True)
            uc = jnp.sum(_lane_blocks_sum(UF[rows, :] * xg), axis=1, keepdims=True)
            a = gc * half_rstd
            b = a * uc
            hc = b * jnp.tanh(a) + b
            if g >= NG - nlate:
                hcols.append(hc)
            else:
                t = DF[rows, :] * hc
                acc = t if acc is None else acc + t
        return acc, hcols

    def gate_scalar(xn, wr8):
        return jax.nn.sigmoid(jnp.sum(xn * wr8, axis=1, keepdims=True))

    ones_split = jnp.concatenate([jnp.ones((8, M), BF), jnp.zeros((8, M), BF)], axis=0)

    cx.wait()
    chunk_copy(NSEM - 2).start()
    cr.wait()
    chunk_copy(NSEM - 1).start()
    x = jnp.broadcast_to(x_s[0].astype(F32), (8, M))
    wr8 = jnp.broadcast_to(wr_s[...].reshape(1, M).astype(F32), (8, M))

    if not cfg["compute1"]:
        for i in range(NCH):
            wait(i)
        o_ref[0] = x[0:1].astype(BF)
        return

    for k, i in enumerate(idx("wq")):
        wait(i)
        with scope("p_wq"):
            repack(wq_n, WQ, SQ, k * 64, 64)
            vpu_transposes(WQ, SQ, k, WQT, NMF)
    with scope("s1_csq"):
        center_wqt()
    for k, i in enumerate(idx("wuk")):
        wait(i)
        with scope("p_wuk"):
            repack(wuk_n, UP, SV, k * 64, 64)
            prep_wuk_transpose(k)
            vpu_transposes(UP, SV, k, UTF, NMF)
    with scope("s1_csa"):
        front_mxu_qabs(front_mxu_q(ones_split, []), [])
        for cb in range(4):
            CSA[pl.ds(cb * H, NMF), :] = QAR[pl.ds(cb * H, NMF), :]
            CSA[pl.ds(cb * H + NMF, NVF), :] = jnp.zeros((NVF, 128), F32)
    with scope("s1_front"):
        mean, rstd = _ln_stats(x)
        front_mxu_qabs(front_mxu_q(_split(x), []), [])
        front_vpu(x, [])
        qa = finish_front(mean, rstd)
    for k, i in enumerate(idx("ckv")):
        wait(i)
        with scope("p_ckv"):
            prep_ckv(k * 8, 8)
    with scope("s1_attn"):
        stage_attn(qa)
    for k, i in enumerate(idx("wuv")):
        wait(i)
        with scope("p_wuv"):
            repack(wuv_n, UV, SV, k * 64, 64)
            vpu_transposes(UV, SV, k, UVT, NMB)
    with scope("s1_ctx"):
        ctx_mxu([])
    acc_v = jnp.zeros((8, M), F32)
    acc_m = jnp.zeros((8, M), F32)
    for i in idx("wo"):
        wait(i)
        h0, nh = CHUNKS[i][1], CHUNKS[i][2]
        with scope("s1_out"):
            if h0 >= NMB:
                unpack_wo(h0, nh)
                acc_v = back_vpu(h0, nh, acc_v, [])
            else:
                acc_m = out_mxu(h0, nh, acc_m, True, [])
    x = x + acc_m + _row_total(acc_v)
    for name, nat, tr, fl in (("wg", wg_n, GT, GF), ("wu", wu_n, UPT, UF)):
        for i in idx(name):
            wait(i)
            r0, n = CHUNKS[i][1], CHUNKS[i][2]
            with scope("p_" + name):
                if r0 >= FM:
                    unpack_rows(nat, r0, n, fl, True)
                else:
                    prep_ffn_mxu(nat, tr, r0, n)
    with scope("s2_cs"):
        g, u = gate_up_mxu_raw(ones_split, [])
        CSG[...] = jnp.concatenate(g, axis=1)
        CSU[...] = jnp.concatenate(u, axis=1)
    wd_idx = idx("wd")
    LATE = cfg["late"]
    wait(wd_idx[0])
    with scope("p_wd"):
        unpack_rows(wd_n, FM, F - FM - LATE, DF, False)
    with scope("s2_gu"):
        mean, rstd = _ln_stats(x)
        xn = (x - mean) * rstd
        hd = gate_up_mxu(_split(x), mean, rstd, [])
        acc_v, hcols = ffn_vpu(x, rstd, [], LATE // 8)
        sg = gate_scalar(xn, wr8)
    acc_m = jnp.zeros((8, M), F32)
    for i in wd_idx[1:]:
        wait(i)
        r0, n = CHUNKS[i][1], CHUNKS[i][2]
        with scope("s2_down"):
            if r0 < FM:
                acc_m = down_mxu(hd, r0 // 128, (r0 + n) // 128, acc_m, True, [])
            else:
                for j in range(n // 16):
                    v = wd_n[pl.ds(r0 + j * 16, 16), :].astype(F32)
                    DF[pl.ds(r0 - FM + j * 16, 16), :] = v
                    acc_v = acc_v + v[0:8] * hcols[2 * j] + v[8:16] * hcols[2 * j + 1]
    acc_m = acc_m + _row_total(acc_v) * rstd
    x = x + xn + acc_m * sg

    if cfg["phase2"]:
        with scope("phase2"):
            mean, rstd = _ln_stats(x)
            marks = []
            front_mxu_qabs(front_mxu_q(_split(x), marks), marks)
            front_vpu(x, marks if cfg["gate"] else [])
            stage_attn(finish_front(mean, rstd))
            marks = []
            ctx_mxu(marks)
            acc_m = out_mxu(0, NMB, jnp.zeros((8, M), F32), False, marks)
            acc_v = back_vpu(NMB, NVB, jnp.zeros((8, M), F32), marks if cfg["gate"] else [])
            x = x + acc_m + _row_total(acc_v)
            mean, rstd = _ln_stats(x)
            xn = (x - mean) * rstd
            marks = []
            hd = gate_up_mxu(_split(x), mean, rstd, marks)
            y = down_mxu(hd, 0, NFM, jnp.zeros((8, M), F32), False, marks)
            acc_v, _ = ffn_vpu(x, rstd, marks if cfg["gate"] else [])
            sg = gate_scalar(xn, wr8)
            x = x + xn + (y + _row_total(acc_v) * rstd) * sg

    o_ref[0] = x[0:1].astype(BF)


def _run(cfg, A_x, A_c_kv, A_w_q, A_w_uk, A_w_uv, A_w_o, B_w_r, B_w_gate, B_w_up, B_w_down):
    any_spec = pl.BlockSpec(memory_space=pl.ANY)
    nmf, nmb = cfg["nmf"], cfg["nmb"]
    nvf, nvb = H - nmf, H - nmb
    fm = cfg["fm"]
    nsem = min(cfg["nsem"], len(_chunks(cfg)))
    scratch = [
        pltpu.VMEM((1, 1, M), BF),
        pltpu.VMEM((M,), BF),
        pltpu.VMEM((M, H, D), BF),
        pltpu.VMEM((DC, H, D), BF),
        pltpu.VMEM((DC, H, D), BF),
        pltpu.VMEM((SK, DC), BF),
        pltpu.VMEM((H, D, M), BF),
        pltpu.VMEM((F, M), BF),
        pltpu.VMEM((F, M), BF),
        pltpu.VMEM((F, M), BF),
        pltpu.VMEM(((H + 2) * SQ, 128), U32),
        pltpu.VMEM(((H + 2) * SV, 128), U32),
        pltpu.VMEM((4 * nmf * 64, 128), U32),
        pltpu.VMEM(((H + 2) * SV, 128), U32),
        pltpu.VMEM((32 * 4 * 64, 128), U32),
        pltpu.VMEM((4 * 2048, 128), U32),
        pltpu.VMEM((fm // 128 * 320, 128), U32),
        pltpu.VMEM((fm // 128 * 320, 128), U32),
        pltpu.VMEM((H * 8, 128), U32),
        pltpu.VMEM((4 * H, 128), U32),
        pltpu.VMEM((nvf * 128, M), F32),
        pltpu.VMEM((nvf * 128, DC), F32),
        pltpu.VMEM((nvb * 128, DC), F32),
        pltpu.VMEM((nvb * 128, M), F32),
        pltpu.VMEM((F - fm, M), F32),
        pltpu.VMEM((F - fm, M), F32),
        pltpu.VMEM((F - fm, M), F32),
        pltpu.VMEM((4 * H, 128), F32),
        pltpu.VMEM((8, fm), F32),
        pltpu.VMEM((8, fm), F32),
        pltpu.VMEM((4 * H, 128), F32),
        pltpu.VMEM((4 * H, 128), F32),
        pltpu.VMEM(((4 * nvf + 2) * SP, 128), F32),
        pltpu.VMEM((nmb * 5 * 64, 128), U32),
        pltpu.VMEM((fm // 128 * 5 * 64, 128), U32),
        pltpu.VMEM((8, 128), jnp.int32),
        pltpu.SemaphoreType.DMA((nsem,)),
    ]
    return pl.pallas_call(
        functools.partial(_kernel, cfg),
        out_shape=jax.ShapeDtypeStruct((1, 1, M), BF),
        in_specs=[any_spec] * 10,
        out_specs=pl.BlockSpec(memory_space=pltpu.VMEM),
        scratch_shapes=scratch,
        compiler_params=pltpu.CompilerParams(vmem_limit_bytes=110 * 1024 * 1024),
    )(A_x, A_c_kv, A_w_q, A_w_uk, A_w_uv, A_w_o, B_w_r, B_w_gate.T, B_w_up.T, B_w_down)


def build(**overrides):
    cfg = dict(DEFAULT_CFG, **overrides)

    @jax.jit
    def fn(A_x, A_c_kv, A_w_q, A_w_uk, A_w_uv, A_w_o, B_x, B_w_r, B_w_gate, B_w_up, B_w_down):
        return _run(cfg, A_x, A_c_kv, A_w_q, A_w_uk, A_w_uv, A_w_o, B_w_r, B_w_gate, B_w_up, B_w_down)
    return fn


@jax.jit
def pallas_interleave_layers__compressed_kv_cla__moe_arch_mod__decode_kernel(
    A_x: jax.Array,
    A_c_kv: jax.Array,
    A_w_q: jax.Array,
    A_w_uk: jax.Array,
    A_w_uv: jax.Array,
    A_w_o: jax.Array,
    B_x: jax.Array,
    B_w_r: jax.Array,
    B_w_gate: jax.Array,
    B_w_up: jax.Array,
    B_w_down: jax.Array,
):
    del B_x
    return _run(DEFAULT_CFG, A_x, A_c_kv, A_w_q, A_w_uk, A_w_uv, A_w_o, B_w_r, B_w_gate, B_w_up,
                B_w_down)
```

```python
import functools

import jax
import jax.numpy as jnp
from jax import lax
from jax.experimental import pallas as pl
from jax.experimental.pallas import tpu as pltpu

M = 640
H = 32
D = 128
DC = 512
SK = 4096
F = 1728
EPS = 1e-5

SQ = 322
SP = 9
SV = 258

BF = jnp.bfloat16
F32 = jnp.float32
U32 = jnp.uint32


def _bf(u32_val):
    return pltpu.bitcast(u32_val, BF)


def _u32(bf_val):
    return pltpu.bitcast(bf_val, U32)


def _dup(v8):
    return jnp.concatenate([v8, v8], axis=0).astype(BF)


def _dot(a, b):
    return jnp.dot(a, b, preferred_element_type=F32)


def _dot_nt(a, b):
    return lax.dot_general(a, b, (((1,), (1,)), ((), ())), preferred_element_type=F32)


def _split(v8):
    hi = pltpu.bitcast(pltpu.bitcast(v8, U32) & jnp.uint32(0xFFFF0000), F32)
    return jnp.concatenate([hi, v8 - hi], axis=0).astype(BF)


def _dot2(a16, b):
    r = _dot(a16, b)
    return r[0:8] + r[8:16]


def _ln_stats(x8):
    s1 = jnp.sum(x8, axis=1, keepdims=True)
    s2 = jnp.sum(x8 * x8, axis=1, keepdims=True)
    mean = s1 * (1.0 / M)
    var = jnp.maximum(s2 * (1.0 / M) - mean * mean, 0.0)
    return mean, lax.rsqrt(var + EPS)


def _swiglu(g, u):
    a = 0.5 * g
    b = a * u
    return b * jnp.tanh(a) + b


def _bcast_row(ref, row):
    return jnp.broadcast_to(ref[pl.ds(row, 1), :], (8, 128))


def _lane_blocks_sum(p):
    n = p.shape[1] // 128
    acc = p[:, 0:128]
    for i in range(1, n):
        acc = acc + p[:, i * 128:(i + 1) * 128]
    return acc


def _row_total(a8):
    return jnp.broadcast_to(jnp.sum(a8, axis=0, keepdims=True), a8.shape)


def _eye():
    r = lax.broadcasted_iota(jnp.int32, (128, 128), 0)
    c = lax.broadcasted_iota(jnp.int32, (128, 128), 1)
    return jnp.where(r == c, 1.0, 0.0).astype(BF)


def _transpose_tile(eye, tile):
    return _u32(_dot_nt(eye, tile).astype(BF))


def _chunks(cfg):
    fm = cfg["fm"]
    nm = cfg["nmb"]
    ch = []
    ch += [("wq", i * 128, 128) for i in range(5)]
    ch += [("wuk", i * 128, 128) for i in range(4)]
    ch += [("ckv", i * 1024, 1024) for i in range(4)]
    ch += [("wuv", i * 128, 128) for i in range(4)]
    ch += [("wo", h0, min(8, H - h0)) for h0 in range(nm, H, 8)]
    ch += [("wo", h0, min(8, nm - h0)) for h0 in range(0, nm, 8)]
    for name in ("wg", "wu"):
        ch += [(name, fm, F - fm)]
        ch += [(name, r0, min(512, fm - r0)) for r0 in range(0, fm, 512)]
    late = cfg["late"]
    ch += [("wd", fm, F - fm - late)]
    r0 = 0
    while r0 < fm - 128:
        n = min(512, fm - 128 - r0)
        ch.append(("wd", r0, n))
        r0 += n
    ch.append(("wd", fm - 128, 128))
    if late:
        ch.append(("wd", F - late, late))
    return ch


DEFAULT_CFG = dict(
    phase2=True, compute1=True, scopes=False,
    u_ckv=4, u_rp=4,
    nmf=18, nmb=16, fm=1024,
    nsem=5, late=128, small_after=0,
    gate=True, lag_f=2, beta_f=1.0, lag_b=1, beta_b=1.0, lag_n=8, beta_n=1.0, gstep=8,
    hmajor=True)


class _NoScope:
    def __enter__(self):
        return self

    def __exit__(self, *a):
        return False


def _kernel(cfg, x_hbm, ckv_hbm, wq_hbm, wuk_hbm, wuv_hbm, wo_hbm, wr_hbm, wg_hbm, wu_hbm, wd_hbm,
            o_ref,
            x_s, wr_s, wq_n, wuk_n, wuv_n, ckv_n, wo_n, wg_n, wu_n, wd_n,
            WQ, UP, UT, UV, CKT, CK, GT, UPT, CL,
            WQT, UTF, UVT, WOF, GF, UF, DF, CSA, CSG, CSU, CLF, QAR, PS, WOU, WDU, FLAG,
            sems):
    NMF = cfg["nmf"]
    NVF = H - NMF
    NMB = cfg["nmb"]
    NVB = H - NMB
    FM = cfg["fm"]
    NFM = FM // 128
    NG = (F - FM) // 8
    CHUNKS = _chunks(cfg)
    NCH = len(CHUNKS)
    NSEM = min(cfg["nsem"], NCH)

    hbm = dict(wq=wq_hbm, wuk=wuk_hbm, wuv=wuv_hbm, wo=wo_hbm, wg=wg_hbm, wu=wu_hbm, wd=wd_hbm,
               ckv=ckv_hbm.at[0])
    vm = dict(wq=wq_n, wuk=wuk_n, wuv=wuv_n, wo=wo_n, wg=wg_n, wu=wu_n, wd=wd_n, ckv=ckv_n)

    def chunk_copy(i):
        name, r0, n = CHUNKS[i]
        return pltpu.make_async_copy(hbm[name].at[pl.ds(r0, n)], vm[name].at[pl.ds(r0, n)],
                                     sems.at[(i + 2) % NSEM])

    def scope(name):
        return jax.named_scope(name) if cfg["scopes"] else _NoScope()

    def wait(i):
        with scope("wait%02d_%s" % (i, CHUNKS[i][0])):
            chunk_copy(i).wait()
        if i + NSEM < NCH:
            chunk_copy(i + NSEM).start()

    def idx(name):
        return [i for i, c in enumerate(CHUNKS) if c[0] == name]

    cx = pltpu.make_async_copy(x_hbm, x_s, sems.at[0])
    cr = pltpu.make_async_copy(wr_hbm, wr_s, sems.at[1])
    for i in range(NSEM - 2):
        if i == cfg["small_after"]:
            cx.start()
            cr.start()
        chunk_copy(i).start()

    FLAG[...] = jnp.ones((8, 128), jnp.int32)

    def repack(src_n, dst, stride, j0, nj):
        def body(j, c):
            a = _u32(src_n[2 * j])
            b = _u32(src_n[2 * j + 1])
            lo = (a & jnp.uint32(0xFFFF)) | (b << 16)
            hi = (a >> 16) | (b & jnp.uint32(0xFFFF0000))
            dst[pl.ds(j, 16, stride=2 * stride), :] = lo
            dst[pl.ds(stride + j, 16, stride=2 * stride), :] = hi
            return c
        lax.fori_loop(j0, j0 + nj, body, 0, unroll=cfg["u_rp"])

    def vpu_transposes(src, stride, kb, dst, NM):
        eye = _eye()

        def body(hv, c):
            tile = _bf(src[pl.ds((NM + hv) * stride + kb * 64, 64), :])
            row = pl.multiple_of(hv * 128, 128)
            dst[pl.ds(row, 128), pl.ds(kb * 128, 128)] = _dot_nt(eye, tile)
            return c
        lax.fori_loop(0, H - NM, body, 0, unroll=True)

    def prep_wuk_transpose(cb):
        eye = _eye()

        def body(h, c):
            tile = _bf(UP[pl.ds(h * SV + cb * 64, 64), :])
            UT[pl.ds((cb * NMF + h) * 64, 64), :] = _transpose_tile(eye, tile)
            return c
        lax.fori_loop(0, NMF, body, 0, unroll=True)

    def prep_ckv(kb0, nkb):
        eye = _eye()

        def body(kb, c):
            r0 = pl.multiple_of(kb * 128, 128)
            for cb in range(4):
                tile = ckv_n[pl.ds(r0, 128), pl.ds(cb * 128, 128)]
                CK[pl.ds(cb * 2048 + kb * 64, 64), :] = _u32(tile)
                CKT[pl.ds((kb * 4 + cb) * 64, 64), :] = _transpose_tile(eye, tile)
            return c
        lax.fori_loop(kb0, kb0 + nkb, body, 0, unroll=cfg["u_ckv"])

    def prep_ffn_mxu(src_n, dst, r0, n):
        eye = _eye()

        def body(nb, c):
            row = pl.multiple_of(nb * 128, 128)
            for kb in range(5):
                tile = src_n[pl.ds(row, 128), pl.ds(kb * 128, 128)]
                dst[pl.ds((nb * 5 + kb) * 64, 64), :] = _transpose_tile(eye, tile)
            return c
        lax.fori_loop(r0 // 128, (r0 + n) // 128, body, 0, unroll=True)

    def centered(v):
        return v - jnp.sum(v, axis=1, keepdims=True) * (1.0 / M)

    def unpack_rows(src, r0, n, dst, center):
        step = 16
        nit = n // step
        unroll = max(u for u in range(1, 13) if nit % u == 0)

        def body(i, c):
            r = pl.multiple_of(i * step, step)
            v = src[pl.ds(r0 + r, step), :].astype(F32)
            dst[pl.ds(r, step), :] = centered(v) if center else v
            return c
        lax.fori_loop(0, nit, body, 0, unroll=unroll)

    def center_wqt():
        for i in range(NVF * 8):
            rows = pl.ds(i * 16, 16)
            WQT[rows, :] = centered(WQT[rows, :])

    def unpack_wo(h0, nh):
        def body(h, c):
            row = pl.multiple_of((h - NMB) * 128, 128)
            WOF[pl.ds(row, 128), :] = wo_n[h].astype(F32)
            return c
        lax.fori_loop(h0, h0 + nh, body, 0)

    def gate(v, marks, frac):
        if not marks or frac <= 0.0:
            return v
        total = marks[-1][0]
        pick = None
        for done, val in marks:
            if done <= frac * total:
                pick = val
        if pick is None:
            return v
        always = FLAG[...] != 0
        return jnp.concatenate(
            [jnp.where(always, v[:, i * 128:(i + 1) * 128], pick) for i in range(v.shape[1] // 128)],
            axis=1)

    def front_mxu_q(xs, marks):
        qs = []
        for h in range(NMF):
            r = _dot2(xs, _bf(WQ[pl.ds(h * SQ, 320), :]))
            qs.append(_split(r))
            marks.append(((marks[-1][0] if marks else 0) + 5, r))
        return qs

    def front_mxu_qabs(qs, marks):
        order = ([(h, cb) for h in range(NMF) for cb in range(4)] if cfg["hmajor"] else
                 [(h, cb) for cb in range(4) for h in range(NMF)])
        for h, cb in order:
            r = _dot2(qs[h], _bf(UT[pl.ds((cb * NMF + h) * 64, 64), :]))
            QAR[pl.ds(cb * H + h, 1), :] = r[0:1]
            marks.append(((marks[-1][0] if marks else 0) + 1, r))

    def front_vpu(xn, marks):
        a = [None] * 4
        for hv in range(NVF):
            xh = gate(xn, marks, cfg["beta_f"] * (hv - cfg["lag_f"]) / NVF)
            for g in range(16):
                rows = pl.ds(hv * 128 + g * 8, 8)
                qc = jnp.sum(_lane_blocks_sum(WQT[rows, :] * xh), axis=1, keepdims=True)
                for cb in range(4):
                    t = UTF[rows, pl.ds(cb * 128, 128)] * qc
                    a[cb] = a[cb] + t if g > 0 else t
            for cb in range(4):
                PS[pl.ds((cb * NVF + hv) * SP, 8), :] = a[cb]
        for cb in range(4):
            for hv0 in range(0, NVF, 8):
                n = min(8, NVF - hv0)
                tot = None
                for s_ in range(8):
                    t = PS[pl.ds((cb * NVF + hv0) * SP + s_, n, stride=SP), :]
                    tot = t if tot is None else tot + t
                QAR[pl.ds(cb * H + NMF + hv0, n), :] = tot

    def finish_front(mean, rstd):
        row = lax.broadcasted_iota(jnp.int32, (H, 1), 0)
        mean32 = jnp.concatenate([mean] * 4, axis=0)
        rstd32 = jnp.concatenate([rstd] * 4, axis=0)
        off = jnp.where(row < NMF, mean32, 0.0)
        mul = rstd32 * (D ** -0.5)
        return jnp.concatenate(
            [((QAR[pl.ds(cb * H, H), :] - off * CSA[pl.ds(cb * H, H), :]) * mul).astype(BF)
             for cb in range(4)], axis=1)

    def scores(qa, nb0, nnb):
        return jnp.concatenate(
            [_dot(qa, _bf(CKT[pl.ds(nb * 256, 256), :])) for nb in range(nb0, nb0 + nnb)], axis=1)

    def pv(p, kb0, nkb):
        return jnp.concatenate(
            [_dot(p, _bf(CK[pl.ds(cb * 2048 + kb0 * 64, nkb * 64), :])) for cb in range(4)], axis=1)

    def stage_attn(qa):
        sa = scores(qa, 0, 16)
        sb = scores(qa, 16, 16)
        ma = jnp.max(sa, axis=1, keepdims=True)
        pa = jnp.exp(sa - ma)
        la = jnp.sum(pa, axis=1, keepdims=True)
        ca = pv(pa.astype(BF), 0, 16)
        m = jnp.maximum(ma, jnp.max(sb, axis=1, keepdims=True))
        pb = jnp.exp(sb - m)
        lb = jnp.sum(pb, axis=1, keepdims=True)
        cbv = pv(pb.astype(BF), 16, 16)
        alpha = jnp.exp(ma - m)
        inv = 1.0 / (alpha * la + lb)
        cl = (alpha * ca + cbv) * inv
        nm8 = -(-NMB // 8) * 8
        nv0 = NMB // 8 * 8
        bits = pltpu.bitcast(cl[0:nm8].astype(BF).astype(F32), U32)
        dupw = bits | (bits >> 16)
        for cb in range(4):
            CL[pl.ds(cb * H, nm8), :] = dupw[:, cb * 128:(cb + 1) * 128]
            CLF[pl.ds(cb * H + nv0, H - nv0), :] = cl[nv0:H, cb * 128:(cb + 1) * 128]

    def ctx_mxu(marks):
        r = [None] * NMB
        for cb in range(4):
            for h in range(NMB):
                lhs = _bf(_bcast_row(CL, cb * H + h))
                t = _dot(lhs, _bf(UV[pl.ds(h * SV + cb * 64, 64), :]))[0:8]
                r[h] = t if cb == 0 else r[h] + t
                marks.append(((marks[-1][0] if marks else 0) + 1, t))
        return [_dup(v) for v in r]

    def out_mxu(ctx, h0, nh, acc, first, marks):
        for h in range(h0, h0 + nh):
            if first:
                w = wo_n[h]
                for mb in range(5):
                    WOU[pl.ds((h * 5 + mb) * 64, 64), :] = _u32(w[:, mb * 128:(mb + 1) * 128])
            else:
                w = jnp.concatenate(
                    [_bf(WOU[pl.ds((h * 5 + mb) * 64, 64), :]) for mb in range(5)], axis=1)
            r = _dot(ctx[h], w)[0:8]
            acc = acc + r
            marks.append(((marks[-1][0] if marks else 0) + 5, r[:, 0:128]))
        return acc

    def back_vpu(h0, nh, acc, marks):
        for h in range(h0, h0 + nh):
            hv = h - NMB
            cl = jnp.concatenate(
                [_bcast_row(CLF, cb * H + h) for cb in range(4)], axis=1)
            cl = gate(cl, marks, cfg["beta_b"] * (hv - cfg["lag_b"]) / NVB)
            for g in range(16):
                rows = pl.ds(hv * 128 + g * 8, 8)
                cc = jnp.sum(_lane_blocks_sum(UVT[rows, :] * cl), axis=1, keepdims=True)
                acc = acc + WOF[rows, :] * cc
        return acc

    def gate_up_mxu_raw(xs, marks):
        g, u = [], []
        for nb in range(NFM):
            g.append(_dot2(xs, _bf(GT[pl.ds(nb * 320, 320), :])))
            marks.append(((marks[-1][0] if marks else 0) + 5, g[-1]))
            u.append(_dot2(xs, _bf(UPT[pl.ds(nb * 320, 320), :])))
            marks.append((marks[-1][0] + 5, u[-1]))
        return g, u

    def gate_up_mxu(xs, mean, rstd, marks):
        g, u = gate_up_mxu_raw(xs, marks)
        hd = []
        for nb in range(NFM):
            cols = pl.ds(nb * 128, 128)
            gg = (g[nb] - mean * CSG[:, cols]) * rstd
            uu = (u[nb] - mean * CSU[:, cols]) * rstd
            hd.append(_dup(_swiglu(gg, uu)))
        return hd

    def down_mxu(hd, nb0, nb1, acc, first, marks):
        for nb in range(nb0, nb1):
            if first:
                w = wd_n[pl.ds(nb * 128, 128), :]
                for mb in range(5):
                    WDU[pl.ds((nb * 5 + mb) * 64, 64), :] = _u32(w[:, mb * 128:(mb + 1) * 128])
            else:
                w = jnp.concatenate(
                    [_bf(WDU[pl.ds((nb * 5 + mb) * 64, 64), :]) for mb in range(5)], axis=1)
            r = _dot(hd[nb], w)[0:8]
            acc = acc + r
            marks.append(((marks[-1][0] if marks else 0) + 5, r[:, 0:128]))
        return acc

    def ffn_vpu(x8, rstd, marks, nlate=0):
        acc = None
        xg = x8
        hcols = []
        half_rstd = 0.5 * rstd
        for g in range(NG):
            if g % cfg["gstep"] == 0:
                xg = gate(x8, marks, cfg["beta_n"] * (g - cfg["lag_n"]) / NG)
            rows = pl.ds(g * 8, 8)
            gc = jnp.sum(_lane_blocks_sum(GF[rows, :] * xg), axis=1, keepdims=True)
            uc = jnp.sum(_lane_blocks_sum(UF[rows, :] * xg), axis=1, keepdims=True)
            a = gc * half_rstd
            b = a * uc
            hc = b * jnp.tanh(a) + b
            if g >= NG - nlate:
                hcols.append(hc)
            else:
                t = DF[rows, :] * hc
                acc = t if acc is None else acc + t
        return acc, hcols

    def gate_scalar(xn, wr8):
        return jax.nn.sigmoid(jnp.sum(xn * wr8, axis=1, keepdims=True))

    ones_split = jnp.concatenate([jnp.ones((8, M), BF), jnp.zeros((8, M), BF)], axis=0)

    cx.wait()
    chunk_copy(NSEM - 2).start()
    cr.wait()
    chunk_copy(NSEM - 1).start()
    x = jnp.broadcast_to(x_s[0].astype(F32), (8, M))
    wr8 = jnp.broadcast_to(wr_s[...].reshape(1, M).astype(F32), (8, M))

    if not cfg["compute1"]:
        for i in range(NCH):
            wait(i)
        o_ref[0] = x[0:1].astype(BF)
        return

    for k, i in enumerate(idx("wq")):
        wait(i)
        with scope("p_wq"):
            repack(wq_n, WQ, SQ, k * 64, 64)
            vpu_transposes(WQ, SQ, k, WQT, NMF)
    with scope("s1_csq"):
        center_wqt()
    for k, i in enumerate(idx("wuk")):
        wait(i)
        with scope("p_wuk"):
            repack(wuk_n, UP, SV, k * 64, 64)
            prep_wuk_transpose(k)
            vpu_transposes(UP, SV, k, UTF, NMF)
    with scope("s1_csa"):
        front_mxu_qabs(front_mxu_q(ones_split, []), [])
        for cb in range(4):
            CSA[pl.ds(cb * H, NMF), :] = QAR[pl.ds(cb * H, NMF), :]
            CSA[pl.ds(cb * H + NMF, NVF), :] = jnp.zeros((NVF, 128), F32)
    with scope("s1_front"):
        mean, rstd = _ln_stats(x)
        front_mxu_qabs(front_mxu_q(_split(x), []), [])
        front_vpu(x, [])
        qa = finish_front(mean, rstd)
    for k, i in enumerate(idx("ckv")):
        wait(i)
        with scope("p_ckv"):
            prep_ckv(k * 8, 8)
    with scope("s1_attn"):
        stage_attn(qa)
    for k, i in enumerate(idx("wuv")):
        wait(i)
        with scope("p_wuv"):
            repack(wuv_n, UV, SV, k * 64, 64)
            vpu_transposes(UV, SV, k, UVT, NMB)
    with scope("s1_ctx"):
        ctx = ctx_mxu([])
    acc_v = jnp.zeros((8, M), F32)
    acc_m = jnp.zeros((8, M), F32)
    for i in idx("wo"):
        wait(i)
        h0, nh = CHUNKS[i][1], CHUNKS[i][2]
        with scope("s1_out"):
            if h0 >= NMB:
                unpack_wo(h0, nh)
                acc_v = back_vpu(h0, nh, acc_v, [])
            else:
                acc_m = out_mxu(ctx, h0, nh, acc_m, True, [])
    x = x + acc_m + _row_total(acc_v)
    for name, nat, tr, fl in (("wg", wg_n, GT, GF), ("wu", wu_n, UPT, UF)):
        for i in idx(name):
            wait(i)
            r0, n = CHUNKS[i][1], CHUNKS[i][2]
            with scope("p_" + name):
                if r0 >= FM:
                    unpack_rows(nat, r0, n, fl, True)
                else:
                    prep_ffn_mxu(nat, tr, r0, n)
    with scope("s2_cs"):
        g, u = gate_up_mxu_raw(ones_split, [])
        CSG[...] = jnp.concatenate(g, axis=1)
        CSU[...] = jnp.concatenate(u, axis=1)
    wd_idx = idx("wd")
    LATE = cfg["late"]
    wait(wd_idx[0])
    with scope("p_wd"):
        unpack_rows(wd_n, FM, F - FM - LATE, DF, False)
    with scope("s2_gu"):
        mean, rstd = _ln_stats(x)
        xn = (x - mean) * rstd
        hd = gate_up_mxu(_split(x), mean, rstd, [])
        acc_v, hcols = ffn_vpu(x, rstd, [], LATE // 8)
        sg = gate_scalar(xn, wr8)
    acc_m = jnp.zeros((8, M), F32)
    for i in wd_idx[1:]:
        wait(i)
        r0, n = CHUNKS[i][1], CHUNKS[i][2]
        with scope("s2_down"):
            if r0 < FM:
                acc_m = down_mxu(hd, r0 // 128, (r0 + n) // 128, acc_m, True, [])
            else:
                for j in range(n // 16):
                    v = wd_n[pl.ds(r0 + j * 16, 16), :].astype(F32)
                    DF[pl.ds(r0 - FM + j * 16, 16), :] = v
                    acc_v = acc_v + v[0:8] * hcols[2 * j] + v[8:16] * hcols[2 * j + 1]
    acc_m = acc_m + _row_total(acc_v) * rstd
    x = x + xn + acc_m * sg

    if cfg["phase2"]:
        with scope("phase2"):
            mean, rstd = _ln_stats(x)
            marks = []
            front_mxu_qabs(front_mxu_q(_split(x), marks), marks)
            front_vpu(x, marks if cfg["gate"] else [])
            stage_attn(finish_front(mean, rstd))
            marks = []
            ctx = ctx_mxu(marks)
            acc_m = out_mxu(ctx, 0, NMB, jnp.zeros((8, M), F32), False, marks)
            acc_v = back_vpu(NMB, NVB, jnp.zeros((8, M), F32), marks if cfg["gate"] else [])
            x = x + acc_m + _row_total(acc_v)
            mean, rstd = _ln_stats(x)
            xn = (x - mean) * rstd
            marks = []
            hd = gate_up_mxu(_split(x), mean, rstd, marks)
            y = down_mxu(hd, 0, NFM, jnp.zeros((8, M), F32), False, marks)
            acc_v, _ = ffn_vpu(x, rstd, marks if cfg["gate"] else [])
            sg = gate_scalar(xn, wr8)
            x = x + xn + (y + _row_total(acc_v) * rstd) * sg

    o_ref[0] = x[0:1].astype(BF)


def _run(cfg, A_x, A_c_kv, A_w_q, A_w_uk, A_w_uv, A_w_o, B_w_r, B_w_gate, B_w_up, B_w_down):
    any_spec = pl.BlockSpec(memory_space=pl.ANY)
    nmf, nmb = cfg["nmf"], cfg["nmb"]
    nvf, nvb = H - nmf, H - nmb
    fm = cfg["fm"]
    nsem = min(cfg["nsem"], len(_chunks(cfg)))
    scratch = [
        pltpu.VMEM((1, 1, M), BF),
        pltpu.VMEM((M,), BF),
        pltpu.VMEM((M, H, D), BF),
        pltpu.VMEM((DC, H, D), BF),
        pltpu.VMEM((DC, H, D), BF),
        pltpu.VMEM((SK, DC), BF),
        pltpu.VMEM((H, D, M), BF),
        pltpu.VMEM((F, M), BF),
        pltpu.VMEM((F, M), BF),
        pltpu.VMEM((F, M), BF),
        pltpu.VMEM(((H + 2) * SQ, 128), U32),
        pltpu.VMEM(((H + 2) * SV, 128), U32),
        pltpu.VMEM((4 * nmf * 64, 128), U32),
        pltpu.VMEM(((H + 2) * SV, 128), U32),
        pltpu.VMEM((32 * 4 * 64, 128), U32),
        pltpu.VMEM((4 * 2048, 128), U32),
        pltpu.VMEM((fm // 128 * 320, 128), U32),
        pltpu.VMEM((fm // 128 * 320, 128), U32),
        pltpu.VMEM((4 * H, 128), U32),
        pltpu.VMEM((nvf * 128, M), F32),
        pltpu.VMEM((nvf * 128, DC), F32),
        pltpu.VMEM((nvb * 128, DC), F32),
        pltpu.VMEM((nvb * 128, M), F32),
        pltpu.VMEM((F - fm, M), F32),
        pltpu.VMEM((F - fm, M), F32),
        pltpu.VMEM((F - fm, M), F32),
        pltpu.VMEM((4 * H, 128), F32),
        pltpu.VMEM((8, fm), F32),
        pltpu.VMEM((8, fm), F32),
        pltpu.VMEM((4 * H, 128), F32),
        pltpu.VMEM((4 * H, 128), F32),
        pltpu.VMEM(((4 * nvf + 2) * SP, 128), F32),
        pltpu.VMEM((nmb * 5 * 64, 128), U32),
        pltpu.VMEM((fm // 128 * 5 * 64, 128), U32),
        pltpu.VMEM((8, 128), jnp.int32),
        pltpu.SemaphoreType.DMA((nsem,)),
    ]
    return pl.pallas_call(
        functools.partial(_kernel, cfg),
        out_shape=jax.ShapeDtypeStruct((1, 1, M), BF),
        in_specs=[any_spec] * 10,
        out_specs=pl.BlockSpec(memory_space=pltpu.VMEM),
        scratch_shapes=scratch,
        compiler_params=pltpu.CompilerParams(vmem_limit_bytes=110 * 1024 * 1024),
    )(A_x, A_c_kv, A_w_q, A_w_uk, A_w_uv, A_w_o, B_w_r, B_w_gate.T, B_w_up.T, B_w_down)


def build(**overrides):
    cfg = dict(DEFAULT_CFG, **overrides)

    @jax.jit
    def fn(A_x, A_c_kv, A_w_q, A_w_uk, A_w_uv, A_w_o, B_x, B_w_r, B_w_gate, B_w_up, B_w_down):
        return _run(cfg, A_x, A_c_kv, A_w_q, A_w_uk, A_w_uv, A_w_o, B_w_r, B_w_gate, B_w_up, B_w_down)
    return fn


@jax.jit
def pallas_interleave_layers__compressed_kv_cla__moe_arch_mod__decode_kernel(
    A_x: jax.Array,
    A_c_kv: jax.Array,
    A_w_q: jax.Array,
    A_w_uk: jax.Array,
    A_w_uv: jax.Array,
    A_w_o: jax.Array,
    B_x: jax.Array,
    B_w_r: jax.Array,
    B_w_gate: jax.Array,
    B_w_up: jax.Array,
    B_w_down: jax.Array,
):
    del B_x
    return _run(DEFAULT_CFG, A_x, A_c_kv, A_w_q, A_w_uk, A_w_uv, A_w_o, B_w_r, B_w_gate, B_w_up,
                B_w_down)
```
